```python
import os as _os
_os.environ.setdefault('JAX_PLATFORMS', 'cpu')
import jax
import jax.numpy as jnp

def _softmax(x, axis=-1):
    return jax.nn.softmax(x, axis=axis)

def _gelu(x):
    return jax.nn.gelu(x, approximate=True)

def _silu(x):
    return jax.nn.silu(x)

def _sigmoid(x):
    return jax.nn.sigmoid(x)

def _layernorm(x, axis=-1, eps=1e-05):
    m = jnp.mean(x, axis=axis, keepdims=True)
    v = jnp.var(x, axis=axis, keepdims=True)
    return (x - m) / jnp.sqrt(v + eps)

def _scatter_add(tgt, idx, src, axis=0):
    return tgt.at[idx].add(src)

def _segment_sum(src, seg, n):
    return jax.ops.segment_sum(src, seg, n)

class _Rng:

    def __init__(self, key):
        self._k = key

    def _next(self):
        self._k, sub = jax.random.split(self._k)
        return sub

    def normal(self, shape):
        return jax.random.normal(self._next(), shape, dtype=jnp.bfloat16)

    def randint(self, lo, hi, shape):
        return jax.random.randint(self._next(), shape, lo, hi, dtype=jnp.int32)

    def uniform(self, shape, lo=0.0, hi=1.0):
        return jax.random.uniform(self._next(), shape, jnp.bfloat16, lo, hi)

    def permutation(self, n):
        return jax.random.permutation(self._next(), n)
kernel_name = 'adaLN_cond__grouped_kv_mqa__mixer_gmlp__prompt'

def setup_inputs():
    _rng = _Rng(jax.random.key(int.from_bytes(__import__("os").urandom(4), "little")))
    _w = lambda a: (lambda t: t.astype(jnp.bfloat16) if jnp.issubdtype(t.dtype, jnp.floating) else t)(jnp.asarray(a))

    def _A_setup():
        B, S, D, H = (1, 2048, 512, 32)
        Dh = D // H
        return {'x': _w((lambda *s: _rng.normal(s) * 0.05)(B, S, D)), 'wq': _w((lambda *s: _rng.normal(s) * 0.05)(D, H * Dh)), 'wk': _w((lambda *s: _rng.normal(s) * 0.05)(D, Dh)), 'wv': _w((lambda *s: _rng.normal(s) * 0.05)(D, Dh)), 'wo': _w((lambda *s: _rng.normal(s) * 0.05)(H * Dh, D))}
    _A_in = _A_setup()

    def _B_setup():
        B, S, D, F = (1, 2048, 512, 1792)
        Fh = F // 2
        return {'x': _w((lambda *s: _rng.normal(s) * 0.05)(B, S, D)), 'w_in': _w((lambda *s: _rng.normal(s) * 0.4)(D, 2 * Fh)), 'w_sp': _w(0.01 * (lambda *s: _rng.normal(s) * 0.4)(S, S)), 'b_sp': _w(1.0 + 0.01 * (lambda *s: _rng.normal(s) * 0.05)(S)), 'w_out': _w((lambda *s: _rng.normal(s) * 0.05)(Fh, D))}
    _B_in = _B_setup()
    return {'A_x': _A_in['x'], 'A_wq': _A_in['wq'], 'A_wk': _A_in['wk'], 'A_wv': _A_in['wv'], 'A_wo': _A_in['wo'], 'B_x': _B_in['x'], 'B_w_in': _B_in['w_in'], 'B_w_sp': _B_in['w_sp'], 'B_b_sp': _B_in['b_sp'], 'B_w_out': _B_in['w_out'], 'c': _w((lambda *s: _rng.normal(s) * 0.05)(1, 512) * 8.0), 'w_mod': _w((lambda *s: _rng.normal(s) * 0.05)(512, 6 * 512) * 512 ** (-0.5) * 8.0)}

def reference(A_x, A_wq, A_wk, A_wv, A_wo, B_x, B_w_in, B_w_sp, B_b_sp, B_w_out, c, w_mod):

    def _A_ref(x, wq, wk, wv, wo):
        B, S, D = x.shape
        H = 32
        Dh = D // H
        q = (lambda x, *d: x.transpose(*d))((x @ wq).reshape(B, S, H, Dh), 0, 2, 1, 3)
        k = x @ wk
        v = x @ wv
        scores = jnp.einsum('bhqd,bkd->bhqk', q, k) * Dh ** (-0.5)
        p = _softmax(scores, axis=-1)
        o = jnp.einsum('bhqk,bkd->bhqd', p, v)
        return (lambda x, *d: x.transpose(*d))(o, 0, 2, 1, 3).reshape(B, S, H * Dh) @ wo

    def _B_ref(x, w_in, w_sp, b_sp, w_out):
        B, S, D = x.shape
        F = w_in.shape[-1]
        Fh = F // 2
        z = _gelu(jnp.einsum('bsd,df->bsf', x, w_in))
        z1 = z[..., :Fh].copy()
        z2 = _layernorm(z[..., Fh:], axis=-1)
        g = jnp.einsum('ts,bsf->btf', w_sp, z2) + b_sp[None, :, None]
        return jnp.einsum('bsf,fd->bsd', z1 * g, w_out)
    x = A_x
    mod = (_silu(c) @ w_mod).reshape(c.shape[0], 6, 1, -1)
    sa, ca, ga, sb, cb, gb = (mod[:, 0].copy(), mod[:, 1].copy(), mod[:, 2].copy(), mod[:, 3].copy(), mod[:, 4].copy(), mod[:, 5].copy())
    h = _layernorm(x, axis=-1) * (1 + ca) + sa
    x = x + ga * _A_ref(h, A_wq, A_wk, A_wv, A_wo)
    h = _layernorm(x, axis=-1) * (1 + cb) + sb
    x = x + gb * _B_ref(h, B_w_in, B_w_sp, B_b_sp, B_w_out)
    return x
```

```python
import functools
import math

import jax
import jax.numpy as jnp
from jax import lax
from jax.experimental import pallas as pl
from jax.experimental.pallas import tpu as pltpu

BF = jnp.bfloat16
F32 = jnp.float32
S, D, H, DH, FH = 2048, 512, 32, 16, 896
EPS = 1e-5
QSCALE = DH ** -0.5 * math.log2(math.e)
NT = (((1,), (1,)), ((), ()))


def _ln(x):
    m = jnp.mean(x, axis=-1, keepdims=True)
    xc = x - m
    v = jnp.mean(xc * xc, axis=-1, keepdims=True)
    return xc * lax.rsqrt(v + EPS)


def _gelu(x):
    c = math.sqrt(2.0 / math.pi)
    return 0.5 * x * (1.0 + jnp.tanh(x * (c + (c * 0.044715) * (x * x))))


def build(QB=512, HU=4, CH=256, LA=2, RA=512, RC=256, RD=256):
    NQB = S // QB
    NCH = S // CH

    def kernel(x_hbm, wq_hbm, wk_hbm, wv_hbm, wo_hbm, win_hbm, wsp_hbm, bsp_hbm, wout_hbm, c_hbm, wmod_hbm,
               out_hbm,
               x_v, wq_v, wo_v, win_v, wsp_v, bsp_v, wout_v, c_v, wmod_v,
               wt_s, qt_s, k_s, vt_s, ot_s, x1_s, z1_s, z2_s, out_s, mod_s, bcol_s, sems, osems):
        NA = S // RA

        def cp(src, dst, i):
            return pltpu.make_async_copy(src, dst, sems.at[i])

        cp_c = cp(c_hbm, c_v, 0)
        cp_m0 = cp(wmod_hbm.at[:, pl.ds(0, 2 * D)], wmod_v.at[:, pl.ds(0, 2 * D)], 1)
        cp_m1 = cp(wmod_hbm.at[:, pl.ds(2 * D, 4 * D)], wmod_v.at[:, pl.ds(2 * D, 4 * D)], 2)
        cp_wq = cp(wq_hbm, wq_v, 3)
        cp_wk = cp(wk_hbm, wt_s.at[pl.ds(D, DH)], 4)
        cp_wv = cp(wv_hbm, wt_s.at[pl.ds(D + DH, DH)], 5)
        cp_wo = cp(wo_hbm, wo_v, 6)
        cp_win = cp(win_hbm, win_v, 7)
        cp_wsp = cp(wsp_hbm, wsp_v, 8)
        cp_bsp = cp(bsp_hbm, bsp_v, 9)
        cp_wout = cp(wout_hbm, wout_v, 10)
        cp_x = [cp(x_hbm.at[pl.ds(i * RA, RA)], x_v.at[pl.ds(i * RA, RA)], 11 + i) for i in range(NA)]

        cp_c.start()
        cp_wq.start()
        cp_wk.start()
        cp_wv.start()
        cp_m0.start()
        for c_ in cp_x:
            c_.start()

        cp_wq.wait()
        wt_s[0:D, :] = wq_v[...].astype(F32).T.astype(BF)
        cp_wk.wait()
        cp_wv.wait()

        cp_c.wait()
        cc = jnp.broadcast_to(c_v[...].astype(F32), (16, D))
        sc = (cc * jax.nn.sigmoid(cc)).astype(BF)
        cp_m0.wait()
        mod0 = jnp.dot(sc, wmod_v[:, 0:2 * D], preferred_element_type=F32)
        sa = mod0[0:1, 0:D]
        ca1 = 1.0 + mod0[0:1, D:2 * D]

        qmax = jnp.zeros((8, 128), F32)
        kmax = jnp.zeros((1, RA), F32)
        vmax = jnp.zeros((DH, RA), F32)
        for i in range(NA):
            cp_x[i].wait()
            if i == NA - 1:
                for c_ in (cp_m1, cp_wo, cp_win, cp_bsp, cp_wout, cp_wsp):
                    c_.start()
            rows = slice(i * RA, (i + 1) * RA)
            h = (_ln(x_v[rows, :].astype(F32)) * ca1 + sa).astype(BF)
            qkv = lax.dot_general(wt_s[...], h, NT, preferred_element_type=F32)
            qb = (qkv[0:D] * QSCALE).astype(BF)
            qt_s[:, rows] = qb
            kt = qkv[D:D + DH].astype(BF)
            vt = qkv[D + DH:D + 2 * DH].astype(BF)
            vt_s[:, rows] = vt
            ktf = kt.astype(F32)
            k_s[rows, :] = ktf.T.astype(BF)
            qf = qb.astype(F32)
            q2 = (qf * qf).reshape(H, 2, 8, RA)
            q2 = jnp.max(q2[:, 0] + q2[:, 1], axis=0)
            for j in range(RA // 128):
                qmax = jnp.maximum(qmax, q2[:, j * 128:(j + 1) * 128])
            kmax = jnp.maximum(kmax, jnp.sum(ktf * ktf, axis=0, keepdims=True))
            vmax = jnp.maximum(vmax, jnp.abs(vt.astype(F32)))
        bound2 = jnp.max(jnp.sum(qmax, axis=0, keepdims=True)) * jnp.max(kmax)
        vm = jnp.max(vmax)
        safe = (bound2 <= 60.0 * 60.0) & (vm <= 2.0 ** 40) & (vm >= 2.0 ** -40)

        @pl.when(safe)
        def _fast():
            def body(it, carry):
                qblk = it // (H // HU)
                h0 = (it % (H // HU)) * HU
                cols = pl.ds(pl.multiple_of(qblk * QB, QB), QB)
                items = [(hh, c) for hh in range(HU) for c in range(NCH)]
                qts, ls, accs, ps = {}, {}, {}, {}
                for t in range(len(items) + LA):
                    if t < len(items):
                        hh, c = items[t]
                        if c == 0:
                            qts[hh] = qt_s[pl.ds(pl.multiple_of((h0 + hh) * DH, DH), DH), cols]
                        s = jnp.dot(k_s[c * CH:(c + 1) * CH, :], qts[hh], preferred_element_type=F32)
                        e = jnp.exp2(s)
                        es = e.reshape(CH // 8, 8, QB).sum(axis=0)
                        ls[hh] = es if c == 0 else ls[hh] + es
                        ps[t] = e.astype(BF)
                    if t >= LA:
                        hh, c = items[t - LA]
                        pv = jnp.dot(vt_s[:, c * CH:(c + 1) * CH], ps.pop(t - LA), preferred_element_type=F32)
                        accs[hh] = pv if c == 0 else accs[hh] + pv
                        if c == NCH - 1:
                            l = ls[hh].sum(axis=0, keepdims=True)
                            ot_s[pl.ds(pl.multiple_of((h0 + hh) * DH, DH), DH), cols] = (
                                accs[hh] * (1.0 / l)).astype(BF)
                return carry

            lax.fori_loop(0, NQB * (H // HU), body, 0)

        @pl.when(jnp.logical_not(safe))
        def _true_max():
            def body(it, carry):
                qblk = it // H
                hh = it % H
                cols = pl.ds(pl.multiple_of(qblk * 128, 128), 128)
                hrows = pl.ds(pl.multiple_of(hh * DH, DH), DH)
                s = jnp.dot(k_s[...], qt_s[hrows, cols], preferred_element_type=F32)
                e = jnp.exp2(s - jnp.max(s, axis=0, keepdims=True))
                l = jnp.sum(e, axis=0, keepdims=True)
                o = jnp.dot(vt_s[...], e.astype(BF), preferred_element_type=F32)
                ot_s[hrows, cols] = (o * (1.0 / l)).astype(BF)
                return carry

            lax.fori_loop(0, (S // 128) * H, body, 0)

        cp_m1.wait()
        mod1 = jnp.dot(sc, wmod_v[:, 2 * D:6 * D], preferred_element_type=F32)
        mod_s[...] = mod1[0:8]
        cp_wo.wait()
        cp_win.wait()

        def body_c(i, carry):
            r0 = pl.multiple_of(i * RC, RC)
            rows = pl.ds(r0, RC)
            ga = mod_s[0:1, 0:D]
            sb = mod_s[0:1, D:2 * D]
            cb1 = 1.0 + mod_s[0:1, 2 * D:3 * D]
            o = ot_s[:, rows].astype(F32).T.astype(BF)
            a = jnp.dot(o, wo_v[...], preferred_element_type=F32)
            x1 = x_v[rows, :].astype(F32) + ga * a
            x1_s[rows, :] = x1
            h2 = (_ln(x1) * cb1 + sb).astype(BF)
            zb = _gelu(jnp.dot(h2, win_v[:, FH:2 * FH], preferred_element_type=F32))
            z2_s[rows, :] = _ln(zb).astype(BF)
            za = _gelu(jnp.dot(h2, win_v[:, 0:FH], preferred_element_type=F32))
            z1_s[rows, :] = za.astype(BF)
            return carry

        lax.fori_loop(0, S // RC, body_c, 0)

        cp_bsp.wait()
        bf = bsp_v[...].astype(F32)
        for r in range(S // 128):
            bcol_s[r * 128:(r + 1) * 128, :] = jnp.broadcast_to(bf[r:r + 1, :], (128, 128)).T
        cp_wout.wait()
        cp_wsp.wait()

        def out_cp(i):
            rows = pl.ds(pl.multiple_of(i * RD, RD), RD)
            return pltpu.make_async_copy(out_s.at[rows], out_hbm.at[rows], osems.at[i])

        def body_d(i, carry):
            r0 = pl.multiple_of(i * RD, RD)
            rows = pl.ds(r0, RD)
            gb = mod_s[0:1, 3 * D:4 * D]
            b = bcol_s[rows, :]
            g = jnp.dot(wsp_v[rows, :], z2_s[...], preferred_element_type=F32)
            g = g + jnp.concatenate([b] * (FH // 128), axis=1)
            y = (z1_s[rows, :].astype(F32) * g).astype(BF)
            o = jnp.dot(y, wout_v[...], preferred_element_type=F32)
            out_s[rows, :] = (x1_s[rows, :] + gb * o).astype(BF)
            out_cp(i).start()
            return carry

        lax.fori_loop(0, S // RD, body_d, 0)
        for i in range(S // RD):
            out_cp(i).wait()

    V = pltpu.VMEM
    scratch = [
        V((S, D), BF), V((D, D), BF), V((D, D), BF),
        V((D, 2 * FH), BF), V((S, S), BF), V((S // 128, 128), BF), V((FH, D), BF), V((1, D), BF), V((D, 6 * D), BF),
        V((D + 2 * DH, D), BF), V((D, S), BF), V((S, DH), BF), V((DH, S), BF), V((D, S), BF),
        V((S, D), F32), V((S, FH), BF), V((S, FH), BF), V((S, D), BF), V((8, 4 * D), F32), V((S, 128), F32),
        pltpu.SemaphoreType.DMA((11 + S // RA,)), pltpu.SemaphoreType.DMA((S // RD,)),
    ]

    def fn(A_x, A_wq, A_wk, A_wv, A_wo, B_x, B_w_in, B_w_sp, B_b_sp, B_w_out, c, w_mod):
        del B_x
        out = pl.pallas_call(
            kernel,
            out_shape=jax.ShapeDtypeStruct((S, D), BF),
            in_specs=[pl.BlockSpec(memory_space=pl.ANY)] * 11,
            out_specs=pl.BlockSpec(memory_space=pl.ANY),
            scratch_shapes=scratch,
            compiler_params=pltpu.CompilerParams(vmem_limit_bytes=100 * 1024 * 1024),
            name="fused",
        )(A_x.reshape(S, D), A_wq, A_wk.T, A_wv.T, A_wo, B_w_in, B_w_sp, B_b_sp.reshape(S // 128, 128), B_w_out, c, w_mod)
        return out.reshape(1, S, D)

    return fn


_fused = build()


@jax.jit
def pallas_adaLN_cond__grouped_kv_mqa__mixer_gmlp__prompt_kernel(
    A_x: jax.Array,
    A_wq: jax.Array,
    A_wk: jax.Array,
    A_wv: jax.Array,
    A_wo: jax.Array,
    B_x: jax.Array,
    B_w_in: jax.Array,
    B_w_sp: jax.Array,
    B_b_sp: jax.Array,
    B_w_out: jax.Array,
    c: jax.Array,
    w_mod: jax.Array,
):
    return _fused(A_x, A_wq, A_wk, A_wv, A_wo, B_x, B_w_in, B_w_sp, B_b_sp, B_w_out, c, w_mod)
```

```python
import math
from fractions import Fraction

import jax
import jax.numpy as jnp
from jax import lax
from jax.experimental import pallas as pl
from jax.experimental.pallas import tpu as pltpu

BF = jnp.bfloat16
F32 = jnp.float32
S, D, H, DH, FH = 2048, 512, 32, 16, 896
EPS = 1e-5
QSCALE = DH ** -0.5 * math.log2(math.e)
NT = (((1,), (1,)), ((), ()))

QB = 512
NJ = QB // 128
NU = (S // QB) * H
NTILE = S // 128
NFENCE = 512


def _ln(x):
    m = jnp.mean(x, axis=-1, keepdims=True)
    xc = x - m
    v = jnp.mean(xc * xc, axis=-1, keepdims=True)
    return xc * lax.rsqrt(v + EPS)


def _gelu(x):
    c = math.sqrt(2.0 / math.pi)
    return 0.5 * x * (1.0 + jnp.tanh(x * (c + (c * 0.044715) * (x * x))))


class _Attention:
    def __init__(self, hu, nv, dl, el, vl, vo, jb, fj, kl, qk, fl, mb):
        self.hu, self.nv, self.dl, self.el, self.vl = hu, nv, dl, el, vl
        self.jb, self.fj, self.kl, self.qk, self.fl = jb, fj, kl, qk, fl
        self.nm = nm = S // 16 - nv
        events = [(Fraction(m + 1), 0, "m", m) for m in range(nm)]
        events += [(Fraction((i + 1) * nm, nv) + vl + vo, 1, "v", i) for i in range(nv)]
        events.sort()
        self.tiles, self.tile_of, self.source = [], {}, {}
        for t in range(NTILE):
            part = events[8 * t:8 * t + 8]
            for pos, e in enumerate(part):
                self.tile_of[e[2:]] = (t, pos)
                self.source[8 * t + 7 - pos] = e[2:]
            self.tiles.append(([e[2:] for e in part], math.ceil(max(e[0] for e in part))))
        cuts = sorted({(end + dl) % nm for _, end in self.tiles})
        self.seam = (cuts[-1], cuts[0]) if mb and cuts[0] else None
        self.deferred = [t for t, (_, end) in enumerate(self.tiles) if end + dl >= nm]
        self.KB0 = 0
        self.QB0 = self.KB0 + nv * DH * 16
        self.VS0 = self.QB0 + 2 * DH * NJ * 8
        self.QS0 = self.VS0 + NTILE * 8
        self.QF0 = self.QS0 + NU * NJ * 8
        self.OT0 = self.QF0 + NU * NJ * DH
        self.PD0 = self.OT0 + NU * NJ * DH
        self.AD0 = self.PD0 + len(self.deferred) * 8 * NJ * 16
        self.LD0 = self.AD0 + NJ * DH
        self.PN0 = self.LD0 + NJ * 8
        self.J0 = self.PN0 + NJ * 8
        self.rows = -(-(self.J0 + (NFENCE + 2) * 8) // 32) * 32
        self.KX0 = nm * 8
        self.ks_rows = -(-(self.KX0 + 16 * 8) // 32) * 32

    def store_keys(self, wk, ks, group, kn16):
        kind, idx = self.source[group]
        if kind == "v":
            for d in range(DH):
                o = self.KB0 + (idx * DH + d) * 16
                wk[o:o + 16, :] = jnp.broadcast_to(kn16[:, d:d + 1], (16, 128))
            return
        ks[idx * 8:(idx + 1) * 8, :] = pltpu.bitcast(kn16.astype(BF), F32)
        if self.seam:
            a, b = self.seam
            if idx >= a:
                o = self.KX0 + (idx - a) * 8
                ks[o:o + 8, :] = pltpu.bitcast(kn16.astype(BF), F32)
            elif idx < b:
                o = self.KX0 + (self.nm - a + idx) * 8
                ks[o:o + 8, :] = pltpu.bitcast(pltpu.roll(kn16, DH, 1).astype(BF), F32)

    def _finish(self, wk, u, acc, lsum):
        l = jnp.concatenate(lsum, axis=1).sum(axis=0, keepdims=True)
        r = pltpu.reciprocal(l, approx=True)
        o = acc * (r * (2.0 - l * r))
        for j in range(NJ):
            wk[pl.ds(pl.multiple_of(self.OT0 + (u * NJ + j) * DH, DH), DH), :] = o[:, j * 128:(j + 1) * 128]

    def _pv(self, wk, t, p):
        vt = pltpu.bitcast(wk[self.VS0 + t * 8:self.VS0 + (t + 1) * 8, :], BF)
        return jnp.dot(vt, p.astype(BF), preferred_element_type=F32)

    def _pd(self, t, pos, j):
        return self.PD0 + ((self.deferred.index(t) * 8 + pos) * NJ + j) * 16

    def _load_pd(self, wk, t):
        return jnp.concatenate(
            [jnp.concatenate([wk[self._pd(t, pos, j):self._pd(t, pos, j) + 16, :] for j in range(NJ)], axis=1)
             for pos in range(7, -1, -1)], axis=0)

    def _load_acc(self, wk):
        return jnp.concatenate([wk[self.AD0 + j * DH:self.AD0 + (j + 1) * DH, :] for j in range(NJ)], axis=1)

    def _load_l(self, wk):
        return [wk[self.LD0 + j * 8:self.LD0 + (j + 1) * 8, :] for j in range(NJ)]

    def _qb_row(self, wk, u, h, d, j):
        r = wk[pl.ds(self.QF0 + (u * NJ + j) * DH + d, 1), :]
        return self.QB0 + (((h % 2) * DH + d) * NJ + j) * 8, jnp.broadcast_to(r, (8, 128))

    def run(self, wk, ks, zs, nrep=1):
        wk[self.PD0:self.LD0, :] = jnp.zeros((self.LD0 - self.PD0, 128), F32)
        wk[self.LD0:self.PN0, :] = jnp.ones((self.PN0 - self.LD0, 128), F32)
        for d in range(DH):
            for j in range(NJ):
                o, v = self._qb_row(wk, 0, 0, d, j)
                wk[o:o + 8, :] = v

        def body(it, carry):
            self._units(it, wk, ks, zs)
            return carry

        if nrep == 1:
            lax.fori_loop(0, NU // self.hu, body, 0)
        else:
            lax.fori_loop(0, nrep * NU // self.hu, lambda it, c: body(it % (NU // self.hu), c), 0)
        acc = self._load_acc(wk)
        for t in self.deferred:
            acc = acc + self._pv(wk, t, self._load_pd(wk, t))
        self._finish(wk, NU - 1, acc, self._load_l(wk))

    def _units(self, it, wk, ks, zs):
        hu, nv, nm, dl, el, vl, jb = self.hu, self.nv, self.nm, self.dl, self.el, self.vl, self.jb
        u0 = it * hu
        ngrp = hu * nm
        junk = pl.multiple_of(self.J0 + zs[0] * 8, 8)
        qts, ls, accs, es, ss, kls, qgen, first_pv = {}, {}, {}, {}, {}, {}, {}, {}
        pend, nfence = [], 0

        def load_q(h):
            b = self.QS0 + (u0 + h) * (NJ * 8)
            qts[h] = pltpu.bitcast(jnp.concatenate(
                [wk[pl.ds(pl.multiple_of(b + j * 8, 8), 8), :] for j in range(NJ)], axis=1), BF)

        def qb_ops(h):
            u = u0 + h if h < hu else jnp.minimum(u0 + h, NU - 1)
            for d in range(DH):
                for j in range(NJ):
                    pend.append(self._qb_row(wk, u, h, d, j))
                    yield

        def emit_p(h, key, j, s16):
            e = jnp.exp2(s16)
            e2 = e[0:8] + e[8:16]
            ls[h, j] = ls[h, j] + e2 if (h, j) in ls else e2
            t, pos = self.tile_of[key]
            if h == hu - 1 and t in self.deferred:
                wk[self._pd(t, pos, j):self._pd(t, pos, j) + 16, :] = e
            else:
                es[h, key, j] = e
            return e

        def vpu_ops():
            for h in range(hu):
                for vi in range(nv):
                    a = [None] * NJ
                    for j0 in range(0, NJ, jb):
                        for d in range(DH):
                            o = self.KB0 + (vi * DH + d) * 16
                            kk = wk[o:o + 16, :].reshape(2, 8, 128)
                            for j in range(j0, j0 + jb):
                                o = self.QB0 + (((h % 2) * DH + d) * NJ + j) * 8
                                pr = kk * wk[o:o + 8, :][None]
                                a[j] = pr if a[j] is None else a[j] + pr
                            if d == DH - 1:
                                for j in range(j0, j0 + jb):
                                    emit_p(h, ("v", vi), j, a[j].reshape(16, 128))
                            yield

        steps = DH * (NJ // jb)
        pv_at, fin_at, pin_at = {}, {}, {}
        for h in range(-1, hu):
            for t, (_, end) in enumerate(self.tiles):
                if (h == -1 and t not in self.deferred) or (h == hu - 1 and t in self.deferred):
                    continue
                x = h * nm + end + dl
                pv_at.setdefault(x, []).append((h, t))
                if t == NTILE - 1:
                    fin_at[x + self.fl] = h
                if t == 0:
                    pin_at[x + self.fl] = h
        cuts = {0, ngrp} | {x for x in pv_at if x < ngrp}
        if not self.seam:
            cuts |= {h * nm for h in range(hu)}
        cuts = sorted(cuts)
        runs = dict(zip(cuts[:-1], cuts[1:]))

        def load_k(a):
            h = a // nm
            if runs[a] > (h + 1) * nm:
                kls[a] = ks[self.KX0:self.KX0 + (runs[a] - a) * 8, :]
            else:
                kls[a] = ks[(a - h * nm) * 8:(runs[a] - h * nm) * 8, :]

        vgen, vdone = vpu_ops(), 0
        for x in range(-max(self.kl, self.qk), ngrp + dl + el + 32):
            if (x + self.qk) % nm == 0 and 0 <= (x + self.qk) // nm < hu:
                load_q((x + self.qk) // nm)
            if x + self.kl - el in runs:
                load_k(x + self.kl - el)
            for h, t in pv_at.get(x, []):
                if h == -1:
                    p = self._load_pd(wk, t)
                    if h not in accs:
                        accs[h] = self._load_acc(wk)
                else:
                    p = jnp.concatenate([jnp.concatenate([es.pop((h, key, j)) for j in range(NJ)], axis=1)
                                         for key in reversed(self.tiles[t][0])], axis=0)
                pv = self._pv(wk, t, p)
                accs[h] = pv if t == 0 else accs[h] + pv
                if t == 0:
                    first_pv[h] = pv
            if x in pin_at:
                for j in range(NJ):
                    wk[self.PN0 + j * 8:self.PN0 + (j + 1) * 8, :] = first_pv[pin_at[x]][0:8, j * 128:(j + 1) * 128]
            if x in fin_at:
                h = fin_at[x]
                if h == -1:
                    self._finish(wk, (u0 + NU - 1) % NU, accs[h], self._load_l(wk))
                else:
                    self._finish(wk, u0 + h, accs[h], [ls[h, j] for j in range(NJ)])
            if x in runs:
                if x not in kls:
                    load_k(x)
                h = x // nm
                keys = pltpu.bitcast(kls.pop(x), BF)
                if runs[x] > (h + 1) * nm:
                    s = jnp.dot(keys[:, 0:2 * DH], jnp.concatenate([qts[h], qts[h + 1]], axis=0),
                                preferred_element_type=F32)
                else:
                    s = jnp.dot(keys[:, 0:DH], qts[h], preferred_element_type=F32)
                for g in range(x, runs[x]):
                    ss[g] = s[(g - x) * 16:(g - x + 1) * 16]
            g = x - el
            if 0 <= g < ngrp:
                s = ss.pop(g)
                for j in range(NJ):
                    e = emit_p(g // nm, ("m", g % nm), j, s[:, j * 128:(j + 1) * 128])
                    if j == self.fj:
                        pace = e[8:16]
                for o, v in pend:
                    wk[o:o + 8, :] = v
                pend.clear()
                nfence += 1
                wk[pl.ds(pl.multiple_of(junk + 8 * (nfence % NFENCE), 8), 8), :] = pace
            hq = (x + nm - 14) // nm
            if 1 <= hq <= hu:
                if hq not in qgen:
                    qgen[hq] = qb_ops(hq)
                next(qgen[hq], None)
            want = min(max(0, ((x - el - vl + 1) * nv * steps) // nm), hu * nv * steps)
            while vdone < want:
                next(vgen)
                vdone += 1
        for j in range(NJ):
            wk[self.AD0 + j * DH:self.AD0 + (j + 1) * DH, :] = accs[hu - 1][:, j * 128:(j + 1) * 128]
            wk[self.LD0 + j * 8:self.LD0 + (j + 1) * 8, :] = ls[hu - 1, j]
        assert not es and not ss and not pend


def build(HU=8, RA=256, RC=256, RD=256, UD=2, PB=(1, 3, 7), NREP=1, STOP=9,
          nv=16, dl=10, el=10, vl=-3, vo=2, jb=2, fj=3, kl=8, qk=9, fl=10, mb=1):
    att = _Attention(HU, nv, dl, el, vl, vo, jb, fj, kl, qk, fl, mb)

    def kernel(x_hbm, wq_hbm, wk_hbm, wv_hbm, wo_hbm, win_hbm, wsp_hbm, bsp_hbm, wout_hbm, c_hbm, wmod_hbm,
               out_hbm,
               wk, ks, x_v, wq_v, wo_v, win_v, wsp_v, wout_v, wmod_v, wt_s, k_s, x1_s, z1_s, z2_s, out_s,
               mod_s, bcol_s, bsp_v, c_v, zs, sems, osems):
        NA = S // RA

        def cp(src, dst, i):
            return pltpu.make_async_copy(src, dst, sems.at[i])

        cp_c = cp(c_hbm, c_v, 0)
        cp_m0 = cp(wmod_hbm.at[:, pl.ds(0, 2 * D)], wmod_v.at[:, pl.ds(0, 2 * D)], 1)
        cp_m1 = cp(wmod_hbm.at[:, pl.ds(2 * D, 4 * D)], wmod_v.at[:, pl.ds(2 * D, 4 * D)], 2)
        cp_wq = cp(wq_hbm, wq_v, 3)
        cp_wk = cp(wk_hbm, wt_s.at[pl.ds(D, DH)], 4)
        cp_wv = cp(wv_hbm, wt_s.at[pl.ds(D + DH, DH)], 5)
        cp_wo = cp(wo_hbm, wo_v, 6)
        cp_win = cp(win_hbm, win_v, 7)
        cp_wsp = cp(wsp_hbm, wsp_v, 8)
        cp_bsp = cp(bsp_hbm, bsp_v, 9)
        cp_wout = cp(wout_hbm, wout_v, 10)
        cp_x = [cp(x_hbm.at[pl.ds(i * RA, RA)], x_v.at[pl.ds(i * RA, RA)], 11 + i) for i in range(NA)]

        for c_ in (cp_wq, cp_c, cp_wk, cp_wv, cp_m0, *cp_x):
            c_.start()

        cp_wq.wait()
        wt_s[0:D, :] = wq_v[...].astype(F32).T.astype(BF)
        cp_wk.wait()
        cp_wv.wait()

        cp_c.wait()
        cc = jnp.broadcast_to(c_v[...].astype(F32), (16, D))
        sc = (cc * jax.nn.sigmoid(cc)).astype(BF)
        cp_m0.wait()
        mod0 = jnp.dot(sc, wmod_v[:, 0:2 * D], preferred_element_type=F32)
        sa = mod0[0:1, 0:D]
        ca1 = 1.0 + mod0[0:1, D:2 * D]

        def norm1(i):
            return (_ln(x_v[i * RA:(i + 1) * RA, :].astype(F32)) * ca1 + sa).astype(BF)

        def project(i, h, stats):
            qmax, kmax, vmax = stats
            kvt = lax.dot_general(wt_s[D:D + 2 * DH, :], h, NT, preferred_element_type=F32)
            qt = lax.dot_general(wt_s[0:D, :], h, NT, preferred_element_type=F32)
            kt = kvt[0:DH].astype(BF).astype(F32)
            vt = kvt[DH:2 * DH].astype(BF)
            vw = pltpu.bitcast(vt, F32)
            kn = jnp.concatenate([kt, jnp.zeros((128 - DH, RA), F32)], axis=0).T
            k_s[i * RA:(i + 1) * RA, :] = kn[:, 0:DH].astype(BF)
            for g in range(RA // 16):
                att.store_keys(wk, ks, i * (RA // 16) + g, kn[g * 16:(g + 1) * 16, :])
            qb = (qt * QSCALE).astype(BF)
            qf = qb.astype(F32)
            qw = pltpu.bitcast(qb, F32)
            for jj in range(RA // 128):
                c = i * (RA // 128) + jj
                blk, j = divmod(c, NJ)
                lanes = slice(jj * 128, (jj + 1) * 128)
                wk[att.VS0 + c * 8:att.VS0 + (c + 1) * 8, :] = vw[:, lanes]
                for hh in range(H):
                    r = (blk * H + hh) * NJ + j
                    wk[att.QS0 + r * 8:att.QS0 + (r + 1) * 8, :] = qw[hh * 8:(hh + 1) * 8, lanes]
                    wk[att.QF0 + r * DH:att.QF0 + (r + 1) * DH, :] = qf[hh * DH:(hh + 1) * DH, lanes]
            q2 = (qf * qf).reshape(H, 2, 8, RA)
            q2 = jnp.max(q2[:, 0] + q2[:, 1], axis=0)
            for j in range(RA // 128):
                qmax = jnp.maximum(qmax, q2[:, j * 128:(j + 1) * 128])
            kmax = jnp.maximum(kmax, jnp.sum(kt * kt, axis=0, keepdims=True))
            vmax = jnp.maximum(vmax, jnp.abs(vt.astype(F32)))
            return qmax, kmax, vmax

        stats = (jnp.zeros((8, 128), F32), jnp.zeros((1, RA), F32), jnp.zeros((DH, RA), F32))
        waited = 0
        hs = {}
        for n, upto in enumerate(PB):
            while waited <= upto:
                cp_x[waited].wait()
                waited += 1
            if waited == NA:
                for c_ in (cp_m1, cp_wo, cp_win, cp_bsp, cp_wout, cp_wsp):
                    c_.start()
            lo = 0 if n == 0 else PB[n - 1]
            hi = NA if n == len(PB) - 1 else upto
            for i in range(lo, hi):
                for i2 in (i, i + 1):
                    if i2 < waited and i2 not in hs:
                        hs[i2] = norm1(i2)
                stats = project(i, hs[i], stats)
        qmax, kmax, vmax = stats
        bound2 = jnp.max(jnp.sum(qmax, axis=0, keepdims=True)) * jnp.max(kmax)
        vm = jnp.max(vmax)
        safe = (bound2 <= 60.0 * 60.0) & (vm <= 2.0 ** 40) & (vm >= 2.0 ** -40)
        zs[0] = jnp.where(safe, 0, 1)

        @pl.when(safe)
        def _fast():
            att.run(wk, ks, zs, NREP)

        @pl.when(jnp.logical_not(safe))
        def _true_max():
            def body(it, carry):
                q = pltpu.bitcast(wk[pl.ds(pl.multiple_of(att.QS0 + it * 8, 8), 8), :], BF)
                s = jnp.dot(k_s[...], q, preferred_element_type=F32)
                e = jnp.exp2(s - jnp.max(s, axis=0, keepdims=True))
                l = jnp.sum(e, axis=0, keepdims=True)
                vt = pltpu.bitcast(jnp.concatenate(
                    [wk[att.VS0 + c * 8:att.VS0 + (c + 1) * 8, :] for c in range(NTILE)], axis=1), BF)
                o = jnp.dot(vt, e.astype(BF), preferred_element_type=F32)
                wk[pl.ds(pl.multiple_of(att.OT0 + it * DH, DH), DH), :] = o * (1.0 / l)
                return carry

            lax.fori_loop(0, NU * NJ, body, 0)

        for c_ in (cp_m1, cp_wo, cp_win, cp_bsp):
            c_.wait()
        mod1 = jnp.dot(sc, wmod_v[:, 2 * D:6 * D], preferred_element_type=F32)
        mod_s[...] = mod1[0:8, 3 * D:4 * D]
        ga = mod1[0:1, 0:D]
        sb = mod1[0:1, D:2 * D]
        cb1 = 1.0 + mod1[0:1, 2 * D:3 * D]

        def mix_in(i):
            rows = slice(i * RC, (i + 1) * RC)
            cols = []
            for c in range(i * (RC // 128), (i + 1) * (RC // 128)):
                blk, j = divmod(c, NJ)
                cols.append(jnp.concatenate(
                    [wk[att.OT0 + ((blk * H + hh) * NJ + j) * DH:att.OT0 + ((blk * H + hh) * NJ + j + 1) * DH, :]
                     for hh in range(H)], axis=0).T)
            o = jnp.concatenate(cols, axis=0).astype(BF)
            a = jnp.dot(o, wo_v[...], preferred_element_type=F32)
            x1 = x_v[rows, :].astype(F32) + ga * a
            x1_s[rows, :] = x1
            return (_ln(x1) * cb1 + sb).astype(BF)

        def mlp_in(i, h2):
            rows = slice(i * RC, (i + 1) * RC)
            zb = _gelu(jnp.dot(h2, win_v[:, FH:2 * FH], preferred_element_type=F32))
            z2_s[rows, :] = _ln(zb).astype(BF)
            za = _gelu(jnp.dot(h2, win_v[:, 0:FH], preferred_element_type=F32))
            z1_s[rows, :] = za.astype(BF)

        h2 = mix_in(0)
        for i in range(S // RC if STOP >= 2 else 0):
            h2_next = mix_in(i + 1) if i + 1 < S // RC else None
            mlp_in(i, h2)
            h2 = h2_next
        bf = bsp_v[...].astype(F32)
        for r in range(S // 128):
            bcol_s[r * 128:(r + 1) * 128, :] = jnp.broadcast_to(bf[r:r + 1, :], (128, 128)).T

        cp_wout.wait()
        cp_wsp.wait()

        def out_cp(i):
            rows = pl.ds(pl.multiple_of(i * RD, RD), RD)
            return pltpu.make_async_copy(out_s.at[rows], out_hbm.at[rows], osems.at[i])

        def gate(i):
            rows = pl.ds(pl.multiple_of(i * RD, RD), RD)
            g = jnp.dot(wsp_v[rows, :], z2_s[...], preferred_element_type=F32)
            g = g + jnp.concatenate([bcol_s[rows, :]] * (FH // 128), axis=1)
            return (z1_s[rows, :].astype(F32) * g).astype(BF)

        def project_out(i, y):
            rows = pl.ds(pl.multiple_of(i * RD, RD), RD)
            o = jnp.dot(y, wout_v[...], preferred_element_type=F32)
            out_s[rows, :] = (x1_s[rows, :] + mod_s[0:1, :] * o).astype(BF)

        def body_d(it, carry):
            ys = [gate(it * UD + u) for u in range(UD)]
            for u in range(UD):
                project_out(it * UD + u, ys[u])
            for u in range(UD):
                out_cp(it * UD + u).start()
            return carry

        if STOP >= 3:
            lax.fori_loop(0, S // RD // UD, body_d, 0)
        else:
            for i in range(S // RD):
                out_cp(i).start()
        for i in range(S // RD):
            out_cp(i).wait()

    V = pltpu.VMEM
    scratch = [
        V((att.rows, 128), F32), V((att.ks_rows, 128), F32),
        V((S, D), BF), V((D, D), BF), V((D, D), BF), V((D, 2 * FH), BF), V((S, S), BF), V((FH, D), BF),
        V((D, 6 * D), BF), V((D + 2 * DH, D), BF), V((S, DH), BF),
        V((S, D), F32), V((S, FH), BF), V((S, FH), BF), V((S, D), BF), V((8, D), F32), V((S, 128), F32),
        V((S // 128, 128), BF), V((1, D), BF),
        pltpu.SMEM((1,), jnp.int32),
        pltpu.SemaphoreType.DMA((11 + S // RA,)), pltpu.SemaphoreType.DMA((S // RD,)),
    ]

    def fn(A_x, A_wq, A_wk, A_wv, A_wo, B_x, B_w_in, B_w_sp, B_b_sp, B_w_out, c, w_mod):
        del B_x
        out = pl.pallas_call(
            kernel,
            out_shape=jax.ShapeDtypeStruct((S, D), BF),
            in_specs=[pl.BlockSpec(memory_space=pl.ANY)] * 11,
            out_specs=pl.BlockSpec(memory_space=pl.ANY),
            scratch_shapes=scratch,
            compiler_params=pltpu.CompilerParams(vmem_limit_bytes=100 * 1024 * 1024),
            name="fused",
        )(A_x.reshape(S, D), A_wq, A_wk.T, A_wv.T, A_wo, B_w_in, B_w_sp, B_b_sp.reshape(S // 128, 128),
          B_w_out, c, w_mod)
        return out.reshape(1, S, D)

    return fn


_fused = build()


@jax.jit
def pallas_adaLN_cond__grouped_kv_mqa__mixer_gmlp__prompt_kernel(
    A_x: jax.Array,
    A_wq: jax.Array,
    A_wk: jax.Array,
    A_wv: jax.Array,
    A_wo: jax.Array,
    B_x: jax.Array,
    B_w_in: jax.Array,
    B_w_sp: jax.Array,
    B_b_sp: jax.Array,
    B_w_out: jax.Array,
    c: jax.Array,
    w_mod: jax.Array,
):
    return _fused(A_x, A_wq, A_wk, A_wv, A_wo, B_x, B_w_in, B_w_sp, B_b_sp, B_w_out, c, w_mod)
```

```python
import math
from fractions import Fraction

import jax
import jax.numpy as jnp
from jax import lax
from jax.experimental import pallas as pl
from jax.experimental.pallas import tpu as pltpu

BF = jnp.bfloat16
F32 = jnp.float32
S, D, H, DH, FH = 2048, 512, 32, 16, 896
EPS = 1e-5
QSCALE = DH ** -0.5 * math.log2(math.e)
NT = (((1,), (1,)), ((), ()))

QB = 512
NJ = QB // 128
NU = (S // QB) * H
NTILE = S // 128
NFENCE = 512


def _ln(x):
    m = jnp.mean(x, axis=-1, keepdims=True)
    xc = x - m
    v = jnp.mean(xc * xc, axis=-1, keepdims=True)
    return xc * lax.rsqrt(v + EPS)


def _gelu(x):
    c = math.sqrt(2.0 / math.pi)
    return 0.5 * x * (1.0 + jnp.tanh(x * (c + (c * 0.044715) * (x * x))))


class _Attention:
    def __init__(self, hu, nv, dl, el, vl, vo, jb, fj, kl, qk, fl, mb, pt=1, dd=0):
        self.hu, self.nv, self.dl, self.el, self.vl = hu, nv, dl, el, vl
        self.jb, self.fj, self.kl, self.qk, self.fl, self.pt = jb, fj, kl, qk, fl, pt
        self.nm = nm = S // 16 - nv
        events = [(Fraction(m + 1), 0, "m", m) for m in range(nm)]
        events += [(Fraction((i + 1) * nm, nv) + vl + vo, 1, "v", i) for i in range(nv)]
        events.sort()
        self.tiles, self.tile_of, self.source = [], {}, {}
        for t in range(NTILE):
            part = events[8 * t:8 * t + 8]
            for pos, e in enumerate(part):
                self.tile_of[e[2:]] = (t, pos)
                self.source[8 * t + 7 - pos] = e[2:]
            self.tiles.append(([e[2:] for e in part], math.ceil(max(e[0] for e in part))))
        cuts = sorted({(end + dl) % nm for _, end in self.tiles})
        self.seam = (cuts[-1], cuts[0]) if mb and cuts[0] else None
        self.deferred = [t for t, (_, end) in enumerate(self.tiles) if end + dl >= nm + dd]
        self.KB0 = 0
        self.QB0 = self.KB0 + nv * DH * 16
        self.QF0 = self.QB0 + 2 * DH * NJ * 8
        self.OT0 = self.QF0 + NU * NJ * DH
        self.PD0 = self.OT0 + NU * NJ * DH
        self.AD0 = self.PD0 + len(self.deferred) * 8 * NJ * 16
        self.LD0 = self.AD0 + NJ * DH
        self.PN0 = self.LD0 + NJ * 8
        self.J0 = self.PN0 + NJ * 8
        self.rows = -(-(self.J0 + (NFENCE + 2) * 8) // 32) * 32
        self.KX0 = nm * 8
        self.VS0 = self.KX0 + 16 * 8
        self.QS0 = self.VS0 + NTILE * 8
        self.ks_rows = -(-(self.QS0 + NU * NJ * 8) // 32) * 32

    def store_keys(self, wk, ks, group, kn16):
        kind, idx = self.source[group]
        if kind == "v":
            for d in range(DH):
                o = self.KB0 + (idx * DH + d) * 16
                wk[o:o + 16, :] = jnp.broadcast_to(kn16[:, d:d + 1], (16, 128))
            return
        ks[idx * 8:(idx + 1) * 8, :] = pltpu.bitcast(kn16.astype(BF), F32)
        if self.seam:
            a, b = self.seam
            if idx >= a:
                o = self.KX0 + (idx - a) * 8
                ks[o:o + 8, :] = pltpu.bitcast(kn16.astype(BF), F32)
            elif idx < b:
                o = self.KX0 + (self.nm - a + idx) * 8
                ks[o:o + 8, :] = pltpu.bitcast(pltpu.roll(kn16, DH, 1).astype(BF), F32)

    def _finish(self, wk, u, acc, lsum):
        l = jnp.concatenate(lsum, axis=1).sum(axis=0, keepdims=True)
        r = pltpu.reciprocal(l, approx=True)
        o = acc * (r * (2.0 - l * r))
        for j in range(NJ):
            wk[pl.ds(pl.multiple_of(self.OT0 + (u * NJ + j) * DH, DH), DH), :] = o[:, j * 128:(j + 1) * 128]

    def _pv(self, ks, t, p):
        vt = pltpu.bitcast(ks[self.VS0 + t * 8:self.VS0 + (t + 1) * 8, :], BF)
        return jnp.dot(vt, p.astype(BF), preferred_element_type=F32)

    def _pd(self, t, pos, j):
        return self.PD0 + ((self.deferred.index(t) * 8 + pos) * NJ + j) * 16

    def _load_pd(self, wk, t):
        return jnp.concatenate(
            [jnp.concatenate([wk[self._pd(t, pos, j):self._pd(t, pos, j) + 16, :] for j in range(NJ)], axis=1)
             for pos in range(7, -1, -1)], axis=0)

    def _load_acc(self, wk):
        return jnp.concatenate([wk[self.AD0 + j * DH:self.AD0 + (j + 1) * DH, :] for j in range(NJ)], axis=1)

    def _load_l(self, wk):
        return [wk[self.LD0 + j * 8:self.LD0 + (j + 1) * 8, :] for j in range(NJ)]

    def _qb_row(self, wk, u, h, d, j):
        r = wk[pl.ds(self.QF0 + (u * NJ + j) * DH + d, 1), :]
        return self.QB0 + (((h % 2) * DH + d) * NJ + j) * 8, jnp.broadcast_to(r, (8, 128))

    def run(self, wk, ks, zs, nrep=1):
        wk[self.PD0:self.LD0, :] = jnp.zeros((self.LD0 - self.PD0, 128), F32)
        wk[self.LD0:self.PN0, :] = jnp.ones((self.PN0 - self.LD0, 128), F32)
        for d in range(DH):
            for j in range(NJ):
                o, v = self._qb_row(wk, 0, 0, d, j)
                wk[o:o + 8, :] = v

        def body(it, carry):
            self._units(it, wk, ks, zs)
            return carry

        if nrep == 1:
            lax.fori_loop(0, NU // self.hu, body, 0)
        else:
            lax.fori_loop(0, nrep * NU // self.hu, lambda it, c: body(it % (NU // self.hu), c), 0)
        acc = self._load_acc(wk)
        for t in self.deferred:
            acc = acc + self._pv(ks, t, self._load_pd(wk, t))
        self._finish(wk, NU - 1, acc, self._load_l(wk))

    def _units(self, it, wk, ks, zs):
        hu, nv, nm, dl, el, vl, jb = self.hu, self.nv, self.nm, self.dl, self.el, self.vl, self.jb
        u0 = it * hu
        ngrp = hu * nm
        junk = pl.multiple_of(self.J0 + zs[0] * 8, 8)
        qts, ls, accs, es, ss, kls, qgen, first_pv = {}, {}, {}, {}, {}, {}, {}, {}
        pend, nfence = [], 0

        def load_q(h):
            b = self.QS0 + (u0 + h) * (NJ * 8)
            qts[h] = pltpu.bitcast(jnp.concatenate(
                [ks[pl.ds(pl.multiple_of(b + j * 8, 8), 8), :] for j in range(NJ)], axis=1), BF)

        def qb_ops(h):
            u = u0 + h if h < hu else jnp.minimum(u0 + h, NU - 1)
            for d in range(DH):
                for j in range(NJ):
                    pend.append(self._qb_row(wk, u, h, d, j))
                    yield

        def emit_p(h, key, j, s16):
            e = jnp.exp2(s16)
            e2 = e[0:8] + e[8:16]
            ls[h, j] = ls[h, j] + e2 if (h, j) in ls else e2
            t, pos = self.tile_of[key]
            if h == hu - 1 and t in self.deferred:
                wk[self._pd(t, pos, j):self._pd(t, pos, j) + 16, :] = e
            else:
                es[h, key, j] = e
            return e

        def vpu_ops():
            for h in range(hu):
                for vi in range(nv):
                    a = [None] * NJ
                    for j0 in range(0, NJ, jb):
                        for d in range(DH):
                            o = self.KB0 + (vi * DH + d) * 16
                            kk = wk[o:o + 16, :].reshape(2, 8, 128)
                            for j in range(j0, j0 + jb):
                                o = self.QB0 + (((h % 2) * DH + d) * NJ + j) * 8
                                pr = kk * wk[o:o + 8, :][None]
                                a[j] = pr if a[j] is None else a[j] + pr
                            if d == DH - 1:
                                for j in range(j0, j0 + jb):
                                    emit_p(h, ("v", vi), j, a[j].reshape(16, 128))
                            yield

        steps = DH * (NJ // jb)
        pv_at, fin_at, pin_at = {}, {}, {}
        for h in range(-1, hu):
            for t, (_, end) in enumerate(self.tiles):
                if (h == -1 and t not in self.deferred) or (h == hu - 1 and t in self.deferred):
                    continue
                x = h * nm + end + dl
                pv_at.setdefault(x, []).append((h, t))
                if t == NTILE - 1:
                    fin_at[x + self.fl] = h
                if t == 0:
                    pin_at[x + self.fl] = h
        cuts = {0, ngrp} | {x for x in pv_at if x < ngrp}
        if not self.seam:
            cuts |= {h * nm for h in range(hu)}
        cuts = sorted(cuts)
        runs = dict(zip(cuts[:-1], cuts[1:]))

        def load_k(a):
            h = a // nm
            if runs[a] > (h + 1) * nm:
                kls[a] = ks[self.KX0:self.KX0 + (runs[a] - a) * 8, :]
            else:
                kls[a] = ks[(a - h * nm) * 8:(runs[a] - h * nm) * 8, :]

        vgen = vpu_ops()
        state = dict(vdone=0, nfence=0)
        pv_before = {}
        for x in pv_at:
            pv_before[x] = len(pv_at[x])

        def ticks(g):
            h, r = divmod(g, nm)
            return h * (nm + NTILE) + r + 1 + sum(1 for _, end in self.tiles if (end + dl) % nm <= r)

        def fence(value):
            for o, v in pend:
                wk[o:o + 8, :] = v
            pend.clear()
            state["nfence"] += 1
            wk[pl.ds(pl.multiple_of(junk + 8 * (state["nfence"] % NFENCE), 8), 8), :] = value

        def advance(want):
            while state["vdone"] < min(want, hu * nv * steps):
                next(vgen)
                state["vdone"] += 1

        pv_results = {}
        for x in range(-max(self.kl, self.qk), ngrp + dl + el + 32):
            if (x + self.qk) % nm == 0 and 0 <= (x + self.qk) // nm < hu:
                load_q((x + self.qk) // nm)
            if x + self.kl - el in runs:
                load_k(x + self.kl - el)
            for h, t in pv_at.get(x, []):
                if h == -1:
                    p = self._load_pd(wk, t)
                    if h not in accs:
                        accs[h] = self._load_acc(wk)
                else:
                    p = jnp.concatenate([jnp.concatenate([es.pop((h, key, j)) for j in range(NJ)], axis=1)
                                         for key in reversed(self.tiles[t][0])], axis=0)
                pv = self._pv(ks, t, p)
                pv_results.setdefault(x, []).append(pv)
                accs[h] = pv if t == 0 else accs[h] + pv
                if t == 0:
                    first_pv[h] = pv
            if x in pin_at:
                for j in range(NJ):
                    wk[self.PN0 + j * 8:self.PN0 + (j + 1) * 8, :] = first_pv[pin_at[x]][0:8, j * 128:(j + 1) * 128]
            if x in fin_at:
                h = fin_at[x]
                if h == -1:
                    self._finish(wk, (u0 + NU - 1) % NU, accs[h], self._load_l(wk))
                else:
                    self._finish(wk, u0 + h, accs[h], [ls[h, j] for j in range(NJ)])
            if x in runs:
                if x not in kls:
                    load_k(x)
                h = x // nm
                keys = pltpu.bitcast(kls.pop(x), BF)
                if runs[x] > (h + 1) * nm:
                    s = jnp.dot(keys[:, 0:2 * DH], jnp.concatenate([qts[h], qts[h + 1]], axis=0),
                                preferred_element_type=F32)
                else:
                    s = jnp.dot(keys[:, 0:DH], qts[h], preferred_element_type=F32)
                for g in range(x, runs[x]):
                    ss[g] = s[(g - x) * 16:(g - x + 1) * 16]
            g = x - el
            if self.pt and 0 <= g < ngrp and g in pv_results:
                fence(pv_results[g][-1][8:16, self.fj * 128:(self.fj + 1) * 128])
                advance(((ticks(g) - 1 - vl) * nv * steps) // (nm + NTILE))
            if 0 <= g < ngrp:
                s = ss.pop(g)
                for j in range(NJ):
                    e = emit_p(g // nm, ("m", g % nm), j, s[:, j * 128:(j + 1) * 128])
                    if j == self.fj:
                        pace = e[8:16]
                fence(pace)
            hq = (x + nm - 14) // nm
            if 1 <= hq <= hu:
                if hq not in qgen:
                    qgen[hq] = qb_ops(hq)
                next(qgen[hq], None)
            if self.pt:
                advance(((ticks(g) - vl) * nv * steps) // (nm + NTILE))
            else:
                advance(((g - vl + 1) * nv * steps) // nm)
        for j in range(NJ):
            wk[self.AD0 + j * DH:self.AD0 + (j + 1) * DH, :] = accs[hu - 1][:, j * 128:(j + 1) * 128]
            wk[self.LD0 + j * 8:self.LD0 + (j + 1) * 8, :] = ls[hu - 1, j]
        assert not es and not ss and not pend


def build(HU=8, RA=256, RC=128, RD=128, UD=4, PB=(1, 3, 7), NREP=1, STOP=9, PIN=1, EARLY=1, DORD='qckv0m1234567', NPRE=1, MSPLIT=2, MODP=0, DFULL=0, dd=0,
          nv=16, dl=9, el=9, vl=-3, vo=1, jb=2, fj=3, kl=8, qk=9, fl=10, mb=1, pt=0):
    att = _Attention(HU, nv, dl, el, vl, vo, jb, fj, kl, qk, fl, mb, pt, dd)

    def kernel(x_hbm, wq_hbm, wk_hbm, wv_hbm, wo_hbm, win_hbm, wsp_hbm, bsp_hbm, wout_hbm, c_hbm, wmod_hbm,
               out_hbm,
               wk, ks, xz, wq_v, wo_v, win_v, wsp_v, wout_v, wmod_v, wt_s, k_s, x1_s, out_s,
               mod_s, bcol_s, bsp_v, c_v, zs, sems, osems):
        NA = S // RA

        def cp(src, dst, i):
            return pltpu.make_async_copy(src, dst, sems.at[i])

        cp_c = cp(c_hbm, c_v, 0)
        cp_m1 = cp(wmod_hbm.at[:, pl.ds(2 * D, 4 * D)], wmod_v.at[:, pl.ds(2 * D, 4 * D)], 2)
        cp_wq = cp(wq_hbm, wq_v, 3)
        cp_wk = cp(wk_hbm, wt_s.at[pl.ds(D, DH)], 4)
        cp_wv = cp(wv_hbm, wt_s.at[pl.ds(D + DH, DH)], 5)
        cp_wo = cp(wo_hbm, wo_v, 6)
        cp_win = cp(win_hbm, win_v, 7)
        cp_wsp = cp(wsp_hbm, wsp_v, 8)
        cp_bsp = cp(bsp_hbm, bsp_v, 9)
        cp_wout = cp(wout_hbm, wout_v, 10)
        cp_x = [cp(x_hbm.at[pl.ds(i * RA, RA)], xz.at[pl.ds(i * RA, RA), pl.ds(0, D)], 11 + i) for i in range(NA)]

        cp_ms = [cp(wmod_hbm.at[pl.ds(i * (D // MSPLIT), D // MSPLIT), pl.ds(0, 2 * D)],
                    wmod_v.at[pl.ds(i * (D // MSPLIT), D // MSPLIT), pl.ds(0, 2 * D)], 11 + NA + i)
                 for i in range(MSPLIT)]
        named = dict(q=[cp_wq], c=[cp_c], k=[cp_wk], v=[cp_wv], m=cp_ms)
        named.update({str(i): [cp_x[i]] for i in range(NA)})
        assert sorted(DORD) == sorted(named)
        for ch in DORD:
            for c_ in named[ch]:
                c_.start()

        cp_wq.wait()
        wt_s[0:D, :] = wq_v[...].astype(F32).T.astype(BF)
        cp_wk.wait()
        cp_wv.wait()

        cp_c.wait()
        cc = jnp.broadcast_to(c_v[...].astype(F32), (16, D))
        sc = (cc * jax.nn.sigmoid(cc)).astype(BF)
        waited = 0
        normed = {}
        for i in range(NPRE):
            cp_x[i].wait()
            waited += 1
            normed[i] = _ln(xz[i * RA:(i + 1) * RA, 0:D].astype(F32))
        mod0 = None
        for i in range(MSPLIT):
            cp_ms[i].wait()
            kr = slice(i * (D // MSPLIT), (i + 1) * (D // MSPLIT))
            part = jnp.dot(sc[:, kr], wmod_v[kr, 0:2 * D], preferred_element_type=F32)
            mod0 = part if mod0 is None else mod0 + part
        sa = mod0[0:1, 0:D]
        ca1 = 1.0 + mod0[0:1, D:2 * D]

        def norm1(i):
            n = normed[i] if i in normed else _ln(xz[i * RA:(i + 1) * RA, 0:D].astype(F32))
            return (n * ca1 + sa).astype(BF)

        def project(i, h, stats):
            qmax, kmax, vmax = stats
            kvt = lax.dot_general(wt_s[D:D + 2 * DH, :], h, NT, preferred_element_type=F32)
            qt = lax.dot_general(wt_s[0:D, :], h, NT, preferred_element_type=F32)
            kt = kvt[0:DH].astype(BF).astype(F32)
            vt = kvt[DH:2 * DH].astype(BF)
            vw = pltpu.bitcast(vt, F32)
            kn = jnp.concatenate([kt, jnp.zeros((128 - DH, RA), F32)], axis=0).T
            k_s[i * RA:(i + 1) * RA, :] = kn[:, 0:DH].astype(BF)
            for g in range(RA // 16):
                att.store_keys(wk, ks, i * (RA // 16) + g, kn[g * 16:(g + 1) * 16, :])
            qb = (qt * QSCALE).astype(BF)
            qf = qb.astype(F32)
            qw = pltpu.bitcast(qb, F32)
            for jj in range(RA // 128):
                c = i * (RA // 128) + jj
                blk, j = divmod(c, NJ)
                lanes = slice(jj * 128, (jj + 1) * 128)
                ks[att.VS0 + c * 8:att.VS0 + (c + 1) * 8, :] = vw[:, lanes]
                for hh in range(H):
                    r = (blk * H + hh) * NJ + j
                    ks[att.QS0 + r * 8:att.QS0 + (r + 1) * 8, :] = qw[hh * 8:(hh + 1) * 8, lanes]
                    wk[att.QF0 + r * DH:att.QF0 + (r + 1) * DH, :] = qf[hh * DH:(hh + 1) * DH, lanes]
            q2 = (qf * qf).reshape(H, 2, 8, RA)
            q2 = jnp.max(q2[:, 0] + q2[:, 1], axis=0)
            for j in range(RA // 128):
                qmax = jnp.maximum(qmax, q2[:, j * 128:(j + 1) * 128])
            kmax = jnp.maximum(kmax, jnp.sum(kt * kt, axis=0, keepdims=True))
            vmax = jnp.maximum(vmax, jnp.abs(vt.astype(F32)))
            return qmax, kmax, vmax

        stats = (jnp.zeros((8, 128), F32), jnp.zeros((1, RA), F32), jnp.zeros((DH, RA), F32))
        hs = {}
        for n, upto in enumerate(PB):
            while waited <= upto:
                cp_x[waited].wait()
                waited += 1
            if waited == NA:
                for c_ in (cp_m1, cp_wo, cp_win, cp_bsp, cp_wout, cp_wsp):
                    c_.start()
            lo = 0 if n == 0 else PB[n - 1]
            hi = NA if n == len(PB) - 1 else upto
            for i in range(lo, hi):
                if MODP and i == NA - MODP:
                    cp_m1.wait()
                for i2 in (i, i + 1):
                    if i2 < waited and i2 not in hs:
                        hs[i2] = norm1(i2)
                stats = project(i, hs[i], stats)
        if MODP:
            mod_s[...] = jnp.dot(sc, wmod_v[:, 2 * D:6 * D], preferred_element_type=F32)[0:8]
        qmax, kmax, vmax = stats
        bound2 = jnp.max(jnp.sum(qmax, axis=0, keepdims=True)) * jnp.max(kmax)
        vm = jnp.max(vmax)
        safe = (bound2 <= 60.0 * 60.0) & (vm <= 2.0 ** 40) & (vm >= 2.0 ** -40)
        zs[0] = jnp.where(safe, 0, 1)
        zs[1] = jnp.minimum(jnp.where(safe, 0, 1), 0)

        @pl.when(safe)
        def _fast():
            att.run(wk, ks, zs, NREP)

        @pl.when(jnp.logical_not(safe))
        def _true_max():
            def body(it, carry):
                q = pltpu.bitcast(ks[pl.ds(pl.multiple_of(att.QS0 + it * 8, 8), 8), :], BF)
                s = jnp.dot(k_s[...], q, preferred_element_type=F32)
                e = jnp.exp2(s - jnp.max(s, axis=0, keepdims=True))
                l = jnp.sum(e, axis=0, keepdims=True)
                vt = pltpu.bitcast(jnp.concatenate(
                    [ks[att.VS0 + c * 8:att.VS0 + (c + 1) * 8, :] for c in range(NTILE)], axis=1), BF)
                o = jnp.dot(vt, e.astype(BF), preferred_element_type=F32)
                wk[pl.ds(pl.multiple_of(att.OT0 + it * DH, DH), DH), :] = o * (1.0 / l)
                return carry

            lax.fori_loop(0, NU * NJ, body, 0)

        for c_ in (cp_wo, cp_win, cp_bsp, cp_wout, cp_wsp):
            c_.wait()
        if not MODP:
            cp_m1.wait()
            mod_s[...] = jnp.dot(sc, wmod_v[:, 2 * D:6 * D], preferred_element_type=F32)[0:8]
        ga = mod_s[0:1, 0:D]
        sb = mod_s[0:1, D:2 * D]
        cb1 = 1.0 + mod_s[0:1, 2 * D:3 * D]

        def mix_in(i):
            rows = slice(i * RC, (i + 1) * RC)
            cols = []
            for c in range(i * (RC // 128), (i + 1) * (RC // 128)):
                blk, j = divmod(c, NJ)
                cols.append(jnp.concatenate(
                    [wk[att.OT0 + ((blk * H + hh) * NJ + j) * DH:att.OT0 + ((blk * H + hh) * NJ + j + 1) * DH, :]
                     for hh in range(H)], axis=0).T)
            o = jnp.concatenate(cols, axis=0).astype(BF)
            a = jnp.dot(o, wo_v[...], preferred_element_type=F32)
            x1 = xz[rows, 0:D].astype(F32) + ga * a
            x1_s[rows, :] = x1
            return (_ln(x1) * cb1 + sb).astype(BF)

        def mlp_in(i, h2):
            rows = pl.ds(pl.multiple_of(i * RC + zero, RC), RC) if PIN else slice(i * RC, (i + 1) * RC)
            zb = _gelu(jnp.dot(h2, win_v[:, FH:2 * FH], preferred_element_type=F32))
            xz[rows, D + FH:D + 2 * FH] = _ln(zb).astype(BF)
            za = _gelu(jnp.dot(h2, win_v[:, 0:FH], preferred_element_type=F32))
            xz[rows, D:D + FH] = za.astype(BF)

        zero = zs[1]
        h2 = mix_in(0)
        for i in range(S // RC if STOP >= 2 else 0):
            h2_next = mix_in(i + 1) if i + 1 < S // RC else None
            mlp_in(i, h2)
            h2 = h2_next
        bf = bsp_v[...].astype(F32)
        for r in range(S // 128):
            bcol_s[r * 128:(r + 1) * 128, :] = jnp.broadcast_to(bf[r:r + 1, :], (128, 128)).T


        def out_cp(i):
            rows = pl.ds(pl.multiple_of(i * RD, RD), RD)
            return pltpu.make_async_copy(out_s.at[rows], out_hbm.at[rows], osems.at[i])

        def gate(i):
            rows = pl.ds(pl.multiple_of(i * RD, RD), RD)
            g = jnp.dot(wsp_v[rows, :], xz[:, D + FH:D + 2 * FH], preferred_element_type=F32)
            g = g + jnp.concatenate([bcol_s[rows, :]] * (FH // 128), axis=1)
            return (xz[rows, D:D + FH].astype(F32) * g).astype(BF)

        def project_out(i, y):
            rows = pl.ds(pl.multiple_of(i * RD, RD), RD)
            o = jnp.dot(y, wout_v[...], preferred_element_type=F32)
            out_s[rows, :] = (x1_s[rows, :] + mod_s[0:1, 3 * D:4 * D] * o).astype(BF)

        def body_d(it, carry):
            ys = [gate(it * UD + u) for u in range(UD)]
            for u in range(UD):
                project_out(it * UD + u, ys[u])
                if EARLY:
                    out_cp(it * UD + u).start()
            for u in range(0 if EARLY else UD):
                out_cp(it * UD + u).start()
            return carry

        if STOP >= 3 and DFULL:
            for it in range(S // RD // UD):
                body_d(it, 0)
        elif STOP >= 3:
            lax.fori_loop(0, S // RD // UD, body_d, 0)
        else:
            for i in range(S // RD):
                out_cp(i).start()
        for i in range(S // RD):
            out_cp(i).wait()

    V = pltpu.VMEM
    scratch = [
        V((att.rows, 128), F32), V((att.ks_rows, 128), F32),
        V((S, D + 2 * FH), BF), V((D, D), BF), V((D, D), BF), V((D, 2 * FH), BF), V((S, S), BF), V((FH, D), BF),
        V((D, 6 * D), BF), V((D + 2 * DH, D), BF), V((S, DH), BF),
        V((S, D), F32), V((S, D), BF), V((8, 4 * D), F32), V((S, 128), F32),
        V((S // 128, 128), BF), V((1, D), BF),
        pltpu.SMEM((2,), jnp.int32),
        pltpu.SemaphoreType.DMA((11 + S // RA + MSPLIT,)), pltpu.SemaphoreType.DMA((S // RD,)),
    ]

    def fn(A_x, A_wq, A_wk, A_wv, A_wo, B_x, B_w_in, B_w_sp, B_b_sp, B_w_out, c, w_mod):
        del B_x
        out = pl.pallas_call(
            kernel,
            out_shape=jax.ShapeDtypeStruct((S, D), BF),
            in_specs=[pl.BlockSpec(memory_space=pl.ANY)] * 11,
            out_specs=pl.BlockSpec(memory_space=pl.ANY),
            scratch_shapes=scratch,
            compiler_params=pltpu.CompilerParams(vmem_limit_bytes=100 * 1024 * 1024),
            name="fused",
        )(A_x.reshape(S, D), A_wq, A_wk.T, A_wv.T, A_wo, B_w_in, B_w_sp, B_b_sp.reshape(S // 128, 128),
          B_w_out, c, w_mod)
        return out.reshape(1, S, D)

    return fn


_fused = build(dd=3)


@jax.jit
def pallas_adaLN_cond__grouped_kv_mqa__mixer_gmlp__prompt_kernel(
    A_x: jax.Array,
    A_wq: jax.Array,
    A_wk: jax.Array,
    A_wv: jax.Array,
    A_wo: jax.Array,
    B_x: jax.Array,
    B_w_in: jax.Array,
    B_w_sp: jax.Array,
    B_b_sp: jax.Array,
    B_w_out: jax.Array,
    c: jax.Array,
    w_mod: jax.Array,
):
    return _fused(A_x, A_wq, A_wk, A_wv, A_wo, B_x, B_w_in, B_w_sp, B_b_sp, B_w_out, c, w_mod)
```

```python
import math
from fractions import Fraction

import jax
import jax.numpy as jnp
from jax import lax
from jax.experimental import pallas as pl
from jax.experimental.pallas import tpu as pltpu

BF = jnp.bfloat16
F32 = jnp.float32
S, D, H, DH, FH = 2048, 512, 32, 16, 896
EPS = 1e-5
QSCALE = DH ** -0.5 * math.log2(math.e)
NT = (((1,), (1,)), ((), ()))

QB = 512
NJ = QB // 128
NU = (S // QB) * H
NTILE = S // 128
NFENCE = 512


def _ln(x):
    m = jnp.mean(x, axis=-1, keepdims=True)
    xc = x - m
    v = jnp.mean(xc * xc, axis=-1, keepdims=True)
    return xc * lax.rsqrt(v + EPS)


def _gelu(x):
    c = math.sqrt(2.0 / math.pi)
    return 0.5 * x * (1.0 + jnp.tanh(x * (c + (c * 0.044715) * (x * x))))


class _Attention:
    def __init__(self, hu, nv, dl, el, vl, vo, jb, fj, kl, qk, fl, mb, pt=1, dd=0, fj2=0, bp=0, sq=1):
        self.sq = sq
        self.hu, self.nv, self.dl, self.el, self.vl = hu, nv, dl, el, vl
        self.jb, self.fj, self.kl, self.qk, self.fl, self.pt = jb, fj, kl, qk, fl, pt
        self.fj2, self.bp = fj2, bp
        self.nm = nm = S // 16 - nv
        events = [(Fraction(m + 1), 0, "m", m) for m in range(nm)]
        events += [(Fraction((i + 1) * nm, nv) + vl + vo, 1, "v", i) for i in range(nv)]
        events.sort()
        self.tiles, self.tile_of, self.source = [], {}, {}
        for t in range(NTILE):
            part = events[8 * t:8 * t + 8]
            for pos, e in enumerate(part):
                self.tile_of[e[2:]] = (t, pos)
                self.source[8 * t + 7 - pos] = e[2:]
            self.tiles.append(([e[2:] for e in part], math.ceil(max(e[0] for e in part))))
        cuts = sorted({(end + dl) % nm for _, end in self.tiles})
        self.seam = (cuts[-1], cuts[0]) if mb and cuts[0] else None
        self.deferred = [t for t, (_, end) in enumerate(self.tiles) if end + dl >= nm + dd]
        self.KB0 = 0
        self.QB0 = self.KB0 + nv * DH * 16
        self.QF0 = self.QB0 + 2 * DH * NJ * 8
        self.OT0 = self.QF0 + NU * NJ * DH
        self.PD0 = self.OT0 + NU * NJ * (DH + 8)
        self.AD0 = self.PD0 + len(self.deferred) * 8 * NJ * 16
        self.LD0 = self.AD0 + NJ * DH
        self.PN0 = self.LD0 + NJ * 8
        self.J0 = self.PN0 + NJ * 8
        self.rows = -(-(self.J0 + (NFENCE + 2) * 8) // 32) * 32
        self.OT1 = self.QF0
        self.PN1 = self.OT1 + NU * NJ * (DH + 8)
        self.J1 = self.PN1 + NJ * 8
        self.rows1 = -(-(self.J1 + (NFENCE + 2) * 8) // 32) * 32
        self.KX0 = nm * 8
        self.VS0 = self.KX0 + 16 * 8
        self.QS0 = self.VS0 + NTILE * 8
        self.ks_rows = -(-(self.QS0 + NU * NJ * 8) // 32) * 32

    def store_keys(self, wks, ks, group, kn16):
        kind, idx = self.source[group]
        if kind == "v":
            for d in range(DH):
                o = self.KB0 + (idx * DH + d) * 16
                wks[d % 2][o:o + 16, :] = jnp.broadcast_to(kn16[:, d:d + 1], (16, 128))
            return
        ks[idx * 8:(idx + 1) * 8, :] = pltpu.bitcast(kn16.astype(BF), F32)
        if self.seam:
            a, b = self.seam
            if idx >= a:
                o = self.KX0 + (idx - a) * 8
                ks[o:o + 8, :] = pltpu.bitcast(kn16.astype(BF), F32)
            elif idx < b:
                o = self.KX0 + (self.nm - a + idx) * 8
                ks[o:o + 8, :] = pltpu.bitcast(pltpu.roll(kn16, DH, 1).astype(BF), F32)

    def out_rows(self, u, j):
        return j % 2, (self.OT0, self.OT1)[j % 2] + (u * NJ + j) * (DH + 8)

    def _finish(self, u, acc, lsum):
        stores = []
        for j in range(NJ):
            c, row = self.out_rows(u, j)
            stores.append((c, row + DH, lsum[j]))
            for half in range(DH // 8):
                stores.append((c, row + half * 8, acc[half * 8:(half + 1) * 8, j * 128:(j + 1) * 128]))
        return stores

    def _pv(self, ks, t, p):
        vt = pltpu.bitcast(ks[self.VS0 + t * 8:self.VS0 + (t + 1) * 8, :], BF)
        return jnp.dot(vt, p.astype(BF), preferred_element_type=F32)

    def _pd(self, t, pos, j):
        return self.PD0 + ((self.deferred.index(t) * 8 + pos) * NJ + j) * 16

    def _load_pd(self, wk, t):
        return jnp.concatenate(
            [jnp.concatenate([wk[self._pd(t, pos, j):self._pd(t, pos, j) + 16, :] for j in range(NJ)], axis=1)
             for pos in range(7, -1, -1)], axis=0)

    def _load_acc(self, wk):
        return jnp.concatenate([wk[self.AD0 + j * DH:self.AD0 + (j + 1) * DH, :] for j in range(NJ)], axis=1)

    def _load_l(self, wk):
        return [wk[self.LD0 + j * 8:self.LD0 + (j + 1) * 8, :] for j in range(NJ)]

    def _qb_row(self, wk, u, h, d, j):
        r = wk[pl.ds(self.QF0 + (u * NJ + j) * DH + d, 1), :]
        return self.QB0 + (((h % 2) * DH + d) * NJ + j) * 8, jnp.broadcast_to(r, (8, 128))

    def run(self, wk, wk1, ks, zs, nrep=1):
        wk[self.PD0:self.LD0, :] = jnp.zeros((self.LD0 - self.PD0, 128), F32)
        wk[self.LD0:self.PN0, :] = jnp.ones((self.PN0 - self.LD0, 128), F32)
        for d in range(DH):
            for j in range(NJ):
                o, v = self._qb_row(wk, 0, 0, d, j)
                (wk, wk1)[d % 2][o:o + 8, :] = v

        def body(it, carry):
            self._units(it, wk, wk1, ks, zs)
            return carry

        if nrep == 1:
            lax.fori_loop(0, NU // self.hu, body, 0)
        else:
            lax.fori_loop(0, nrep * NU // self.hu, lambda it, c: body(it % (NU // self.hu), c), 0)
        acc = self._load_acc(wk)
        for t in self.deferred:
            acc = acc + self._pv(ks, t, self._load_pd(wk, t))
        for c, o, v in self._finish(NU - 1, acc, self._load_l(wk)):
            (wk, wk1)[c][o:o + 8, :] = v

    def _units(self, it, wk, wk1, ks, zs):
        hu, nv, nm, dl, el, vl, jb = self.hu, self.nv, self.nm, self.dl, self.el, self.vl, self.jb
        u0 = it * hu
        ngrp = hu * nm
        chains = (wk, wk1)
        junk = (self.J0 + zs[0] * 8, self.J1 + zs[0] * 8)
        qts, ls, accs, es, ss, kls, qgen, first_pv = {}, {}, {}, {}, {}, {}, {}, {}
        pend, late = [], []

        def load_q(h):
            b = self.QS0 + (u0 + h) * (NJ * 8)
            qts[h] = pltpu.bitcast(jnp.concatenate(
                [ks[pl.ds(pl.multiple_of(b + j * 8, 8), 8), :] for j in range(NJ)], axis=1), BF)

        def qb_ops(h):
            u = u0 + h if h < hu else jnp.minimum(u0 + h, NU - 1)
            for d in range(DH):
                for j in range(NJ):
                    pend.append((d % 2,) + self._qb_row(wk, u, h, d, j))
                    yield

        def emit_p(h, key, j, s16):
            e = jnp.exp2(s16)
            e2 = e[0:8] + e[8:16]
            ls[h, j] = ls[h, j] + e2 if (h, j) in ls else e2
            t, pos = self.tile_of[key]
            if h == hu - 1 and t in self.deferred:
                wk[self._pd(t, pos, j):self._pd(t, pos, j) + 16, :] = e
            else:
                es[h, key, j] = e
            return e

        partial, count, last = {}, {}, {}

        def vpu_ops(c):
            for h in range(hu):
                for vi in range(nv):
                    for j0 in range(0, NJ, jb):
                        for d in range(c, DH, 2):
                            o = self.KB0 + (vi * DH + d) * 16
                            kk = chains[c][o:o + 16, :].reshape(2, 8, 128)
                            for j in range(j0, j0 + jb):
                                o = self.QB0 + (((h % 2) * DH + d) * NJ + j) * 8
                                pr = kk * chains[c][o:o + 8, :][None]
                                key = (h, vi, j)
                                partial[key] = partial[key] + pr if key in partial else pr
                                count[key] = count.get(key, 0) + 1
                                last[c] = pr
                                if count[key] == DH:
                                    emit_p(h, ("v", vi), j, partial.pop(key).reshape(16, 128))
                            yield

        steps = DH * (NJ // jb)
        pv_at, fin_at, pin_at = {}, {}, {}
        for h in range(-1, hu):
            for t, (_, end) in enumerate(self.tiles):
                if (h == -1 and t not in self.deferred) or (h == hu - 1 and t in self.deferred):
                    continue
                x = h * nm + end + dl
                pv_at.setdefault(x, []).append((h, t))
                if t == NTILE - 1:
                    fin_at[x + self.fl] = h
                if t == 0:
                    pin_at[x + self.fl] = h
        cuts = {0, ngrp} | {x for x in pv_at if x < ngrp}
        if not self.seam:
            cuts |= {h * nm for h in range(hu)}
        cuts = sorted(cuts)
        runs = dict(zip(cuts[:-1], cuts[1:]))

        def load_k(a):
            h = a // nm
            if runs[a] > (h + 1) * nm:
                kls[a] = ks[self.KX0:self.KX0 + (runs[a] - a) * 8, :]
            else:
                kls[a] = ks[(a - h * nm) * 8:(runs[a] - h * nm) * 8, :]

        vgen = (vpu_ops(0), vpu_ops(1))
        vdone, nfence = [0, 0], [0, 0]

        def ticks(g):
            h, r = divmod(g, nm)
            return h * (nm + NTILE) + r + 1 + sum(1 for _, end in self.tiles if (end + dl) % nm <= r)

        def pace_store(c, value):
            nfence[c] += 1
            chains[c][pl.ds(pl.multiple_of(junk[c] + 8 * (nfence[c] % NFENCE), 8), 8), :] = value

        def tick(values, halves, period):
            for c, o, v in pend:
                chains[c][o:o + 8, :] = v
            pend.clear()
            for c in range(2):
                for item in [item for item in late if item[0] == c][:self.sq]:
                    late[:] = [other for other in late if other is not item]
                    o = item[1] if isinstance(item[1], int) else pl.multiple_of(item[1], 8)
                    chains[c][pl.ds(o, 8), :] = item[2]
                if values:
                    if self.bp and c in last:
                        pace_store(c, last[c][1])
                    pace_store(c, values[c])
                while vdone[c] < min(((halves + c + 1) * nv * steps) // (4 * period), hu * nv * steps // 2):
                    next(vgen[c])
                    vdone[c] += 1

        pv_results = {}
        for x in range(-max(self.kl, self.qk), ngrp + dl + el + 32):
            if (x + self.qk) % nm == 0 and 0 <= (x + self.qk) // nm < hu:
                load_q((x + self.qk) // nm)
            if x + self.kl - el in runs:
                load_k(x + self.kl - el)
            for h, t in pv_at.get(x, []):
                if h == -1:
                    p = self._load_pd(wk, t)
                    if h not in accs:
                        accs[h] = self._load_acc(wk)
                else:
                    p = jnp.concatenate([jnp.concatenate([es.pop((h, key, j)) for j in range(NJ)], axis=1)
                                         for key in reversed(self.tiles[t][0])], axis=0)
                pv = self._pv(ks, t, p)
                pv_results.setdefault(x, []).append(pv)
                accs[h] = pv if t == 0 else accs[h] + pv
                if t == 0:
                    first_pv[h] = pv
            if x in pin_at:
                for j in range(NJ):
                    late.append((j % 2, (self.PN0, self.PN1)[j % 2] + j * 8,
                                 first_pv[pin_at[x]][0:8, j * 128:(j + 1) * 128]))
            if x in fin_at:
                h = fin_at[x]
                if h == -1:
                    late.extend(self._finish((u0 + NU - 1) % NU, accs[h], self._load_l(wk)))
                else:
                    late.extend(self._finish(u0 + h, accs[h], [ls[h, j] for j in range(NJ)]))
            if x in runs:
                if x not in kls:
                    load_k(x)
                h = x // nm
                keys = pltpu.bitcast(kls.pop(x), BF)
                if runs[x] > (h + 1) * nm:
                    s = jnp.dot(keys[:, 0:2 * DH], jnp.concatenate([qts[h], qts[h + 1]], axis=0),
                                preferred_element_type=F32)
                else:
                    s = jnp.dot(keys[:, 0:DH], qts[h], preferred_element_type=F32)
                for g in range(x, runs[x]):
                    ss[g] = s[(g - x) * 16:(g - x + 1) * 16]
            g = x - el
            if self.pt and 0 <= g < ngrp and g in pv_results:
                pv = pv_results[g][-1]
                tick((pv[0:8, self.fj2 * 128:(self.fj2 + 1) * 128], pv[8:16, self.fj * 128:(self.fj + 1) * 128]),
                     2 * (ticks(g) - 2 - vl), nm + NTILE)
            values = None
            if 0 <= g < ngrp:
                s = ss.pop(g)
                e = [emit_p(g // nm, ("m", g % nm), j, s[:, j * 128:(j + 1) * 128]) for j in range(NJ)]
                values = (e[self.fj2][0:8], e[self.fj][8:16])
            if self.pt:
                tick(values, 2 * (ticks(g) - 1 - vl), nm + NTILE)
            else:
                tick(values, 2 * (g - vl), nm)
            hq = (x + nm - 14) // nm
            if 1 <= hq <= hu:
                if hq not in qgen:
                    qgen[hq] = qb_ops(hq)
                next(qgen[hq], None)
        for j in range(NJ):
            wk[self.AD0 + j * DH:self.AD0 + (j + 1) * DH, :] = accs[hu - 1][:, j * 128:(j + 1) * 128]
            wk[self.LD0 + j * 8:self.LD0 + (j + 1) * 8, :] = ls[hu - 1, j]
        assert not es and not ss and not pend and not late


def build(HU=8, RA=256, RC=128, RD=128, UD=4, PB=(1, 3, 7), NREP=1, STOP=9, PIN=1, EARLY=1, DORD='qckv0m1234567', NPRE=1, MSPLIT=2, MODP=0, DFULL=0, dd=4,
          nv=19, dl=9, el=9, vl=-3, vo=2, jb=2, fj=2, kl=8, qk=9, fl=9, mb=1, pt=1, fj2=1, bp=0, sq=1):
    att = _Attention(HU, nv, dl, el, vl, vo, jb, fj, kl, qk, fl, mb, pt, dd, fj2, bp, sq)

    def kernel(x_hbm, wq_hbm, wk_hbm, wv_hbm, wo_hbm, win_hbm, wsp_hbm, bsp_hbm, wout_hbm, c_hbm, wmod_hbm,
               out_hbm,
               wk, wk1, ks, xz, wq_v, wo_v, win_v, wsp_v, wout_v, wmod_v, wt_s, k_s, x1_s, out_s,
               mod_s, bcol_s, bsp_v, c_v, zs, sems, osems):
        NA = S // RA

        def cp(src, dst, i):
            return pltpu.make_async_copy(src, dst, sems.at[i])

        cp_c = cp(c_hbm, c_v, 0)
        cp_m1 = cp(wmod_hbm.at[:, pl.ds(2 * D, 4 * D)], wmod_v.at[:, pl.ds(2 * D, 4 * D)], 2)
        cp_wq = cp(wq_hbm, wq_v, 3)
        cp_wk = cp(wk_hbm, wt_s.at[pl.ds(D, DH)], 4)
        cp_wv = cp(wv_hbm, wt_s.at[pl.ds(D + DH, DH)], 5)
        cp_wo = cp(wo_hbm, wo_v, 6)
        cp_win = cp(win_hbm, win_v, 7)
        cp_wsp = cp(wsp_hbm, wsp_v, 8)
        cp_bsp = cp(bsp_hbm, bsp_v, 9)
        cp_wout = cp(wout_hbm, wout_v, 10)
        cp_x = [cp(x_hbm.at[pl.ds(i * RA, RA)], xz.at[pl.ds(i * RA, RA), pl.ds(0, D)], 11 + i) for i in range(NA)]

        cp_ms = [cp(wmod_hbm.at[pl.ds(i * (D // MSPLIT), D // MSPLIT), pl.ds(0, 2 * D)],
                    wmod_v.at[pl.ds(i * (D // MSPLIT), D // MSPLIT), pl.ds(0, 2 * D)], 11 + NA + i)
                 for i in range(MSPLIT)]
        named = dict(q=[cp_wq], c=[cp_c], k=[cp_wk], v=[cp_wv], m=cp_ms)
        named.update({str(i): [cp_x[i]] for i in range(NA)})
        assert sorted(DORD) == sorted(named)
        for ch in DORD:
            for c_ in named[ch]:
                c_.start()

        cp_wq.wait()
        wt_s[0:D, :] = wq_v[...].astype(F32).T.astype(BF)
        cp_wk.wait()
        cp_wv.wait()

        cp_c.wait()
        cc = jnp.broadcast_to(c_v[...].astype(F32), (16, D))
        sc = (cc * jax.nn.sigmoid(cc)).astype(BF)
        waited = 0
        normed = {}
        for i in range(NPRE):
            cp_x[i].wait()
            waited += 1
            normed[i] = _ln(xz[i * RA:(i + 1) * RA, 0:D].astype(F32))
        mod0 = None
        for i in range(MSPLIT):
            cp_ms[i].wait()
            kr = slice(i * (D // MSPLIT), (i + 1) * (D // MSPLIT))
            part = jnp.dot(sc[:, kr], wmod_v[kr, 0:2 * D], preferred_element_type=F32)
            mod0 = part if mod0 is None else mod0 + part
        sa = mod0[0:1, 0:D]
        ca1 = 1.0 + mod0[0:1, D:2 * D]

        def norm1(i):
            n = normed[i] if i in normed else _ln(xz[i * RA:(i + 1) * RA, 0:D].astype(F32))
            return (n * ca1 + sa).astype(BF)

        def project(i, h, stats):
            qmax, kmax, vmax = stats
            kvt = lax.dot_general(wt_s[D:D + 2 * DH, :], h, NT, preferred_element_type=F32)
            qt = lax.dot_general(wt_s[0:D, :], h, NT, preferred_element_type=F32)
            kt = kvt[0:DH].astype(BF).astype(F32)
            vt = kvt[DH:2 * DH].astype(BF)
            vw = pltpu.bitcast(vt, F32)
            kn = jnp.concatenate([kt, jnp.zeros((128 - DH, RA), F32)], axis=0).T
            k_s[i * RA:(i + 1) * RA, :] = kn[:, 0:DH].astype(BF)
            for g in range(RA // 16):
                att.store_keys((wk, wk1), ks, i * (RA // 16) + g, kn[g * 16:(g + 1) * 16, :])
            qb = (qt * QSCALE).astype(BF)
            qf = qb.astype(F32)
            qw = pltpu.bitcast(qb, F32)
            for jj in range(RA // 128):
                c = i * (RA // 128) + jj
                blk, j = divmod(c, NJ)
                lanes = slice(jj * 128, (jj + 1) * 128)
                ks[att.VS0 + c * 8:att.VS0 + (c + 1) * 8, :] = vw[:, lanes]
                for hh in range(H):
                    r = (blk * H + hh) * NJ + j
                    ks[att.QS0 + r * 8:att.QS0 + (r + 1) * 8, :] = qw[hh * 8:(hh + 1) * 8, lanes]
                    wk[att.QF0 + r * DH:att.QF0 + (r + 1) * DH, :] = qf[hh * DH:(hh + 1) * DH, lanes]
            q2 = (qf * qf).reshape(H, 2, 8, RA)
            q2 = jnp.max(q2[:, 0] + q2[:, 1], axis=0)
            for j in range(RA // 128):
                qmax = jnp.maximum(qmax, q2[:, j * 128:(j + 1) * 128])
            kmax = jnp.maximum(kmax, jnp.sum(kt * kt, axis=0, keepdims=True))
            vmax = jnp.maximum(vmax, jnp.abs(vt.astype(F32)))
            return qmax, kmax, vmax

        stats = (jnp.zeros((8, 128), F32), jnp.zeros((1, RA), F32), jnp.zeros((DH, RA), F32))
        hs = {}
        for n, upto in enumerate(PB):
            while waited <= upto:
                cp_x[waited].wait()
                waited += 1
            if waited == NA:
                for c_ in (cp_m1, cp_wo, cp_win, cp_bsp, cp_wout, cp_wsp):
                    c_.start()
            lo = 0 if n == 0 else PB[n - 1]
            hi = NA if n == len(PB) - 1 else upto
            for i in range(lo, hi):
                if MODP and i == NA - MODP:
                    cp_m1.wait()
                for i2 in (i, i + 1):
                    if i2 < waited and i2 not in hs:
                        hs[i2] = norm1(i2)
                stats = project(i, hs[i], stats)
        if MODP:
            mod_s[...] = jnp.dot(sc, wmod_v[:, 2 * D:6 * D], preferred_element_type=F32)[0:8]
        qmax, kmax, vmax = stats
        bound2 = jnp.max(jnp.sum(qmax, axis=0, keepdims=True)) * jnp.max(kmax)
        vm = jnp.max(vmax)
        safe = (bound2 <= 60.0 * 60.0) & (vm <= 2.0 ** 40) & (vm >= 2.0 ** -40)
        zs[0] = jnp.where(safe, 0, 1)
        zs[1] = jnp.minimum(jnp.where(safe, 0, 1), 0)

        @pl.when(safe)
        def _fast():
            att.run(wk, wk1, ks, zs, NREP)

        @pl.when(jnp.logical_not(safe))
        def _true_max():
            def body(it, carry):
                q = pltpu.bitcast(ks[pl.ds(pl.multiple_of(att.QS0 + it * 8, 8), 8), :], BF)
                s = jnp.dot(k_s[...], q, preferred_element_type=F32)
                e = jnp.exp2(s - jnp.max(s, axis=0, keepdims=True))
                l = jnp.sum(e, axis=0, keepdims=True)
                vt = pltpu.bitcast(jnp.concatenate(
                    [ks[att.VS0 + c * 8:att.VS0 + (c + 1) * 8, :] for c in range(NTILE)], axis=1), BF)
                o = jnp.dot(vt, e.astype(BF), preferred_element_type=F32)
                o = jnp.concatenate([o, jnp.broadcast_to(l * 0.125, (8, 128))], axis=0)
                wk[pl.ds(pl.multiple_of(att.OT0 + it * (DH + 8), 8), DH + 8), :] = o
                wk1[pl.ds(pl.multiple_of(att.OT1 + it * (DH + 8), 8), DH + 8), :] = o
                return carry

            lax.fori_loop(0, NU * NJ, body, 0)

        for c_ in (cp_wo, cp_win, cp_bsp, cp_wout, cp_wsp):
            c_.wait()
        if not MODP:
            cp_m1.wait()
            mod_s[...] = jnp.dot(sc, wmod_v[:, 2 * D:6 * D], preferred_element_type=F32)[0:8]
        ga = mod_s[0:1, 0:D]
        sb = mod_s[0:1, D:2 * D]
        cb1 = 1.0 + mod_s[0:1, 2 * D:3 * D]

        def mix_in(i):
            rows = slice(i * RC, (i + 1) * RC)
            cols = []
            for c in range(i * (RC // 128), (i + 1) * (RC // 128)):
                blk, j = divmod(c, NJ)
                tiles = [att.out_rows(blk * H + hh, j) for hh in range(H)]
                heads = []
                for c_, o in tiles:
                    l = jnp.sum((wk, wk1)[c_][o + DH:o + DH + 8, :], axis=0, keepdims=True)
                    r = pltpu.reciprocal(l, approx=True)
                    heads.append((wk, wk1)[c_][o:o + DH, :] * (r * (2.0 - l * r)))
                cols.append(jnp.concatenate(heads, axis=0).T)
            o = jnp.concatenate(cols, axis=0).astype(BF)
            a = jnp.dot(o, wo_v[...], preferred_element_type=F32)
            x1 = xz[rows, 0:D].astype(F32) + ga * a
            x1_s[rows, :] = x1
            return (_ln(x1) * cb1 + sb).astype(BF)

        def mlp_in(i, h2):
            rows = pl.ds(pl.multiple_of(i * RC + zero, RC), RC) if PIN else slice(i * RC, (i + 1) * RC)
            zb = _gelu(jnp.dot(h2, win_v[:, FH:2 * FH], preferred_element_type=F32))
            xz[rows, D + FH:D + 2 * FH] = _ln(zb).astype(BF)
            za = _gelu(jnp.dot(h2, win_v[:, 0:FH], preferred_element_type=F32))
            xz[rows, D:D + FH] = za.astype(BF)

        zero = zs[1]
        h2 = mix_in(0)
        for i in range(S // RC if STOP >= 2 else 0):
            h2_next = mix_in(i + 1) if i + 1 < S // RC else None
            mlp_in(i, h2)
            h2 = h2_next
        bf = bsp_v[...].astype(F32)
        for r in range(S // 128):
            bcol_s[r * 128:(r + 1) * 128, :] = jnp.broadcast_to(bf[r:r + 1, :], (128, 128)).T


        def out_cp(i):
            rows = pl.ds(pl.multiple_of(i * RD, RD), RD)
            return pltpu.make_async_copy(out_s.at[rows], out_hbm.at[rows], osems.at[i])

        def gate(i):
            rows = pl.ds(pl.multiple_of(i * RD, RD), RD)
            g = jnp.dot(wsp_v[rows, :], xz[:, D + FH:D + 2 * FH], preferred_element_type=F32)
            g = g + jnp.concatenate([bcol_s[rows, :]] * (FH // 128), axis=1)
            return (xz[rows, D:D + FH].astype(F32) * g).astype(BF)

        def project_out(i, y):
            rows = pl.ds(pl.multiple_of(i * RD, RD), RD)
            o = jnp.dot(y, wout_v[...], preferred_element_type=F32)
            out_s[rows, :] = (x1_s[rows, :] + mod_s[0:1, 3 * D:4 * D] * o).astype(BF)

        def body_d(it, carry):
            ys = [gate(it * UD + u) for u in range(UD)]
            for u in range(UD):
                project_out(it * UD + u, ys[u])
                if EARLY:
                    out_cp(it * UD + u).start()
            for u in range(0 if EARLY else UD):
                out_cp(it * UD + u).start()
            return carry

        if STOP >= 3 and DFULL:
            for it in range(S // RD // UD):
                body_d(it, 0)
        elif STOP >= 3:
            lax.fori_loop(0, S // RD // UD, body_d, 0)
        else:
            for i in range(S // RD):
                out_cp(i).start()
        for i in range(S // RD):
            out_cp(i).wait()

    V = pltpu.VMEM
    scratch = [
        V((att.rows, 128), F32), V((att.rows1, 128), F32), V((att.ks_rows, 128), F32),
        V((S, D + 2 * FH), BF), V((D, D), BF), V((D, D), BF), V((D, 2 * FH), BF), V((S, S), BF), V((FH, D), BF),
        V((D, 6 * D), BF), V((D + 2 * DH, D), BF), V((S, DH), BF),
        V((S, D), F32), V((S, D), BF), V((8, 4 * D), F32), V((S, 128), F32),
        V((S // 128, 128), BF), V((1, D), BF),
        pltpu.SMEM((2,), jnp.int32),
        pltpu.SemaphoreType.DMA((11 + S // RA + MSPLIT,)), pltpu.SemaphoreType.DMA((S // RD,)),
    ]

    def fn(A_x, A_wq, A_wk, A_wv, A_wo, B_x, B_w_in, B_w_sp, B_b_sp, B_w_out, c, w_mod):
        del B_x
        out = pl.pallas_call(
            kernel,
            out_shape=jax.ShapeDtypeStruct((S, D), BF),
            in_specs=[pl.BlockSpec(memory_space=pl.ANY)] * 11,
            out_specs=pl.BlockSpec(memory_space=pl.ANY),
            scratch_shapes=scratch,
            compiler_params=pltpu.CompilerParams(vmem_limit_bytes=100 * 1024 * 1024),
            name="fused",
        )(A_x.reshape(S, D), A_wq, A_wk.T, A_wv.T, A_wo, B_w_in, B_w_sp, B_b_sp.reshape(S // 128, 128),
          B_w_out, c, w_mod)
        return out.reshape(1, S, D)

    return fn


_fused = build()


@jax.jit
def pallas_adaLN_cond__grouped_kv_mqa__mixer_gmlp__prompt_kernel(
    A_x: jax.Array,
    A_wq: jax.Array,
    A_wk: jax.Array,
    A_wv: jax.Array,
    A_wo: jax.Array,
    B_x: jax.Array,
    B_w_in: jax.Array,
    B_w_sp: jax.Array,
    B_b_sp: jax.Array,
    B_w_out: jax.Array,
    c: jax.Array,
    w_mod: jax.Array,
):
    return _fused(A_x, A_wq, A_wk, A_wv, A_wo, B_x, B_w_in, B_w_sp, B_b_sp, B_w_out, c, w_mod)
```

```python
import math

import jax
import jax.numpy as jnp
from jax import lax
from jax.experimental import pallas as pl
from jax.experimental.pallas import tpu as pltpu

BF = jnp.bfloat16
F32 = jnp.float32
S, D, H, DH, FH = 2048, 512, 32, 16, 896
EPS = 1e-5
QSCALE = DH ** -0.5 * math.log2(math.e)
NT = (((1,), (1,)), ((), ()))

SCORE_LIMIT = 96.0
V_MIN, V_MAX = 2.0 ** -16, 2.0 ** 16

QB = 512
NJ = QB // 128
NU = (S // QB) * H
NTILE = S // 128
RA = 256
X_WAITS = (1, 3, 7)
RC = 128
RD, UD = 128, 4

HU = 8
NV = 19
NM = S // 16 - NV
PV_LAG = 9
EXP_LAG = 9
STORE_LAG = 9
Q_LEAD = 9
VPU_LEAD = 3
VPU_SLOT = -1
DRAIN = 4
PACE = (1, 2)
NPACE = 512

KB0 = 0
QB0 = KB0 + NV * DH * 16
QF0 = QB0 + 2 * DH * NJ * 8
OT0 = (QF0 + NU * NJ * DH, QF0)
OT_ROWS = (NU + 1) * NJ * (DH + 8)
PD0 = OT0[0] + OT_ROWS
AD0 = PD0 + 8 * NJ * 16
LD0 = AD0 + NJ * DH
PIN0 = (LD0 + NJ * 8, OT0[1] + OT_ROWS)
PACE0 = (PIN0[0] + NJ * 8, PIN0[1] + NJ * 8)
KS0 = 0
KX0 = KS0 + NM * 8
VS0 = KX0 + 16 * 8
QS0 = VS0 + NTILE * 8


def _round_rows(rows):
    return -(-rows // 32) * 32


def _plan_tiles():
    events = [((m + 1) * NV, 0, "m", m) for m in range(NM)]
    events += [((i + 1) * NM + VPU_SLOT * NV, 1, "v", i) for i in range(NV)]
    events.sort()
    tiles = []
    for t in range(NTILE):
        part = events[8 * t:8 * t + 8]
        tiles.append(([e[2:] for e in part], -(-max(e[0] for e in part) // NV)))
    return tiles


TILES = _plan_tiles()
PLACE = {key: (t, pos) for t, (keys, _) in enumerate(TILES) for pos, key in enumerate(keys)}
SOURCE = {8 * t + 7 - pos: key for key, (t, pos) in PLACE.items()}
PV_TIMES = sorted({(end + PV_LAG) % NM for _, end in TILES})
DEFERRED = [t for t, (_, end) in enumerate(TILES) if end + PV_LAG >= NM + DRAIN]
assert DEFERRED == [NTILE - 1] and PV_TIMES[0] > 0


def _layernorm(x):
    m = jnp.mean(x, axis=-1, keepdims=True)
    xc = x - m
    v = jnp.mean(xc * xc, axis=-1, keepdims=True)
    return xc * lax.rsqrt(v + EPS)


def _gelu(x):
    c = math.sqrt(2.0 / math.pi)
    return 0.5 * x * (1.0 + jnp.tanh(x * (c + (c * 0.044715) * (x * x))))


def _store_keys(chains, packed, group, keys):
    kind, idx = SOURCE[group]
    if kind == "v":
        for d in range(DH):
            o = KB0 + (idx * DH + d) * 16
            chains[d % 2][o:o + 16, :] = jnp.broadcast_to(keys[:, d:d + 1], (16, 128))
        return
    packed[KS0 + idx * 8:KS0 + (idx + 1) * 8, :] = pltpu.bitcast(keys.astype(BF), F32)
    first, last = PV_TIMES[-1], PV_TIMES[0]
    if idx >= first:
        o = KX0 + (idx - first) * 8
        packed[o:o + 8, :] = pltpu.bitcast(keys.astype(BF), F32)
    elif idx < last:
        o = KX0 + (NM - first + idx) * 8
        packed[o:o + 8, :] = pltpu.bitcast(pltpu.roll(keys, DH, 1).astype(BF), F32)


def _result_rows(u, j):
    return j % 2, OT0[j % 2] + (u * NJ + j) * (DH + 8)


def _result_stores(u, acc, sums):
    stores = []
    for j in range(NJ):
        c, row = _result_rows(u, j)
        stores.append((c, row + DH, sums[j]))
        for half in range(DH // 8):
            stores.append((c, row + half * 8, acc[half * 8:(half + 1) * 8, j * 128:(j + 1) * 128]))
    return stores


def _pv(packed, t, p):
    vt = pltpu.bitcast(packed[VS0 + t * 8:VS0 + (t + 1) * 8, :], BF)
    return jnp.dot(vt, p.astype(BF), preferred_element_type=F32)


def _carried_row(pos, j):
    return PD0 + (pos * NJ + j) * 16


def _carried_p(even):
    return jnp.concatenate(
        [jnp.concatenate([even[_carried_row(pos, j):_carried_row(pos, j) + 16, :] for j in range(NJ)], axis=1)
         for pos in range(7, -1, -1)], axis=0)


def _carried_acc(even):
    return jnp.concatenate([even[AD0 + j * DH:AD0 + (j + 1) * DH, :] for j in range(NJ)], axis=1)


def _carried_sums(even):
    return [even[LD0 + j * 8:LD0 + (j + 1) * 8, :] for j in range(NJ)]


def _query_row(h, d, j):
    return QB0 + (((h % 2) * DH + d) * NJ + j) * 8


def _broadcast_query(even, u, d, j):
    return jnp.broadcast_to(even[pl.ds(QF0 + (u * NJ + j) * DH + d, 1), :], (8, 128))


def _attention_units(it, chains, packed, zero):
    even = chains[0]
    u0 = it * HU
    ngrp = HU * NM
    pace_base = (PACE0[0] + zero * 8, PACE0[1] + zero * 8)
    queries, sums, accs, probs, scores, first_pv, pv_results = {}, {}, {}, {}, {}, {}, {}
    staged, late = [], []

    def stage_queries(h):
        u = u0 + h if h < HU else jnp.minimum(u0 + h, NU - 1)
        for d in range(DH):
            for j in range(NJ):
                staged.append((d % 2, _query_row(h, d, j), _broadcast_query(even, u, d, j)))
                yield

    def exponentiate(h, key, j, s):
        e = jnp.exp2(s)
        pair = e[0:8] + e[8:16]
        sums[h, j] = sums[h, j] + pair if (h, j) in sums else pair
        t, pos = PLACE[key]
        if h == HU - 1 and t in DEFERRED:
            even[_carried_row(pos, j):_carried_row(pos, j) + 16, :] = e
        else:
            probs[h, key, j] = e
        return e

    partial, count = {}, {}

    def vpu_scores(c):
        for h in range(HU):
            for i in range(NV):
                for j0 in range(0, NJ, 2):
                    for d in range(c, DH, 2):
                        o = KB0 + (i * DH + d) * 16
                        k = chains[c][o:o + 16, :].reshape(2, 8, 128)
                        for j in (j0, j0 + 1):
                            o = _query_row(h, d, j)
                            term = k * chains[c][o:o + 8, :][None]
                            key = (h, i, j)
                            partial[key] = partial[key] + term if key in partial else term
                            count[key] = count.get(key, 0) + 1
                            if count[key] == DH:
                                exponentiate(h, ("v", i), j, partial.pop(key).reshape(16, 128))
                        yield

    pv_at, result_at, pin_at = {}, {}, {}
    for h in range(-1, HU):
        for t, (_, end) in enumerate(TILES):
            if (h == -1 and t not in DEFERRED) or (h == HU - 1 and t in DEFERRED):
                continue
            x = h * NM + end + PV_LAG
            pv_at.setdefault(x, []).append((h, t))
            if t == NTILE - 1:
                result_at[x + STORE_LAG] = h
            if t == 0:
                pin_at[x + STORE_LAG] = h
    cuts = sorted({0, ngrp} | {x for x in pv_at if x < ngrp})
    runs = dict(zip(cuts[:-1], cuts[1:]))

    vpu = (vpu_scores(0), vpu_scores(1))
    vpu_steps = NV * DH
    done, paced = [0, 0], [0, 0]

    def slots(g):
        h, r = divmod(g, NM)
        return h * (NM + NTILE) + r + 1 + sum(1 for _, end in TILES if (end + PV_LAG) % NM <= r)

    def tick(values, slot):
        for c, o, v in staged:
            chains[c][o:o + 8, :] = v
        staged.clear()
        for c in range(2):
            for item in [item for item in late if item[0] == c][:1]:
                late[:] = [other for other in late if other is not item]
                o = item[1] if isinstance(item[1], int) else pl.multiple_of(item[1], 8)
                chains[c][pl.ds(o, 8), :] = item[2]
            if values:
                paced[c] += 1
                o = pl.multiple_of(pace_base[c] + 8 * (paced[c] % NPACE), 8)
                chains[c][pl.ds(o, 8), :] = values[c]
            want = ((2 * (slot + VPU_LEAD) + c + 1) * vpu_steps) // (2 * (NM + NTILE))
            while done[c] < min(want, HU * vpu_steps):
                next(vpu[c])
                done[c] += 1

    staging = {}
    for x in range(-Q_LEAD, ngrp + PV_LAG + EXP_LAG + 32):
        if (x + Q_LEAD) % NM == 0 and (x + Q_LEAD) // NM < HU:
            h = (x + Q_LEAD) // NM
            o = QS0 + (u0 + h) * (NJ * 8)
            queries[h] = pltpu.bitcast(jnp.concatenate(
                [packed[pl.ds(pl.multiple_of(o + j * 8, 8), 8), :] for j in range(NJ)], axis=1), BF)
        for h, t in pv_at.get(x, []):
            if h == -1:
                p = _carried_p(even)
                accs[h] = _carried_acc(even)
            else:
                p = jnp.concatenate([jnp.concatenate([probs.pop((h, key, j)) for j in range(NJ)], axis=1)
                                     for key in reversed(TILES[t][0])], axis=0)
            pv = _pv(packed, t, p)
            pv_results[x] = pv
            accs[h] = pv if t == 0 else accs[h] + pv
            if t == 0:
                first_pv[h] = pv
        if x in pin_at:
            for j in range(NJ):
                late.append((j % 2, PIN0[j % 2] + j * 8, first_pv[pin_at[x]][0:8, j * 128:(j + 1) * 128]))
        if x in result_at:
            h = result_at[x]
            if h == -1:
                late.extend(_result_stores((u0 + NU - 1) % NU, accs[h], _carried_sums(even)))
            else:
                late.extend(_result_stores(u0 + h, accs[h], [sums[h, j] for j in range(NJ)]))
        if x in runs:
            h = x // NM
            if runs[x] > (h + 1) * NM:
                k = pltpu.bitcast(packed[KX0:KX0 + (runs[x] - x) * 8, :], BF)
                s = jnp.dot(k[:, 0:2 * DH], jnp.concatenate([queries[h], queries[h + 1]], axis=0),
                            preferred_element_type=F32)
            else:
                k = pltpu.bitcast(packed[KS0 + (x - h * NM) * 8:KS0 + (runs[x] - h * NM) * 8, :], BF)
                s = jnp.dot(k[:, 0:DH], queries[h], preferred_element_type=F32)
            for g in range(x, runs[x]):
                scores[g] = s[(g - x) * 16:(g - x + 1) * 16]
        g = x - EXP_LAG
        values = None
        if 0 <= g < ngrp:
            if g in pv_results:
                pv = pv_results[g]
                tick((pv[0:8, PACE[0] * 128:(PACE[0] + 1) * 128], pv[8:16, PACE[1] * 128:(PACE[1] + 1) * 128]),
                     slots(g) - 2)
            s = scores.pop(g)
            e = [exponentiate(g // NM, ("m", g % NM), j, s[:, j * 128:(j + 1) * 128]) for j in range(NJ)]
            values = (e[PACE[0]][0:8], e[PACE[1]][8:16])
        tick(values, slots(g) - 1)
        h = (x + NM - 14) // NM
        if 1 <= h <= HU:
            if h not in staging:
                staging[h] = stage_queries(h)
            next(staging[h], None)
    for j in range(NJ):
        even[AD0 + j * DH:AD0 + (j + 1) * DH, :] = accs[HU - 1][:, j * 128:(j + 1) * 128]
        even[LD0 + j * 8:LD0 + (j + 1) * 8, :] = sums[HU - 1, j]
    assert not probs and not scores and not staged and not late and not partial


def _kernel(x_hbm, wq_hbm, wkt_hbm, wvt_hbm, wo_hbm, win_hbm, wsp_hbm, bsp_hbm, wout_hbm, c_hbm, wmod_hbm,
            out_hbm,
            even, odd, packed, xz, wq_v, wo_v, win_v, wsp_v, wout_v, wmod_v, wt_s, k_s, x1_s, out_s,
            gb_s, bias_s, bsp_v, c_v, flags, sems, out_sems):
    chains = (even, odd)
    copies = [
        (wq_hbm, wq_v), (c_hbm, c_v),
        (wkt_hbm, wt_s.at[pl.ds(D, DH)]), (wvt_hbm, wt_s.at[pl.ds(D + DH, DH)]),
        (wmod_hbm.at[pl.ds(0, D // 2), pl.ds(0, 2 * D)], wmod_v.at[pl.ds(0, D // 2), pl.ds(0, 2 * D)]),
        (wmod_hbm.at[pl.ds(D // 2, D // 2), pl.ds(0, 2 * D)], wmod_v.at[pl.ds(D // 2, D // 2), pl.ds(0, 2 * D)]),
        (wmod_hbm.at[:, pl.ds(2 * D, 4 * D)], wmod_v.at[:, pl.ds(2 * D, 4 * D)]),
        (wo_hbm, wo_v), (win_hbm, win_v), (bsp_hbm, bsp_v), (wout_hbm, wout_v), (wsp_hbm, wsp_v),
    ]
    copies += [(x_hbm.at[pl.ds(i * RA, RA)], xz.at[pl.ds(i * RA, RA), pl.ds(0, D)]) for i in range(S // RA)]
    copies = [pltpu.make_async_copy(src, dst, sems.at[i]) for i, (src, dst) in enumerate(copies)]
    cp_wq, cp_c, cp_wk, cp_wv = copies[0:4]
    cp_mod, cp_late, cp_x = copies[4:6], copies[6:12], copies[12:]
    for cp in (cp_wq, cp_c, cp_wk, cp_wv, cp_x[0], *cp_mod, *cp_x[1:]):
        cp.start()

    cp_wq.wait()
    wt_s[0:D, :] = wq_v[...].astype(F32).T.astype(BF)
    cp_wk.wait()
    cp_wv.wait()
    cp_c.wait()
    cond = jnp.broadcast_to(c_v[...].astype(F32), (16, D))
    cond = (cond * jax.nn.sigmoid(cond)).astype(BF)
    cp_x[0].wait()
    first_norm = _layernorm(xz[0:RA, 0:D].astype(F32))
    mod = None
    for i, cp in enumerate(cp_mod):
        cp.wait()
        rows = slice(i * (D // 2), (i + 1) * (D // 2))
        part = jnp.dot(cond[:, rows], wmod_v[rows, 0:2 * D], preferred_element_type=F32)
        mod = part if mod is None else mod + part
    shift_a = mod[0:1, 0:D]
    scale_a = 1.0 + mod[0:1, D:2 * D]

    def modulated(i):
        n = first_norm if i == 0 else _layernorm(xz[i * RA:(i + 1) * RA, 0:D].astype(F32))
        return (n * scale_a + shift_a).astype(BF)

    def project(i, h, stats):
        q_max, k_max, v_max = stats
        kvt = lax.dot_general(wt_s[D:D + 2 * DH, :], h, NT, preferred_element_type=F32)
        qt = lax.dot_general(wt_s[0:D, :], h, NT, preferred_element_type=F32)
        kt = kvt[0:DH].astype(BF).astype(F32)
        vt = kvt[DH:2 * DH].astype(BF)
        v_words = pltpu.bitcast(vt, F32)
        keys = jnp.concatenate([kt, jnp.zeros((128 - DH, RA), F32)], axis=0).T
        k_s[i * RA:(i + 1) * RA, :] = keys[:, 0:DH].astype(BF)
        for g in range(RA // 16):
            _store_keys(chains, packed, i * (RA // 16) + g, keys[g * 16:(g + 1) * 16, :])
        q = (qt * QSCALE).astype(BF)
        qf = q.astype(F32)
        q_words = pltpu.bitcast(q, F32)
        for jj in range(RA // 128):
            t = i * (RA // 128) + jj
            block, j = divmod(t, NJ)
            lanes = slice(jj * 128, (jj + 1) * 128)
            packed[VS0 + t * 8:VS0 + (t + 1) * 8, :] = v_words[:, lanes]
            for head in range(H):
                r = (block * H + head) * NJ + j
                packed[QS0 + r * 8:QS0 + (r + 1) * 8, :] = q_words[head * 8:(head + 1) * 8, lanes]
                even[QF0 + r * DH:QF0 + (r + 1) * DH, :] = qf[head * DH:(head + 1) * DH, lanes]
        q2 = (qf * qf).reshape(H, 2, 8, RA)
        q2 = jnp.max(q2[:, 0] + q2[:, 1], axis=0)
        for j in range(RA // 128):
            q_max = jnp.maximum(q_max, q2[:, j * 128:(j + 1) * 128])
        k_max = jnp.maximum(k_max, jnp.sum(kt * kt, axis=0, keepdims=True))
        v_max = jnp.maximum(v_max, jnp.abs(vt.astype(F32)))
        return q_max, k_max, v_max

    stats = (jnp.zeros((8, 128), F32), jnp.zeros((1, RA), F32), jnp.zeros((DH, RA), F32))
    arrived, hs = 1, {}
    for n, upto in enumerate(X_WAITS):
        while arrived <= upto:
            cp_x[arrived].wait()
            arrived += 1
        last = n == len(X_WAITS) - 1
        if last:
            for cp in cp_late:
                cp.start()
        for i in range(X_WAITS[n - 1] if n else 0, S // RA if last else upto):
            for ahead in (i, i + 1):
                if ahead < arrived and ahead not in hs:
                    hs[ahead] = modulated(ahead)
            stats = project(i, hs[i], stats)
            if (i + 1) * RA == QB:
                even[PD0:LD0, :] = jnp.zeros((LD0 - PD0, 128), F32)
                even[LD0:LD0 + NJ * 8, :] = jnp.ones((NJ * 8, 128), F32)
                for d in range(DH):
                    for j in range(NJ):
                        o = _query_row(0, d, j)
                        chains[d % 2][o:o + 8, :] = _broadcast_query(even, 0, d, j)
    q_max, k_max, v_max = stats
    bound = jnp.max(jnp.sum(q_max, axis=0, keepdims=True)) * jnp.max(k_max)
    v_top = jnp.max(v_max)
    safe = (bound <= SCORE_LIMIT * SCORE_LIMIT) & (v_top <= V_MAX) & (v_top >= V_MIN)
    flags[0] = jnp.where(safe, 0, 1)
    flags[1] = jnp.minimum(jnp.where(safe, 0, 1), 0)

    @pl.when(safe)
    def _unshifted():
        def body(it, carry):
            _attention_units(it, chains, packed, flags[0])
            return carry

        lax.fori_loop(0, NU // HU, body, 0)

    @pl.when(jnp.logical_not(safe))
    def _shifted_by_row_max():
        def body(it, carry):
            q = pltpu.bitcast(packed[pl.ds(pl.multiple_of(QS0 + it * 8, 8), 8), :], BF)
            s = jnp.dot(k_s[...], q, preferred_element_type=F32)
            e = jnp.exp2(s - jnp.max(s, axis=0, keepdims=True))
            total = jnp.sum(e, axis=0, keepdims=True)
            vt = pltpu.bitcast(jnp.concatenate(
                [packed[VS0 + t * 8:VS0 + (t + 1) * 8, :] for t in range(NTILE)], axis=1), BF)
            o = jnp.dot(vt, e.astype(BF), preferred_element_type=F32)
            o = jnp.concatenate([o, jnp.broadcast_to(total * 0.125, (8, 128))], axis=0)
            for c in range(2):
                chains[c][pl.ds(pl.multiple_of(OT0[c] + it * (DH + 8), 8), DH + 8), :] = o
            return carry

        lax.fori_loop(0, NU * NJ, body, 0)

    for cp in cp_late:
        cp.wait()
    acc = _carried_acc(even) + _pv(packed, NTILE - 1, _carried_p(even))
    for c, o, v in _result_stores(NU - 1 + flags[0], acc, _carried_sums(even)):
        chains[c][pl.ds(pl.multiple_of(o, 8), 8), :] = v

    def modulation(i):
        return jnp.dot(cond, wmod_v[:, i * D:(i + 1) * D], preferred_element_type=F32)[0:8]

    mods = []

    def mix(i):
        rows = slice(i * RC, (i + 1) * RC)
        block, j = divmod(i, NJ)
        heads = []
        for head in range(H):
            c, o = _result_rows(block * H + head, j)
            total = jnp.sum(chains[c][o + DH:o + DH + 8, :], axis=0, keepdims=True)
            r = pltpu.reciprocal(total, approx=True)
            heads.append(chains[c][o:o + DH, :] * (r * (2.0 - total * r)))
        attn = jnp.concatenate(heads, axis=0).T.astype(BF)
        if i == 0:
            mods.extend([modulation(2)[0:1], modulation(3)[0:1], 1.0 + modulation(4)[0:1]])
            gb_s[...] = modulation(5)
        gate_a, shift_b, scale_b = mods
        a = jnp.dot(attn, wo_v[...], preferred_element_type=F32)
        x1 = xz[rows, 0:D].astype(F32) + gate_a * a
        x1_s[rows, :] = x1
        return (_layernorm(x1) * scale_b + shift_b).astype(BF)

    zero = flags[1]
    h = mix(0)
    for i in range(S // RC):
        rows = pl.ds(pl.multiple_of(i * RC + zero, RC), RC)
        h_next = mix(i + 1) if i + 1 < S // RC else None
        z2 = _gelu(jnp.dot(h, win_v[:, FH:2 * FH], preferred_element_type=F32))
        xz[rows, D + FH:D + 2 * FH] = _layernorm(z2).astype(BF)
        z1 = _gelu(jnp.dot(h, win_v[:, 0:FH], preferred_element_type=F32))
        xz[rows, D:D + FH] = z1.astype(BF)
        h = h_next
    bias = bsp_v[...].astype(F32)
    for r in range(S // 128):
        bias_s[r * 128:(r + 1) * 128, :] = jnp.broadcast_to(bias[r:r + 1, :], (128, 128)).T

    def out_copy(i):
        rows = pl.ds(pl.multiple_of(i * RD, RD), RD)
        return pltpu.make_async_copy(out_s.at[rows], out_hbm.at[rows], out_sems.at[i])

    def gated(i):
        rows = pl.ds(pl.multiple_of(i * RD, RD), RD)
        g = jnp.dot(wsp_v[rows, :], xz[:, D + FH:D + 2 * FH], preferred_element_type=F32)
        g = g + jnp.concatenate([bias_s[rows, :]] * (FH // 128), axis=1)
        return (xz[rows, D:D + FH].astype(F32) * g).astype(BF)

    def finish(it, carry):
        ys = [gated(it * UD + u) for u in range(UD)]
        for u in range(UD):
            rows = pl.ds(pl.multiple_of((it * UD + u) * RD, RD), RD)
            o = jnp.dot(ys[u], wout_v[...], preferred_element_type=F32)
            out_s[rows, :] = (x1_s[rows, :] + gb_s[0:1, :] * o).astype(BF)
            out_copy(it * UD + u).start()
        return carry

    lax.fori_loop(0, S // RD // UD, finish, 0)
    for i in range(S // RD):
        out_copy(i).wait()


@jax.jit
def pallas_adaLN_cond__grouped_kv_mqa__mixer_gmlp__prompt_kernel(
    A_x: jax.Array,
    A_wq: jax.Array,
    A_wk: jax.Array,
    A_wv: jax.Array,
    A_wo: jax.Array,
    B_x: jax.Array,
    B_w_in: jax.Array,
    B_w_sp: jax.Array,
    B_b_sp: jax.Array,
    B_w_out: jax.Array,
    c: jax.Array,
    w_mod: jax.Array,
):
    del B_x
    vmem = pltpu.VMEM
    scratch = [
        vmem((_round_rows(PACE0[0] + (NPACE + 2) * 8), 128), F32),
        vmem((_round_rows(PACE0[1] + (NPACE + 2) * 8), 128), F32),
        vmem((_round_rows(QS0 + NU * NJ * 8), 128), F32),
        vmem((S, D + 2 * FH), BF),
        vmem((D, D), BF), vmem((D, D), BF), vmem((D, 2 * FH), BF), vmem((S, S), BF), vmem((FH, D), BF),
        vmem((D, 6 * D), BF), vmem((D + 2 * DH, D), BF), vmem((S, DH), BF),
        vmem((S, D), F32), vmem((S, D), BF), vmem((8, D), F32), vmem((S, 128), F32),
        vmem((S // 128, 128), BF), vmem((1, D), BF),
        pltpu.SMEM((2,), jnp.int32),
        pltpu.SemaphoreType.DMA((12 + S // RA,)), pltpu.SemaphoreType.DMA((S // RD,)),
    ]
    out = pl.pallas_call(
        _kernel,
        out_shape=jax.ShapeDtypeStruct((S, D), BF),
        in_specs=[pl.BlockSpec(memory_space=pl.ANY)] * 11,
        out_specs=pl.BlockSpec(memory_space=pl.ANY),
        scratch_shapes=scratch,
        compiler_params=pltpu.CompilerParams(vmem_limit_bytes=100 * 1024 * 1024),
        name="fused",
    )(A_x.reshape(S, D), A_wq, A_wk.T, A_wv.T, A_wo, B_w_in, B_w_sp, B_b_sp.reshape(S // 128, 128),
      B_w_out, c, w_mod)
    return out.reshape(1, S, D)
```

```python
import math

import jax
import jax.numpy as jnp
from jax import lax
from jax.experimental import pallas as pl
from jax.experimental.pallas import tpu as pltpu

BF = jnp.bfloat16
F32 = jnp.float32
S, D, H, DH, FH = 2048, 512, 32, 16, 896
EPS = 1e-5
QSCALE = DH ** -0.5 * math.log2(math.e)
NT = (((1,), (1,)), ((), ()))

SCORE_LIMIT = 96.0
V_MIN, V_MAX = 2.0 ** -16, 2.0 ** 16

QB = 512
NJ = QB // 128
NU = (S // QB) * H
NTILE = S // 128
RA = 256
X_WAITS = (1, 3, 7)
RC = 128
RD = 128
OUT_K = 384

HU = 8
NV = 19
NM = S // 16 - NV
PV_LAG = 9
EXP_LAG = 9
STORE_LAG = 10
Q_LEAD = 9
VPU_LEAD = 3
VPU_SLOT = -1
DRAIN = 4
PACE = (1, 2)
NPACE = 512
NFLAGS = 66

KB0 = 0
QB0 = KB0 + NV * DH * 16
QF0 = QB0 + 2 * DH * NJ * 8
OT0 = (QF0 + NU * NJ * DH, QF0)
OT_ROWS = (NU + 1) * NJ * (DH + 8)
PD0 = OT0[0] + OT_ROWS
AD0 = PD0 + 8 * NJ * 16
LD0 = AD0 + NJ * DH
PIN0 = (LD0 + NJ * 8, OT0[1] + OT_ROWS)
PACE0 = (PIN0[0] + NJ * 8, PIN0[1] + NJ * 8)
KS0 = 0
KX0 = KS0 + NM * 8
VS0 = KX0 + 16 * 8
QS0 = VS0 + NTILE * 8


def _round_rows(rows):
    return -(-rows // 32) * 32


def _plan_tiles():
    events = [((m + 1) * NV, 0, "m", m) for m in range(NM)]
    events += [((i + 1) * NM + VPU_SLOT * NV, 1, "v", i) for i in range(NV)]
    events.sort()
    tiles = []
    for t in range(NTILE):
        part = events[8 * t:8 * t + 8]
        tiles.append(([e[2:] for e in part], -(-max(e[0] for e in part) // NV)))
    return tiles


TILES = _plan_tiles()
PLACE = {key: (t, pos) for t, (keys, _) in enumerate(TILES) for pos, key in enumerate(keys)}
SOURCE = {8 * t + 7 - pos: key for key, (t, pos) in PLACE.items()}
PV_TIMES = sorted({(end + PV_LAG) % NM for _, end in TILES})
DEFERRED = [t for t, (_, end) in enumerate(TILES) if end + PV_LAG >= NM + DRAIN]
assert DEFERRED == [NTILE - 1] and PV_TIMES[0] > 0


STRASSEN = (
    (((1, 0),), ((1, 1), (-1, 3)), ((1, 1), (1, 3))),
    (((1, 0), (1, 1)), ((1, 3),), ((-1, 0), (1, 1))),
    (((1, 0), (1, 3)), ((1, 0), (1, 3)), ((1, 0), (1, 3))),
    (((1, 2), (1, 3)), ((1, 0),), ((1, 2), (-1, 3))),
    (((1, 2), (-1, 0)), ((1, 0), (1, 1)), ((1, 3),)),
    (((1, 3),), ((1, 2), (-1, 0)), ((1, 0), (1, 2))),
    (((1, 1), (-1, 3)), ((1, 2), (1, 3)), ((1, 0),)),
)


def _dot(a, b):
    return jnp.dot(a, b, preferred_element_type=F32)


def _combine(terms, blocks):
    out = blocks[terms[0][1]]
    for sign, i in terms[1:]:
        out = out + blocks[i] if sign > 0 else out - blocks[i]
    return out


def _scatter(acc, terms, m):
    for sign, i in terms:
        if acc[i] is None:
            acc[i] = (sign, m)
        elif acc[i][0] > 0:
            acc[i] = (1, acc[i][1] + m if sign > 0 else acc[i][1] - m)
        else:
            assert sign > 0
            acc[i] = (1, m - acc[i][1])


def _layernorm(x):
    m = jnp.mean(x, axis=-1, keepdims=True)
    xc = x - m
    v = jnp.mean(xc * xc, axis=-1, keepdims=True)
    return xc * lax.rsqrt(v + EPS)


def _gelu(x):
    c = math.sqrt(2.0 / math.pi)
    return 0.5 * x * (1.0 + jnp.tanh(x * (c + (c * 0.044715) * (x * x))))


def _store_keys(chains, packed, group, keys):
    kind, idx = SOURCE[group]
    if kind == "v":
        for d in range(DH):
            o = KB0 + (idx * DH + d) * 16
            chains[d % 2][o:o + 16, :] = jnp.broadcast_to(keys[:, d:d + 1], (16, 128))
        return
    packed[KS0 + idx * 8:KS0 + (idx + 1) * 8, :] = pltpu.bitcast(keys.astype(BF), F32)
    first, last = PV_TIMES[-1], PV_TIMES[0]
    if idx >= first:
        o = KX0 + (idx - first) * 8
        packed[o:o + 8, :] = pltpu.bitcast(keys.astype(BF), F32)
    elif idx < last:
        o = KX0 + (NM - first + idx) * 8
        packed[o:o + 8, :] = pltpu.bitcast(pltpu.roll(keys, DH, 1).astype(BF), F32)


def _result_rows(u, j):
    return j % 2, OT0[j % 2] + (u * NJ + j) * (DH + 8)


def _result_stores(u, acc, sums):
    stores = []
    for j in range(NJ):
        c, row = _result_rows(u, j)
        stores.append((c, row + DH, sums[j]))
        for half in range(DH // 8):
            stores.append((c, row + half * 8, acc[half * 8:(half + 1) * 8, j * 128:(j + 1) * 128]))
    return stores


def _pv(packed, t, p):
    vt = pltpu.bitcast(packed[VS0 + t * 8:VS0 + (t + 1) * 8, :], BF)
    return jnp.dot(vt, p.astype(BF), preferred_element_type=F32)


def _carried_row(pos, j):
    return PD0 + (pos * NJ + j) * 16


def _carried_p(even):
    return jnp.concatenate(
        [jnp.concatenate([even[_carried_row(pos, j):_carried_row(pos, j) + 16, :] for j in range(NJ)], axis=1)
         for pos in range(7, -1, -1)], axis=0)


def _carried_acc(even):
    return jnp.concatenate([even[AD0 + j * DH:AD0 + (j + 1) * DH, :] for j in range(NJ)], axis=1)


def _carried_sums(even):
    return [even[LD0 + j * 8:LD0 + (j + 1) * 8, :] for j in range(NJ)]


def _query_row(h, d, j):
    return QB0 + (((h % 2) * DH + d) * NJ + j) * 8


def _broadcast_query(even, u, d, j):
    return jnp.broadcast_to(even[pl.ds(QF0 + (u * NJ + j) * DH + d, 1), :], (8, 128))


def _attention_units(it, chains, packed, zero):
    even = chains[0]
    u0 = it * HU
    ngrp = HU * NM
    pace_base = (PACE0[0] + zero * 8, PACE0[1] + zero * 8)
    queries, sums, accs, probs, scores, first_pv, pv_results = {}, {}, {}, {}, {}, {}, {}
    staged, late = [], []

    def stage_queries(h):
        u = u0 + h if h < HU else jnp.minimum(u0 + h, NU - 1)
        for d in range(DH):
            for j in range(NJ):
                staged.append((d % 2, _query_row(h, d, j), _broadcast_query(even, u, d, j)))
                yield

    def exponentiate(h, key, j, s):
        e = jnp.exp2(s)
        pair = e[0:8] + e[8:16]
        sums[h, j] = sums[h, j] + pair if (h, j) in sums else pair
        t, pos = PLACE[key]
        if h == HU - 1 and t in DEFERRED:
            even[_carried_row(pos, j):_carried_row(pos, j) + 16, :] = e
        else:
            probs[h, key, j] = e
        return e

    partial, count = {}, {}

    def vpu_scores(c):
        for h in range(HU):
            for i in range(NV):
                for j0 in range(0, NJ, 2):
                    for d in range(c, DH, 2):
                        o = KB0 + (i * DH + d) * 16
                        k = chains[c][o:o + 16, :].reshape(2, 8, 128)
                        for j in (j0, j0 + 1):
                            o = _query_row(h, d, j)
                            term = k * chains[c][o:o + 8, :][None]
                            key = (h, i, j)
                            partial[key] = partial[key] + term if key in partial else term
                            count[key] = count.get(key, 0) + 1
                            if count[key] == DH:
                                exponentiate(h, ("v", i), j, partial.pop(key).reshape(16, 128))
                        yield

    pv_at, result_at, pin_at = {}, {}, {}
    for h in range(-1, HU):
        for t, (_, end) in enumerate(TILES):
            if (h == -1 and t not in DEFERRED) or (h == HU - 1 and t in DEFERRED):
                continue
            x = h * NM + end + PV_LAG
            pv_at.setdefault(x, []).append((h, t))
            if t == NTILE - 1:
                result_at[x + STORE_LAG] = h
            if t == 0:
                pin_at[x + STORE_LAG] = h
    cuts = sorted({0, ngrp} | {x for x in pv_at if x < ngrp})
    runs = dict(zip(cuts[:-1], cuts[1:]))

    vpu = (vpu_scores(0), vpu_scores(1))
    vpu_steps = NV * DH
    done, paced = [0, 0], [0, 0]

    def slots(g):
        h, r = divmod(g, NM)
        return h * (NM + NTILE) + r + 1 + sum(1 for _, end in TILES if (end + PV_LAG) % NM <= r)

    def tick(values, slot):
        for c, o, v in staged:
            chains[c][o:o + 8, :] = v
        staged.clear()
        for c in range(2):
            for item in [item for item in late if item[0] == c][:1]:
                late[:] = [other for other in late if other is not item]
                o = item[1] if isinstance(item[1], int) else pl.multiple_of(item[1], 8)
                chains[c][pl.ds(o, 8), :] = item[2]
            if values:
                paced[c] += 1
                o = pl.multiple_of(pace_base[c] + 8 * (paced[c] % NPACE), 8)
                chains[c][pl.ds(o, 8), :] = values[c]
            want = ((2 * (slot + VPU_LEAD) + c + 1) * vpu_steps * 4 + 6 * (NM + NTILE)) // (8 * (NM + NTILE))
            while done[c] < min(want, HU * vpu_steps):
                next(vpu[c])
                done[c] += 1

    staging = {}
    for x in range(-Q_LEAD, ngrp + PV_LAG + EXP_LAG + 32):
        if (x + Q_LEAD) % NM == 0 and (x + Q_LEAD) // NM < HU:
            h = (x + Q_LEAD) // NM
            o = QS0 + (u0 + h) * (NJ * 8)
            queries[h] = pltpu.bitcast(jnp.concatenate(
                [packed[pl.ds(pl.multiple_of(o + j * 8, 8), 8), :] for j in range(NJ)], axis=1), BF)
        for h, t in pv_at.get(x, []):
            if h == -1:
                p = _carried_p(even)
                accs[h] = _carried_acc(even)
            else:
                p = jnp.concatenate([jnp.concatenate([probs.pop((h, key, j)) for j in range(NJ)], axis=1)
                                     for key in reversed(TILES[t][0])], axis=0)
            pv = _pv(packed, t, p)
            pv_results[x] = pv
            accs[h] = pv if t == 0 else accs[h] + pv
            if t == 0:
                first_pv[h] = pv
        if x in pin_at:
            for j in range(NJ):
                late.append((j % 2, PIN0[j % 2] + j * 8, first_pv[pin_at[x]][0:8, j * 128:(j + 1) * 128]))
        if x in result_at:
            h = result_at[x]
            if h == -1:
                late.extend(_result_stores((u0 + NU - 1) % NU, accs[h], _carried_sums(even)))
            else:
                late.extend(_result_stores(u0 + h, accs[h], [sums[h, j] for j in range(NJ)]))
        if x in runs:
            h = x // NM
            if runs[x] > (h + 1) * NM:
                k = pltpu.bitcast(packed[KX0:KX0 + (runs[x] - x) * 8, :], BF)
                s = jnp.dot(k[:, 0:2 * DH], jnp.concatenate([queries[h], queries[h + 1]], axis=0),
                            preferred_element_type=F32)
            else:
                k = pltpu.bitcast(packed[KS0 + (x - h * NM) * 8:KS0 + (runs[x] - h * NM) * 8, :], BF)
                s = jnp.dot(k[:, 0:DH], queries[h], preferred_element_type=F32)
            for g in range(x, runs[x]):
                scores[g] = s[(g - x) * 16:(g - x + 1) * 16]
        g = x - EXP_LAG
        values = None
        if 0 <= g < ngrp:
            if g in pv_results:
                pv = pv_results[g]
                tick((pv[0:8, PACE[0] * 128:(PACE[0] + 1) * 128], pv[8:16, PACE[1] * 128:(PACE[1] + 1) * 128]),
                     slots(g) - 2)
            s = scores.pop(g)
            e = [exponentiate(g // NM, ("m", g % NM), j, s[:, j * 128:(j + 1) * 128]) for j in range(NJ)]
            values = (e[PACE[0]][0:8], e[PACE[1]][8:16])
        tick(values, slots(g) - 1)
        h, r = divmod(x + NM - 14, NM)
        if 1 <= h <= HU:
            if h not in staging:
                staging[h] = [stage_queries(h), 0]
            while staging[h][1] < min(DH * NJ, ((r + 1) * 4) // 5):
                next(staging[h][0])
                staging[h][1] += 1
    for j in range(NJ):
        even[AD0 + j * DH:AD0 + (j + 1) * DH, :] = accs[HU - 1][:, j * 128:(j + 1) * 128]
        even[LD0 + j * 8:LD0 + (j + 1) * 8, :] = sums[HU - 1, j]
    assert not probs and not scores and not staged and not late and not partial


def _kernel(x_hbm, wq_hbm, wkt_hbm, wvt_hbm, wo_hbm, win_hbm, wsp_hbm, bsp_hbm, wout_hbm, c_hbm, wmod_hbm,
            out_hbm,
            even, odd, packed, xz, wq_v, wo_v, win_v, wsp_v, wout_v, wmod_v, wt_s, k_s, x1_s, out_s,
            z2_s, wout_s, gb_s, bias_s, bsp_v, c_v, flags, sems, out_sems):
    chains = (even, odd)
    copies = [
        (wq_hbm, wq_v), (c_hbm, c_v),
        (wkt_hbm, wt_s.at[pl.ds(D, DH)]), (wvt_hbm, wt_s.at[pl.ds(D + DH, DH)]),
        (wmod_hbm.at[pl.ds(0, D // 2), pl.ds(0, 2 * D)], wmod_v.at[pl.ds(0, D // 2), pl.ds(0, 2 * D)]),
        (wmod_hbm.at[pl.ds(D // 2, D // 2), pl.ds(0, 2 * D)], wmod_v.at[pl.ds(D // 2, D // 2), pl.ds(0, 2 * D)]),
        (wmod_hbm.at[:, pl.ds(2 * D, 4 * D)], wmod_v.at[:, pl.ds(2 * D, 4 * D)]),
        (wo_hbm, wo_v), (win_hbm, win_v), (bsp_hbm, bsp_v), (wout_hbm, wout_v), (wsp_hbm, wsp_v),
    ]
    copies += [(x_hbm.at[pl.ds(i * RA, RA)], xz.at[pl.ds(i * RA, RA), pl.ds(0, D)]) for i in range(S // RA)]
    copies = [pltpu.make_async_copy(src, dst, sems.at[i]) for i, (src, dst) in enumerate(copies)]
    cp_wq, cp_c, cp_wk, cp_wv = copies[0:4]
    cp_mod, cp_late, cp_x = copies[4:6], copies[6:12], copies[12:]
    for cp in (cp_wq, cp_c, cp_wk, cp_wv, cp_x[0], *cp_mod, *cp_x[1:]):
        cp.start()

    cp_wq.wait()
    wt_s[0:D, :] = wq_v[...].astype(F32).T.astype(BF)
    cp_wk.wait()
    cp_wv.wait()
    cp_c.wait()
    cond = jnp.broadcast_to(c_v[...].astype(F32), (16, D))
    cond = (cond * jax.nn.sigmoid(cond)).astype(BF)
    cp_x[0].wait()
    first_norm = _layernorm(xz[0:RA, 0:D].astype(F32))
    mod = None
    for i, cp in enumerate(cp_mod):
        cp.wait()
        rows = slice(i * (D // 2), (i + 1) * (D // 2))
        part = jnp.dot(cond[:, rows], wmod_v[rows, 0:2 * D], preferred_element_type=F32)
        mod = part if mod is None else mod + part
    shift_a = mod[0:1, 0:D]
    scale_a = 1.0 + mod[0:1, D:2 * D]

    def modulated(i):
        n = first_norm if i == 0 else _layernorm(xz[i * RA:(i + 1) * RA, 0:D].astype(F32))
        return (n * scale_a + shift_a).astype(BF)

    def project(i, h, stats):
        q_max, k_max, v_max = stats
        kvt = lax.dot_general(wt_s[D:D + 2 * DH, :], h, NT, preferred_element_type=F32)
        qt = lax.dot_general(wt_s[0:D, :], h, NT, preferred_element_type=F32)
        kt = kvt[0:DH].astype(BF).astype(F32)
        vt = kvt[DH:2 * DH].astype(BF)
        v_words = pltpu.bitcast(vt, F32)
        keys = jnp.concatenate([kt, jnp.zeros((128 - DH, RA), F32)], axis=0).T
        k_s[i * RA:(i + 1) * RA, :] = keys[:, 0:DH].astype(BF)
        for g in range(RA // 16):
            _store_keys(chains, packed, i * (RA // 16) + g, keys[g * 16:(g + 1) * 16, :])
        q = (qt * QSCALE).astype(BF)
        qf = q.astype(F32)
        q_words = pltpu.bitcast(q, F32)
        for jj in range(RA // 128):
            t = i * (RA // 128) + jj
            block, j = divmod(t, NJ)
            lanes = slice(jj * 128, (jj + 1) * 128)
            packed[VS0 + t * 8:VS0 + (t + 1) * 8, :] = v_words[:, lanes]
            for head in range(H):
                r = (block * H + head) * NJ + j
                packed[QS0 + r * 8:QS0 + (r + 1) * 8, :] = q_words[head * 8:(head + 1) * 8, lanes]
                even[QF0 + r * DH:QF0 + (r + 1) * DH, :] = qf[head * DH:(head + 1) * DH, lanes]
        q2 = (qf * qf).reshape(H, 2, 8, RA)
        q2 = jnp.max(q2[:, 0] + q2[:, 1], axis=0)
        for j in range(RA // 128):
            q_max = jnp.maximum(q_max, q2[:, j * 128:(j + 1) * 128])
        k_max = jnp.maximum(k_max, jnp.sum(kt * kt, axis=0, keepdims=True))
        v_max = jnp.maximum(v_max, jnp.abs(vt.astype(F32)))
        return q_max, k_max, v_max

    stats = (jnp.zeros((8, 128), F32), jnp.zeros((1, RA), F32), jnp.zeros((DH, RA), F32))
    arrived, hs = 1, {}
    for n, upto in enumerate(X_WAITS):
        while arrived <= upto:
            cp_x[arrived].wait()
            arrived += 1
        last = n == len(X_WAITS) - 1
        if last:
            for cp in cp_late:
                cp.start()
        for i in range(X_WAITS[n - 1] if n else 0, S // RA if last else upto):
            for ahead in (i, i + 1):
                if ahead < arrived and ahead not in hs:
                    hs[ahead] = modulated(ahead)
            stats = project(i, hs[i], stats)
            if (i + 1) * RA == QB:
                even[PD0:LD0, :] = jnp.zeros((LD0 - PD0, 128), F32)
                even[LD0:LD0 + NJ * 8, :] = jnp.ones((NJ * 8, 128), F32)
                for d in range(DH):
                    for j in range(NJ):
                        o = _query_row(0, d, j)
                        chains[d % 2][o:o + 8, :] = _broadcast_query(even, 0, d, j)
    q_max, k_max, v_max = stats
    bound = jnp.max(jnp.sum(q_max, axis=0, keepdims=True)) * jnp.max(k_max)
    v_top = jnp.max(v_max)
    safe = (bound <= SCORE_LIMIT * SCORE_LIMIT) & (v_top <= V_MAX) & (v_top >= V_MIN)
    flags[0] = jnp.where(safe, 0, 1)
    for n in range(1, NFLAGS):
        flags[n] = jnp.minimum(jnp.where(safe, 0, 1), 0)

    @pl.when(safe)
    def _unshifted():
        def body(it, carry):
            _attention_units(it, chains, packed, flags[0])
            return carry

        lax.fori_loop(0, NU // HU, body, 0)

    @pl.when(jnp.logical_not(safe))
    def _shifted_by_row_max():
        def body(it, carry):
            q = pltpu.bitcast(packed[pl.ds(pl.multiple_of(QS0 + it * 8, 8), 8), :], BF)
            s = jnp.dot(k_s[...], q, preferred_element_type=F32)
            e = jnp.exp2(s - jnp.max(s, axis=0, keepdims=True))
            total = jnp.sum(e, axis=0, keepdims=True)
            vt = pltpu.bitcast(jnp.concatenate(
                [packed[VS0 + t * 8:VS0 + (t + 1) * 8, :] for t in range(NTILE)], axis=1), BF)
            o = jnp.dot(vt, e.astype(BF), preferred_element_type=F32)
            o = jnp.concatenate([o, jnp.broadcast_to(total * 0.125, (8, 128))], axis=0)
            for c in range(2):
                chains[c][pl.ds(pl.multiple_of(OT0[c] + it * (DH + 8), 8), DH + 8), :] = o
            return carry

        lax.fori_loop(0, NU * NJ, body, 0)

    for cp in cp_late:
        cp.wait()
    acc = _carried_acc(even) + _pv(packed, NTILE - 1, _carried_p(even))
    for c, o, v in _result_stores(NU - 1 + flags[0], acc, _carried_sums(even)):
        chains[c][pl.ds(pl.multiple_of(o, 8), 8), :] = v

    def modulation(i):
        return jnp.dot(cond, wmod_v[:, i * D:(i + 1) * D], preferred_element_type=F32)[0:8]

    gate_a, shift_b, scale_b = modulation(2)[0:1], modulation(3)[0:1], 1.0 + modulation(4)[0:1]
    gb_s[...] = modulation(5)
    blocks = [wout_v[k * OUT_K:(k + 1) * OUT_K, n * (D // 2):(n + 1) * (D // 2)].astype(F32)
              for k in range(2) for n in range(2)]
    for n, (_, terms, _) in enumerate(STRASSEN):
        if len(terms) > 1:
            wout_s[:, n * (D // 2):(n + 1) * (D // 2)] = _combine(terms, blocks).astype(BF)

    def mix(i):
        rows = slice(i * RC, (i + 1) * RC)
        block, j = divmod(i, NJ)
        heads = []
        for head in range(H):
            c, o = _result_rows(block * H + head, j)
            total = jnp.sum(chains[c][o + DH:o + DH + 8, :], axis=0, keepdims=True)
            r = pltpu.reciprocal(total, approx=True)
            heads.append(chains[c][o:o + DH, :] * (r * (2.0 - total * r)))
        a = _dot(jnp.concatenate(heads, axis=0).T.astype(BF), wo_v[...])
        x1 = xz[rows, 0:D].astype(F32) + gate_a * a
        x1_s[rows, :] = x1
        return (_layernorm(x1) * scale_b + shift_b).astype(BF)

    zero = flags[1]
    h = mix(0)
    for i in range(S // RC):
        rows = pl.ds(pl.multiple_of(i * RC + zero, RC), RC)
        h_next = mix(i + 1) if i + 1 < S // RC else None
        z2 = _gelu(_dot(h, win_v[:, FH:2 * FH]))
        xz[rows, D + FH:D + 2 * FH] = _layernorm(z2).astype(BF)
        z1 = _gelu(_dot(h, win_v[:, 0:FH]))
        xz[rows, D:D + FH] = z1.astype(BF)
        h = h_next
    bias = bsp_v[...].astype(F32)
    for r in range(S // 128):
        bias_s[r * 128:(r + 1) * 128, 0:128] = jnp.broadcast_to(bias[r:r + 1, :], (128, 128)).T

    def out_copy(i):
        rows = pl.ds(pl.multiple_of(i * RD, RD), RD)
        return pltpu.make_async_copy(out_s.at[rows], out_hbm.at[rows], out_sems.at[i])

    quarter = S // 4

    def prepare(it, carry):
        rows = pl.ds(pl.multiple_of(it * quarter, quarter), quarter)
        bias_s[rows, 128:256] = bias_s[rows, 0:128] + _dot(wsp_v[rows, :], xz[:, D + FH + 768:D + 2 * FH])
        for r0 in range(0, RD, 16):
            z = [xz[pl.ds(pl.multiple_of(q * quarter + it * RD + r0, 16), 16), D + FH:D + FH + 768].astype(F32)
                 for q in range(4)]
            part = pl.ds(pl.multiple_of(it * RD + r0, 16), 16)
            for p1, (_, b1, _) in enumerate(STRASSEN):
                y = [_combine(b1, [z[2 * ka + kb][:, (2 * na + nb) * 128:(2 * na + nb + 1) * 128]
                                   for ka in range(2) for na in range(2)])
                     for kb in range(2) for nb in range(2)]
                for p2, (_, b2, _) in enumerate(STRASSEN):
                    n = p1 * 7 + p2
                    if len(b1) * len(b2) > 1:
                        z2_s[part, n * 128:(n + 1) * 128] = _combine(b2, y).astype(BF)
                for kb in range(2):
                    n = 49 + 2 * p1 + kb
                    if len(b1) > 1:
                        z2_s[part, n * 128:(n + 1) * 128] = _combine(
                            b1, [z[2 * ka + kb][:, 512 + na * 128:512 + (na + 1) * 128]
                                 for ka in range(2) for na in range(2)]).astype(BF)
        return carry

    lax.fori_loop(0, quarter // RD, prepare, 0)

    def finish(it, carry):
        rows = [pl.ds(pl.multiple_of(q * quarter + it * RD, RD), RD) for q in range(4)]

        def product(n, terms, width, rhs):
            base = it * RD + flags[2 + n]
            lhs = [wsp_v[pl.ds(pl.multiple_of(q * quarter + base, RD), RD), col:col + width]
                   for _, q, col in terms]
            if len(terms) > 1:
                lhs = [_combine([(sign, i) for i, (sign, _, _) in enumerate(terms)],
                                [block.astype(F32) for block in lhs]).astype(BF)]
            return _dot(lhs[0], rhs)

        def two_levels(p1, p2):
            (a1, b1, _), (a2, b2, _) = STRASSEN[p1], STRASSEN[p2]
            n = p1 * 7 + p2
            if len(b1) * len(b2) > 1:
                rhs = z2_s[:, n * 128:(n + 1) * 128]
            else:
                (ka, na), (kb, nb) = divmod(b1[0][1], 2), divmod(b2[0][1], 2)
                col = D + FH + (2 * na + nb) * 128
                rhs = xz[(2 * ka + kb) * quarter:(2 * ka + kb + 1) * quarter, col:col + 128]
            terms = [(s1 * s2, 2 * (i1 // 2) + i2 // 2, (2 * (i1 % 2) + i2 % 2) * quarter)
                     for s1, i1 in a1 for s2, i2 in a2]
            return product(n, terms, quarter, rhs)

        def one_level(p1, b):
            a1, b1, _ = STRASSEN[p1]
            if len(b1) > 1:
                col = (49 + 2 * p1) * 128
                rhs = jnp.concatenate([z2_s[:, col:col + 128], z2_s[:, col + 128:col + 256]], axis=0)
            else:
                ka, na = divmod(b1[0][1], 2)
                col = D + FH + 512 + na * 128
                rhs = xz[ka * (S // 2):(ka + 1) * (S // 2), col:col + 128]
            terms = [(s1, 2 * (i1 // 2) + b, (i1 % 2) * (S // 2)) for s1, i1 in a1]
            return product(49 + 2 * p1 + b, terms, S // 2, rhs)

        two = [[None] * 4 for _ in range(4)]
        one = [[None] * 4 for _ in range(2)]
        for p1, (_, _, c1) in enumerate(STRASSEN):
            inner = [None] * 4
            for p2, (_, _, c2) in enumerate(STRASSEN):
                _scatter(inner, c2, two_levels(p1, p2))
            for k in range(4):
                _scatter(two[k], c1, inner[k][1])
            for b in range(2):
                _scatter(one[b], c1, one_level(p1, b))
        ys = []
        for q in range(4):
            a, b = divmod(q, 2)
            parts = [two[2 * b + nb][2 * a + na][1] for na in range(2) for nb in range(2)]
            parts += [one[b][2 * a][1], one[b][2 * a + 1][1]]
            bias_q = bias_s[rows[q], 0:128]
            g = jnp.concatenate([part + bias_q for part in parts] + [bias_s[rows[q], 128:256]], axis=1)
            ys.append(xz[rows[q], D:D + FH].astype(F32) * g)
        for b in range(2):
            blocks = [ys[q][:, k * OUT_K:(k + 1) * OUT_K] for q in (b, b + 2) for k in range(2)]
            acc = [None] * 4
            for n, (a_terms, b_terms, c_terms) in enumerate(STRASSEN):
                if len(b_terms) > 1:
                    rhs = wout_s[:, n * (D // 2):(n + 1) * (D // 2)]
                else:
                    k, m = divmod(b_terms[0][1], 2)
                    rhs = wout_v[k * OUT_K:(k + 1) * OUT_K, m * (D // 2):(m + 1) * (D // 2)]
                _scatter(acc, c_terms, _dot(_combine(a_terms, blocks).astype(BF), rhs))
            for n, q in enumerate((b, b + 2)):
                rest = _dot(ys[q][:, 2 * OUT_K:FH].astype(BF), wout_v[2 * OUT_K:FH, :])
                mixed = jnp.concatenate([acc[2 * n][1], acc[2 * n + 1][1]], axis=1) + rest
                out_s[rows[q], :] = (x1_s[rows[q], :] + gb_s[0:1, :] * mixed).astype(BF)
                out_copy(q * (quarter // RD) + it).start()
        return carry

    lax.fori_loop(0, S // 4 // RD, finish, 0)
    for i in range(S // RD):
        out_copy(i).wait()


@jax.jit
def pallas_adaLN_cond__grouped_kv_mqa__mixer_gmlp__prompt_kernel(
    A_x: jax.Array,
    A_wq: jax.Array,
    A_wk: jax.Array,
    A_wv: jax.Array,
    A_wo: jax.Array,
    B_x: jax.Array,
    B_w_in: jax.Array,
    B_w_sp: jax.Array,
    B_b_sp: jax.Array,
    B_w_out: jax.Array,
    c: jax.Array,
    w_mod: jax.Array,
):
    del B_x
    vmem = pltpu.VMEM
    scratch = [
        vmem((_round_rows(PACE0[0] + (NPACE + 2) * 8), 128), F32),
        vmem((_round_rows(PACE0[1] + (NPACE + 2) * 8), 128), F32),
        vmem((_round_rows(QS0 + NU * NJ * 8), 128), F32),
        vmem((S, D + 2 * FH), BF),
        vmem((D, D), BF), vmem((D, D), BF), vmem((D, 2 * FH), BF), vmem((S, S), BF), vmem((FH, D), BF),
        vmem((D, 6 * D), BF), vmem((D + 2 * DH, D), BF), vmem((S, DH), BF),
        vmem((S, D), F32), vmem((S, D), BF),
        vmem((S // 4, (49 + 14) * 128), BF), vmem((OUT_K, 7 * D // 2), BF),
        vmem((8, D), F32), vmem((S, 256), F32),
        vmem((S // 128, 128), BF), vmem((1, D), BF),
        pltpu.SMEM((NFLAGS,), jnp.int32),
        pltpu.SemaphoreType.DMA((12 + S // RA,)), pltpu.SemaphoreType.DMA((S // RD,)),
    ]
    out = pl.pallas_call(
        _kernel,
        out_shape=jax.ShapeDtypeStruct((S, D), BF),
        in_specs=[pl.BlockSpec(memory_space=pl.ANY)] * 11,
        out_specs=pl.BlockSpec(memory_space=pl.ANY),
        scratch_shapes=scratch,
        compiler_params=pltpu.CompilerParams(vmem_limit_bytes=110 * 1024 * 1024),
        name="fused",
    )(A_x.reshape(S, D), A_wq, A_wk.T, A_wv.T, A_wo, B_w_in, B_w_sp, B_b_sp.reshape(S // 128, 128),
      B_w_out, c, w_mod)
    return out.reshape(1, S, D)
```

```python
import math

import jax
import jax.numpy as jnp
from jax import lax
from jax.experimental import pallas as pl
from jax.experimental.pallas import tpu as pltpu

BF = jnp.bfloat16
F32 = jnp.float32
S, D, H, DH, FH = 2048, 512, 32, 16, 896
EPS = 1e-5
QSCALE = DH ** -0.5 * math.log2(math.e)
NT = (((1,), (1,)), ((), ()))

SCORE_LIMIT = 96.0
V_MIN, V_MAX = 2.0 ** -16, 2.0 ** 16

QB = 512
NJ = QB // 128
NU = (S // QB) * H
NTILE = S // 128
RA = 256
X_WAITS = (1, 3, 7)
RC = 128
RD = 128
OUT_K = 384

HU = 8
NV = 19
NM = S // 16 - NV
PV_LAG = 9
EXP_LAG = 9
STORE_LAG = 10
Q_LEAD = 9
VPU_LEAD = 3
VPU_SLOT = -1
DRAIN = 4
PACE = (1, 2)
NPACE = 512
NFLAGS = 66

KB0 = 0
QB0 = KB0 + NV * DH * 16
QF0 = QB0 + 2 * DH * NJ * 8
OT0 = (QF0 + NU * NJ * DH, QF0)
OT_ROWS = (NU + 1) * NJ * (DH + 8)
PD0 = OT0[0] + OT_ROWS
AD0 = PD0 + 8 * NJ * 16
LD0 = AD0 + NJ * DH
PIN0 = (LD0 + NJ * 8, OT0[1] + OT_ROWS)
PACE0 = (PIN0[0] + NJ * 8, PIN0[1] + NJ * 8)
KS0 = 0
KX0 = KS0 + NM * 8
VS0 = KX0 + 16 * 8
QS0 = VS0 + NTILE * 8


def _round_rows(rows):
    return -(-rows // 32) * 32


def _plan_tiles():
    events = [((m + 1) * NV, 0, "m", m) for m in range(NM)]
    events += [((i + 1) * NM + VPU_SLOT * NV, 1, "v", i) for i in range(NV)]
    events.sort()
    tiles = []
    for t in range(NTILE):
        part = events[8 * t:8 * t + 8]
        tiles.append(([e[2:] for e in part], -(-max(e[0] for e in part) // NV)))
    return tiles


TILES = _plan_tiles()
PLACE = {key: (t, pos) for t, (keys, _) in enumerate(TILES) for pos, key in enumerate(keys)}
SOURCE = {8 * t + 7 - pos: key for key, (t, pos) in PLACE.items()}
PV_TIMES = sorted({(end + PV_LAG) % NM for _, end in TILES})
DEFERRED = [t for t, (_, end) in enumerate(TILES) if end + PV_LAG >= NM + DRAIN]
assert DEFERRED == [NTILE - 1] and PV_TIMES[0] > 0


STRASSEN = (
    (((1, 0),), ((1, 1), (-1, 3)), ((1, 1), (1, 3))),
    (((1, 0), (1, 1)), ((1, 3),), ((-1, 0), (1, 1))),
    (((1, 0), (1, 3)), ((1, 0), (1, 3)), ((1, 0), (1, 3))),
    (((1, 2), (1, 3)), ((1, 0),), ((1, 2), (-1, 3))),
    (((1, 2), (-1, 0)), ((1, 0), (1, 1)), ((1, 3),)),
    (((1, 3),), ((1, 2), (-1, 0)), ((1, 0), (1, 2))),
    (((1, 1), (-1, 3)), ((1, 2), (1, 3)), ((1, 0),)),
)


def _dot(a, b):
    return jnp.dot(a, b, preferred_element_type=F32)


def _combine(terms, blocks):
    out = blocks[terms[0][1]]
    for sign, i in terms[1:]:
        out = out + blocks[i] if sign > 0 else out - blocks[i]
    return out


def _scatter(acc, terms, m):
    for sign, i in terms:
        if acc[i] is None:
            acc[i] = (sign, m)
        elif acc[i][0] > 0:
            acc[i] = (1, acc[i][1] + m if sign > 0 else acc[i][1] - m)
        elif sign > 0:
            acc[i] = (1, m - acc[i][1])
        else:
            acc[i] = (-1, acc[i][1] + m)


def _total(entry):
    sign, value = entry
    assert sign > 0
    return value


def _layernorm(x):
    m = jnp.mean(x, axis=-1, keepdims=True)
    xc = x - m
    v = jnp.mean(xc * xc, axis=-1, keepdims=True)
    return xc * lax.rsqrt(v + EPS)


def _gelu(x):
    c = math.sqrt(2.0 / math.pi)
    return 0.5 * x * (1.0 + jnp.tanh(x * (c + (c * 0.044715) * (x * x))))


def _store_keys(chains, packed, group, keys):
    kind, idx = SOURCE[group]
    if kind == "v":
        for d in range(DH):
            o = KB0 + (idx * DH + d) * 16
            chains[d % 2][o:o + 16, :] = jnp.broadcast_to(keys[:, d:d + 1], (16, 128))
        return
    packed[KS0 + idx * 8:KS0 + (idx + 1) * 8, :] = pltpu.bitcast(keys.astype(BF), F32)
    first, last = PV_TIMES[-1], PV_TIMES[0]
    if idx >= first:
        o = KX0 + (idx - first) * 8
        packed[o:o + 8, :] = pltpu.bitcast(keys.astype(BF), F32)
    elif idx < last:
        o = KX0 + (NM - first + idx) * 8
        packed[o:o + 8, :] = pltpu.bitcast(pltpu.roll(keys, DH, 1).astype(BF), F32)


def _result_rows(u, j):
    return j % 2, OT0[j % 2] + (u * NJ + j) * (DH + 8)


def _result_stores(u, acc, sums):
    stores = []
    for j in range(NJ):
        c, row = _result_rows(u, j)
        stores.append((c, row + DH, sums[j]))
        for half in range(DH // 8):
            stores.append((c, row + half * 8, acc[half * 8:(half + 1) * 8, j * 128:(j + 1) * 128]))
    return stores


def _pv(packed, t, p):
    vt = pltpu.bitcast(packed[VS0 + t * 8:VS0 + (t + 1) * 8, :], BF)
    return jnp.dot(vt, p.astype(BF), preferred_element_type=F32)


def _carried_row(pos, j):
    return PD0 + (pos * NJ + j) * 16


def _carried_p(even):
    return jnp.concatenate(
        [jnp.concatenate([even[_carried_row(pos, j):_carried_row(pos, j) + 16, :] for j in range(NJ)], axis=1)
         for pos in range(7, -1, -1)], axis=0)


def _carried_acc(even):
    return jnp.concatenate([even[AD0 + j * DH:AD0 + (j + 1) * DH, :] for j in range(NJ)], axis=1)


def _carried_sums(even):
    return [even[LD0 + j * 8:LD0 + (j + 1) * 8, :] for j in range(NJ)]


def _query_row(h, d, j):
    return QB0 + (((h % 2) * DH + d) * NJ + j) * 8


def _broadcast_query(even, u, d, j):
    return jnp.broadcast_to(even[pl.ds(QF0 + (u * NJ + j) * DH + d, 1), :], (8, 128))


def _attention_units(it, chains, packed, zero):
    even = chains[0]
    u0 = it * HU
    ngrp = HU * NM
    pace_base = (PACE0[0] + zero * 8, PACE0[1] + zero * 8)
    queries, sums, accs, probs, scores, first_pv, pv_results = {}, {}, {}, {}, {}, {}, {}
    staged, late = [], []

    def stage_queries(h):
        u = u0 + h if h < HU else jnp.minimum(u0 + h, NU - 1)
        for d in range(DH):
            for j in range(NJ):
                staged.append((d % 2, _query_row(h, d, j), _broadcast_query(even, u, d, j)))
                yield

    def exponentiate(h, key, j, s):
        e = jnp.exp2(s)
        pair = e[0:8] + e[8:16]
        sums[h, j] = sums[h, j] + pair if (h, j) in sums else pair
        t, pos = PLACE[key]
        if h == HU - 1 and t in DEFERRED:
            even[_carried_row(pos, j):_carried_row(pos, j) + 16, :] = e
        else:
            probs[h, key, j] = e
        return e

    partial, count = {}, {}

    def vpu_scores(c):
        for h in range(HU):
            for i in range(NV):
                for j0 in range(0, NJ, 2):
                    for d in range(c, DH, 2):
                        o = KB0 + (i * DH + d) * 16
                        k = chains[c][o:o + 16, :].reshape(2, 8, 128)
                        for j in (j0, j0 + 1):
                            o = _query_row(h, d, j)
                            term = k * chains[c][o:o + 8, :][None]
                            key = (h, i, j)
                            partial[key] = partial[key] + term if key in partial else term
                            count[key] = count.get(key, 0) + 1
                            if count[key] == DH:
                                exponentiate(h, ("v", i), j, partial.pop(key).reshape(16, 128))
                        yield

    pv_at, result_at, pin_at = {}, {}, {}
    for h in range(-1, HU):
        for t, (_, end) in enumerate(TILES):
            if (h == -1 and t not in DEFERRED) or (h == HU - 1 and t in DEFERRED):
                continue
            x = h * NM + end + PV_LAG
            pv_at.setdefault(x, []).append((h, t))
            if t == NTILE - 1:
                result_at[x + STORE_LAG] = h
            if t == 0:
                pin_at[x + STORE_LAG] = h
    cuts = sorted({0, ngrp} | {x for x in pv_at if x < ngrp})
    runs = dict(zip(cuts[:-1], cuts[1:]))

    vpu = (vpu_scores(0), vpu_scores(1))
    vpu_steps = NV * DH
    done, paced = [0, 0], [0, 0]

    def slots(g):
        h, r = divmod(g, NM)
        return h * (NM + NTILE) + r + 1 + sum(1 for _, end in TILES if (end + PV_LAG) % NM <= r)

    def tick(values, slot):
        for c, o, v in staged:
            chains[c][o:o + 8, :] = v
        staged.clear()
        for c in range(2):
            for item in [item for item in late if item[0] == c][:1]:
                late[:] = [other for other in late if other is not item]
                o = item[1] if isinstance(item[1], int) else pl.multiple_of(item[1], 8)
                chains[c][pl.ds(o, 8), :] = item[2]
            if values:
                paced[c] += 1
                o = pl.multiple_of(pace_base[c] + 8 * (paced[c] % NPACE), 8)
                chains[c][pl.ds(o, 8), :] = values[c]
            want = ((2 * (slot + VPU_LEAD) + c + 1) * vpu_steps * 4 + 6 * (NM + NTILE)) // (8 * (NM + NTILE))
            while done[c] < min(want, HU * vpu_steps):
                next(vpu[c])
                done[c] += 1

    staging = {}
    for x in range(-Q_LEAD, ngrp + PV_LAG + EXP_LAG + 32):
        if (x + Q_LEAD) % NM == 0 and (x + Q_LEAD) // NM < HU:
            h = (x + Q_LEAD) // NM
            o = QS0 + (u0 + h) * (NJ * 8)
            queries[h] = pltpu.bitcast(jnp.concatenate(
                [packed[pl.ds(pl.multiple_of(o + j * 8, 8), 8), :] for j in range(NJ)], axis=1), BF)
        for h, t in pv_at.get(x, []):
            if h == -1:
                p = _carried_p(even)
                accs[h] = _carried_acc(even)
            else:
                p = jnp.concatenate([jnp.concatenate([probs.pop((h, key, j)) for j in range(NJ)], axis=1)
                                     for key in reversed(TILES[t][0])], axis=0)
            pv = _pv(packed, t, p)
            pv_results[x] = pv
            accs[h] = pv if t == 0 else accs[h] + pv
            if t == 0:
                first_pv[h] = pv
        if x in pin_at:
            for j in range(NJ):
                late.append((j % 2, PIN0[j % 2] + j * 8, first_pv[pin_at[x]][0:8, j * 128:(j + 1) * 128]))
        if x in result_at:
            h = result_at[x]
            if h == -1:
                late.extend(_result_stores((u0 + NU - 1) % NU, accs[h], _carried_sums(even)))
            else:
                late.extend(_result_stores(u0 + h, accs[h], [sums[h, j] for j in range(NJ)]))
        if x in runs:
            h = x // NM
            if runs[x] > (h + 1) * NM:
                k = pltpu.bitcast(packed[KX0:KX0 + (runs[x] - x) * 8, :], BF)
                s = jnp.dot(k[:, 0:2 * DH], jnp.concatenate([queries[h], queries[h + 1]], axis=0),
                            preferred_element_type=F32)
            else:
                k = pltpu.bitcast(packed[KS0 + (x - h * NM) * 8:KS0 + (runs[x] - h * NM) * 8, :], BF)
                s = jnp.dot(k[:, 0:DH], queries[h], preferred_element_type=F32)
            for g in range(x, runs[x]):
                scores[g] = s[(g - x) * 16:(g - x + 1) * 16]
        g = x - EXP_LAG
        values = None
        if 0 <= g < ngrp:
            if g in pv_results:
                pv = pv_results[g]
                tick((pv[0:8, PACE[0] * 128:(PACE[0] + 1) * 128], pv[8:16, PACE[1] * 128:(PACE[1] + 1) * 128]),
                     slots(g) - 2)
            s = scores.pop(g)
            e = [exponentiate(g // NM, ("m", g % NM), j, s[:, j * 128:(j + 1) * 128]) for j in range(NJ)]
            values = (e[PACE[0]][0:8], e[PACE[1]][8:16])
        tick(values, slots(g) - 1)
        h, r = divmod(x + NM - 14, NM)
        if 1 <= h <= HU:
            if h not in staging:
                staging[h] = [stage_queries(h), 0]
            while staging[h][1] < min(DH * NJ, ((r + 1) * 4) // 5):
                next(staging[h][0])
                staging[h][1] += 1
    for j in range(NJ):
        even[AD0 + j * DH:AD0 + (j + 1) * DH, :] = accs[HU - 1][:, j * 128:(j + 1) * 128]
        even[LD0 + j * 8:LD0 + (j + 1) * 8, :] = sums[HU - 1, j]
    assert not probs and not scores and not staged and not late and not partial


def _kernel(x_hbm, wq_hbm, wkt_hbm, wvt_hbm, wo_hbm, win_hbm, wsp_hbm, bsp_hbm, wout_hbm, c_hbm, wmod_hbm,
            out_hbm,
            even, odd, packed, xz, wq_v, wo_v, win_v, wsp_v, wout_v, wmod_v, wt_s, k_s, x1_s, out_s,
            z2_s, wout_s, gb_s, bias_s, bsp_v, c_v, flags, sems, out_sems):
    chains = (even, odd)
    copies = [
        (wq_hbm, wq_v), (c_hbm, c_v),
        (wkt_hbm, wt_s.at[pl.ds(D, DH)]), (wvt_hbm, wt_s.at[pl.ds(D + DH, DH)]),
        (wmod_hbm.at[pl.ds(0, D // 2), pl.ds(0, 2 * D)], wmod_v.at[pl.ds(0, D // 2), pl.ds(0, 2 * D)]),
        (wmod_hbm.at[pl.ds(D // 2, D // 2), pl.ds(0, 2 * D)], wmod_v.at[pl.ds(D // 2, D // 2), pl.ds(0, 2 * D)]),
        (wmod_hbm.at[:, pl.ds(2 * D, 4 * D)], wmod_v.at[:, pl.ds(2 * D, 4 * D)]),
        (wo_hbm, wo_v), (win_hbm, win_v), (bsp_hbm, bsp_v), (wout_hbm, wout_v), (wsp_hbm, wsp_v),
    ]
    copies += [(x_hbm.at[pl.ds(i * RA, RA)], xz.at[pl.ds(i * RA, RA), pl.ds(0, D)]) for i in range(S // RA)]
    copies = [pltpu.make_async_copy(src, dst, sems.at[i]) for i, (src, dst) in enumerate(copies)]
    cp_wq, cp_c, cp_wk, cp_wv = copies[0:4]
    cp_mod, cp_late, cp_x = copies[4:6], copies[6:12], copies[12:]
    for cp in (cp_wq, cp_c, cp_wk, cp_wv, cp_x[0], *cp_mod, *cp_x[1:]):
        cp.start()

    cp_wq.wait()
    wt_s[0:D, :] = wq_v[...].astype(F32).T.astype(BF)
    cp_wk.wait()
    cp_wv.wait()
    cp_c.wait()
    cond = jnp.broadcast_to(c_v[...].astype(F32), (16, D))
    cond = (cond * jax.nn.sigmoid(cond)).astype(BF)
    cp_x[0].wait()
    first_norm = _layernorm(xz[0:RA, 0:D].astype(F32))
    mod = None
    for i, cp in enumerate(cp_mod):
        cp.wait()
        rows = slice(i * (D // 2), (i + 1) * (D // 2))
        part = jnp.dot(cond[:, rows], wmod_v[rows, 0:2 * D], preferred_element_type=F32)
        mod = part if mod is None else mod + part
    shift_a = mod[0:1, 0:D]
    scale_a = 1.0 + mod[0:1, D:2 * D]

    def modulated(i):
        n = first_norm if i == 0 else _layernorm(xz[i * RA:(i + 1) * RA, 0:D].astype(F32))
        return (n * scale_a + shift_a).astype(BF)

    def project(i, h, stats):
        q_max, k_max, v_max = stats
        kvt = lax.dot_general(wt_s[D:D + 2 * DH, :], h, NT, preferred_element_type=F32)
        qt = lax.dot_general(wt_s[0:D, :], h, NT, preferred_element_type=F32)
        kt = kvt[0:DH].astype(BF).astype(F32)
        vt = kvt[DH:2 * DH].astype(BF)
        v_words = pltpu.bitcast(vt, F32)
        keys = jnp.concatenate([kt, jnp.zeros((128 - DH, RA), F32)], axis=0).T
        k_s[i * RA:(i + 1) * RA, :] = keys[:, 0:DH].astype(BF)
        for g in range(RA // 16):
            _store_keys(chains, packed, i * (RA // 16) + g, keys[g * 16:(g + 1) * 16, :])
        q = (qt * QSCALE).astype(BF)
        qf = q.astype(F32)
        q_words = pltpu.bitcast(q, F32)
        for jj in range(RA // 128):
            t = i * (RA // 128) + jj
            block, j = divmod(t, NJ)
            lanes = slice(jj * 128, (jj + 1) * 128)
            packed[VS0 + t * 8:VS0 + (t + 1) * 8, :] = v_words[:, lanes]
            for head in range(H):
                r = (block * H + head) * NJ + j
                packed[QS0 + r * 8:QS0 + (r + 1) * 8, :] = q_words[head * 8:(head + 1) * 8, lanes]
                even[QF0 + r * DH:QF0 + (r + 1) * DH, :] = qf[head * DH:(head + 1) * DH, lanes]
        q2 = (qf * qf).reshape(H, 2, 8, RA)
        q2 = jnp.max(q2[:, 0] + q2[:, 1], axis=0)
        for j in range(RA // 128):
            q_max = jnp.maximum(q_max, q2[:, j * 128:(j + 1) * 128])
        k_max = jnp.maximum(k_max, jnp.sum(kt * kt, axis=0, keepdims=True))
        v_max = jnp.maximum(v_max, jnp.abs(vt.astype(F32)))
        return q_max, k_max, v_max

    stats = (jnp.zeros((8, 128), F32), jnp.zeros((1, RA), F32), jnp.zeros((DH, RA), F32))
    arrived, hs = 1, {}
    for n, upto in enumerate(X_WAITS):
        while arrived <= upto:
            cp_x[arrived].wait()
            arrived += 1
        last = n == len(X_WAITS) - 1
        if last:
            for cp in cp_late:
                cp.start()
        for i in range(X_WAITS[n - 1] if n else 0, S // RA if last else upto):
            for ahead in (i, i + 1):
                if ahead < arrived and ahead not in hs:
                    hs[ahead] = modulated(ahead)
            stats = project(i, hs[i], stats)
            if (i + 1) * RA == QB:
                even[PD0:LD0, :] = jnp.zeros((LD0 - PD0, 128), F32)
                even[LD0:LD0 + NJ * 8, :] = jnp.ones((NJ * 8, 128), F32)
                for d in range(DH):
                    for j in range(NJ):
                        o = _query_row(0, d, j)
                        chains[d % 2][o:o + 8, :] = _broadcast_query(even, 0, d, j)
    q_max, k_max, v_max = stats
    bound = jnp.max(jnp.sum(q_max, axis=0, keepdims=True)) * jnp.max(k_max)
    v_top = jnp.max(v_max)
    safe = (bound <= SCORE_LIMIT * SCORE_LIMIT) & (v_top <= V_MAX) & (v_top >= V_MIN)
    flags[0] = jnp.where(safe, 0, 1)
    for n in range(1, NFLAGS):
        flags[n] = jnp.minimum(jnp.where(safe, 0, 1), 0)

    @pl.when(safe)
    def _unshifted():
        def body(it, carry):
            _attention_units(it, chains, packed, flags[0])
            return carry

        lax.fori_loop(0, NU // HU, body, 0)

    @pl.when(jnp.logical_not(safe))
    def _shifted_by_row_max():
        def body(it, carry):
            q = pltpu.bitcast(packed[pl.ds(pl.multiple_of(QS0 + it * 8, 8), 8), :], BF)
            s = jnp.dot(k_s[...], q, preferred_element_type=F32)
            e = jnp.exp2(s - jnp.max(s, axis=0, keepdims=True))
            total = jnp.sum(e, axis=0, keepdims=True)
            vt = pltpu.bitcast(jnp.concatenate(
                [packed[VS0 + t * 8:VS0 + (t + 1) * 8, :] for t in range(NTILE)], axis=1), BF)
            o = jnp.dot(vt, e.astype(BF), preferred_element_type=F32)
            o = jnp.concatenate([o, jnp.broadcast_to(total * 0.125, (8, 128))], axis=0)
            for c in range(2):
                chains[c][pl.ds(pl.multiple_of(OT0[c] + it * (DH + 8), 8), DH + 8), :] = o
            return carry

        lax.fori_loop(0, NU * NJ, body, 0)

    for cp in cp_late:
        cp.wait()
    acc = _carried_acc(even) + _pv(packed, NTILE - 1, _carried_p(even))
    for c, o, v in _result_stores(NU - 1 + flags[0], acc, _carried_sums(even)):
        chains[c][pl.ds(pl.multiple_of(o, 8), 8), :] = v

    def modulation(i):
        return jnp.dot(cond, wmod_v[:, i * D:(i + 1) * D], preferred_element_type=F32)[0:8]

    gate_a, shift_b, scale_b = modulation(2)[0:1], modulation(3)[0:1], 1.0 + modulation(4)[0:1]
    gb_s[...] = modulation(5)
    blocks = [wout_v[k * OUT_K:(k + 1) * OUT_K, n * (D // 2):(n + 1) * (D // 2)].astype(F32)
              for k in range(2) for n in range(2)]
    for n, (_, terms, _) in enumerate(STRASSEN):
        if len(terms) > 1:
            wout_s[:, n * (D // 2):(n + 1) * (D // 2)] = _combine(terms, blocks).astype(BF)

    def mix(i):
        rows = slice(i * RC, (i + 1) * RC)
        block, j = divmod(i, NJ)
        heads = []
        for head in range(H):
            c, o = _result_rows(block * H + head, j)
            total = jnp.sum(chains[c][o + DH:o + DH + 8, :], axis=0, keepdims=True)
            r = pltpu.reciprocal(total, approx=True)
            heads.append(chains[c][o:o + DH, :] * (r * (2.0 - total * r)))
        a = _dot(jnp.concatenate(heads, axis=0).T.astype(BF), wo_v[...])
        x1 = xz[rows, 0:D].astype(F32) + gate_a * a
        x1_s[rows, :] = x1
        return (_layernorm(x1) * scale_b + shift_b).astype(BF)

    zero = flags[1]
    h = mix(0)
    for i in range(S // RC):
        rows = pl.ds(pl.multiple_of(i * RC + zero, RC), RC)
        h_next = mix(i + 1) if i + 1 < S // RC else None
        z2 = _gelu(_dot(h, win_v[:, FH:2 * FH]))
        xz[rows, D + FH:D + 2 * FH] = _layernorm(z2).astype(BF)
        z1 = _gelu(_dot(h, win_v[:, 0:FH]))
        xz[rows, D:D + FH] = z1.astype(BF)
        h = h_next
    bias = bsp_v[...].astype(F32)
    for r in range(S // 128):
        bias_s[r * 128:(r + 1) * 128, 0:128] = jnp.broadcast_to(bias[r:r + 1, :], (128, 128)).T

    def out_copy(i):
        rows = pl.ds(pl.multiple_of(i * RD, RD), RD)
        return pltpu.make_async_copy(out_s.at[rows], out_hbm.at[rows], out_sems.at[i])

    quarter = S // 4

    def prepare(it, carry):
        rows = pl.ds(pl.multiple_of(it * quarter, quarter), quarter)
        bias_s[rows, 128:256] = bias_s[rows, 0:128] + _dot(wsp_v[rows, :], xz[:, D + FH + 768:D + 2 * FH])
        for r0 in range(0, RD, 16):
            z = [xz[pl.ds(pl.multiple_of(q * quarter + it * RD + r0, 16), 16), D + FH:D + FH + 768].astype(F32)
                 for q in range(4)]
            part = pl.ds(pl.multiple_of(it * RD + r0, 16), 16)
            for p1, (_, b1, _) in enumerate(STRASSEN):
                y = [_combine(b1, [z[2 * ka + kb][:, (2 * na + nb) * 128:(2 * na + nb + 1) * 128]
                                   for ka in range(2) for na in range(2)])
                     for kb in range(2) for nb in range(2)]
                for p2, (_, b2, _) in enumerate(STRASSEN):
                    n = p1 * 7 + p2
                    if len(b1) * len(b2) > 1:
                        z2_s[part, n * 128:(n + 1) * 128] = _combine(b2, y).astype(BF)
                for kb in range(2):
                    n = 49 + 2 * p1 + kb
                    if len(b1) > 1:
                        z2_s[part, n * 128:(n + 1) * 128] = _combine(
                            b1, [z[2 * ka + kb][:, 512 + na * 128:512 + (na + 1) * 128]
                                 for ka in range(2) for na in range(2)]).astype(BF)
        return carry

    lax.fori_loop(0, quarter // RD, prepare, 0)

    def finish(it, carry):
        rows = [pl.ds(pl.multiple_of(q * quarter + it * RD, RD), RD) for q in range(4)]

        def product(n, terms, width, rhs):
            base = it * RD + flags[2 + n]
            lhs = [wsp_v[pl.ds(pl.multiple_of(q * quarter + base, RD), RD), col:col + width]
                   for _, q, col in terms]
            if len(terms) > 1:
                lhs = [_combine([(sign, i) for i, (sign, _, _) in enumerate(terms)],
                                [block.astype(F32) for block in lhs]).astype(BF)]
            return _dot(lhs[0], rhs)

        def two_levels(p1, p2):
            (a1, b1, _), (a2, b2, _) = STRASSEN[p1], STRASSEN[p2]
            n = p1 * 7 + p2
            if len(b1) * len(b2) > 1:
                rhs = z2_s[:, n * 128:(n + 1) * 128]
            else:
                (ka, na), (kb, nb) = divmod(b1[0][1], 2), divmod(b2[0][1], 2)
                col = D + FH + (2 * na + nb) * 128
                rhs = xz[(2 * ka + kb) * quarter:(2 * ka + kb + 1) * quarter, col:col + 128]
            terms = [(s1 * s2, 2 * (i1 // 2) + i2 // 2, (2 * (i1 % 2) + i2 % 2) * quarter)
                     for s1, i1 in a1 for s2, i2 in a2]
            return product(n, terms, quarter, rhs)

        def one_level(p1, b):
            a1, b1, _ = STRASSEN[p1]
            if len(b1) > 1:
                col = (49 + 2 * p1) * 128
                rhs = jnp.concatenate([z2_s[:, col:col + 128], z2_s[:, col + 128:col + 256]], axis=0)
            else:
                ka, na = divmod(b1[0][1], 2)
                col = D + FH + 512 + na * 128
                rhs = xz[ka * (S // 2):(ka + 1) * (S // 2), col:col + 128]
            terms = [(s1, 2 * (i1 // 2) + b, (i1 % 2) * (S // 2)) for s1, i1 in a1]
            return product(49 + 2 * p1 + b, terms, S // 2, rhs)

        two = [[None] * 4 for _ in range(4)]
        one = [[None] * 4 for _ in range(2)]
        for p1 in (1, 2, 6, 3, 5, 4, 0):
            c1 = STRASSEN[p1][2]
            inner = [None] * 4
            for p2 in (3, 5, 1, 6, 2, 0, 4):
                _scatter(inner, STRASSEN[p2][2], two_levels(p1, p2))
            for k in range(4):
                _scatter(two[k], c1, _total(inner[k]))
            for b in range(2):
                _scatter(one[b], c1, one_level(p1, b))
        ys = []
        for q in range(4):
            a, b = divmod(q, 2)
            parts = [_total(two[2 * b + nb][2 * a + na]) for na in range(2) for nb in range(2)]
            parts += [_total(one[b][2 * a]), _total(one[b][2 * a + 1])]
            bias_q = bias_s[rows[q], 0:128]
            g = jnp.concatenate([part + bias_q for part in parts] + [bias_s[rows[q], 128:256]], axis=1)
            ys.append(xz[rows[q], D:D + FH].astype(F32) * g)
        for b in range(2):
            blocks = [ys[q][:, k * OUT_K:(k + 1) * OUT_K] for q in (b, b + 2) for k in range(2)]
            acc = [None] * 4
            for n in (5, 6, 1, 4, 0, 2, 3):
                a_terms, b_terms, c_terms = STRASSEN[n]
                if len(b_terms) > 1:
                    rhs = wout_s[:, n * (D // 2):(n + 1) * (D // 2)]
                else:
                    k, m = divmod(b_terms[0][1], 2)
                    rhs = wout_v[k * OUT_K:(k + 1) * OUT_K, m * (D // 2):(m + 1) * (D // 2)]
                _scatter(acc, c_terms, _dot(_combine(a_terms, blocks).astype(BF), rhs))
            for n, q in enumerate((b, b + 2)):
                rest = _dot(ys[q][:, 2 * OUT_K:FH].astype(BF), wout_v[2 * OUT_K:FH, :])
                mixed = jnp.concatenate([_total(acc[2 * n]), _total(acc[2 * n + 1])], axis=1) + rest
                out_s[rows[q], :] = (x1_s[rows[q], :] + gb_s[0:1, :] * mixed).astype(BF)
                out_copy(q * (quarter // RD) + it).start()
        return carry

    lax.fori_loop(0, S // 4 // RD, finish, 0)
    for i in range(S // RD):
        out_copy(i).wait()


@jax.jit
def pallas_adaLN_cond__grouped_kv_mqa__mixer_gmlp__prompt_kernel(
    A_x: jax.Array,
    A_wq: jax.Array,
    A_wk: jax.Array,
    A_wv: jax.Array,
    A_wo: jax.Array,
    B_x: jax.Array,
    B_w_in: jax.Array,
    B_w_sp: jax.Array,
    B_b_sp: jax.Array,
    B_w_out: jax.Array,
    c: jax.Array,
    w_mod: jax.Array,
):
    del B_x
    vmem = pltpu.VMEM
    scratch = [
        vmem((_round_rows(PACE0[0] + (NPACE + 2) * 8), 128), F32),
        vmem((_round_rows(PACE0[1] + (NPACE + 2) * 8), 128), F32),
        vmem((_round_rows(QS0 + NU * NJ * 8), 128), F32),
        vmem((S, D + 2 * FH), BF),
        vmem((D, D), BF), vmem((D, D), BF), vmem((D, 2 * FH), BF), vmem((S, S), BF), vmem((FH, D), BF),
        vmem((D, 6 * D), BF), vmem((D + 2 * DH, D), BF), vmem((S, DH), BF),
        vmem((S, D), F32), vmem((S, D), BF),
        vmem((S // 4, (49 + 14) * 128), BF), vmem((OUT_K, 7 * D // 2), BF),
        vmem((8, D), F32), vmem((S, 256), F32),
        vmem((S // 128, 128), BF), vmem((1, D), BF),
        pltpu.SMEM((NFLAGS,), jnp.int32),
        pltpu.SemaphoreType.DMA((12 + S // RA,)), pltpu.SemaphoreType.DMA((S // RD,)),
    ]
    out = pl.pallas_call(
        _kernel,
        out_shape=jax.ShapeDtypeStruct((S, D), BF),
        in_specs=[pl.BlockSpec(memory_space=pl.ANY)] * 11,
        out_specs=pl.BlockSpec(memory_space=pl.ANY),
        scratch_shapes=scratch,
        compiler_params=pltpu.CompilerParams(vmem_limit_bytes=110 * 1024 * 1024),
        name="fused",
    )(A_x.reshape(S, D), A_wq, A_wk.T, A_wv.T, A_wo, B_w_in, B_w_sp, B_b_sp.reshape(S // 128, 128),
      B_w_out, c, w_mod)
    return out.reshape(1, S, D)
```

```python
import math

import jax
import jax.numpy as jnp
from jax import lax
from jax.experimental import pallas as pl
from jax.experimental.pallas import tpu as pltpu

BF = jnp.bfloat16
F32 = jnp.float32
S, D, H, DH, FH = 2048, 512, 32, 16, 896
EPS = 1e-5
QSCALE = DH ** -0.5 * math.log2(math.e)
NT = (((1,), (1,)), ((), ()))

SCORE_LIMIT = 96.0
V_MIN, V_MAX = 2.0 ** -16, 2.0 ** 16

QB = 512
NJ = QB // 128
NU = (S // QB) * H
NTILE = S // 128
RA = 256
X_WAITS = (1, 3, 7)
RC = 128
RD = 128
OUT_K = 384

HU = 8
NV = 19
NM = S // 16 - NV
PV_LAG = 9
EXP_LAG = 9
STORE_LAG = 10
Q_LEAD = 9
VPU_LEAD = 3
VPU_SLOT = -1
DRAIN = 4
PACE = (1, 2)
NPACE = 512
NFLAGS = 66

KB0 = 0
QB0 = KB0 + NV * DH * 16
QF0 = QB0 + 2 * DH * NJ * 8
OT0 = (QF0 + NU * NJ * DH, QF0)
OT_ROWS = (NU + 1) * NJ * (DH + 8)
PD0 = OT0[0] + OT_ROWS
AD0 = PD0 + 8 * NJ * 16
LD0 = AD0 + NJ * DH
PIN0 = (LD0 + NJ * 8, OT0[1] + OT_ROWS)
PACE0 = (PIN0[0] + NJ * 8, PIN0[1] + NJ * 8)
KS0 = 0
KX0 = KS0 + NM * 8
VS0 = KX0 + 16 * 8
QS0 = VS0 + NTILE * 8


def _round_rows(rows):
    return -(-rows // 32) * 32


def _plan_tiles():
    events = [((m + 1) * NV, 0, "m", m) for m in range(NM)]
    events += [((i + 1) * NM + VPU_SLOT * NV, 1, "v", i) for i in range(NV)]
    events.sort()
    tiles = []
    for t in range(NTILE):
        part = events[8 * t:8 * t + 8]
        tiles.append(([e[2:] for e in part], -(-max(e[0] for e in part) // NV)))
    return tiles


TILES = _plan_tiles()
PLACE = {key: (t, pos) for t, (keys, _) in enumerate(TILES) for pos, key in enumerate(keys)}
SOURCE = {8 * t + 7 - pos: key for key, (t, pos) in PLACE.items()}
PV_TIMES = sorted({(end + PV_LAG) % NM for _, end in TILES})
DEFERRED = [t for t, (_, end) in enumerate(TILES) if end + PV_LAG >= NM + DRAIN]
assert DEFERRED == [NTILE - 1] and PV_TIMES[0] > 0


STRASSEN = (
    (((1, 0),), ((1, 1), (-1, 3)), ((1, 1), (1, 3))),
    (((1, 0), (1, 1)), ((1, 3),), ((-1, 0), (1, 1))),
    (((1, 0), (1, 3)), ((1, 0), (1, 3)), ((1, 0), (1, 3))),
    (((1, 2), (1, 3)), ((1, 0),), ((1, 2), (-1, 3))),
    (((1, 2), (-1, 0)), ((1, 0), (1, 1)), ((1, 3),)),
    (((1, 3),), ((1, 2), (-1, 0)), ((1, 0), (1, 2))),
    (((1, 1), (-1, 3)), ((1, 2), (1, 3)), ((1, 0),)),
)


def _dot(a, b):
    return jnp.dot(a, b, preferred_element_type=F32)


def _combine(terms, blocks):
    out = blocks[terms[0][1]]
    for sign, i in terms[1:]:
        out = out + blocks[i] if sign > 0 else out - blocks[i]
    return out


def _scatter(acc, terms, m):
    for sign, i in terms:
        if acc[i] is None:
            acc[i] = (sign, m)
        elif acc[i][0] > 0:
            acc[i] = (1, acc[i][1] + m if sign > 0 else acc[i][1] - m)
        elif sign > 0:
            acc[i] = (1, m - acc[i][1])
        else:
            acc[i] = (-1, acc[i][1] + m)


def _total(entry):
    sign, value = entry
    assert sign > 0
    return value


def _layernorm(x):
    m = jnp.mean(x, axis=-1, keepdims=True)
    xc = x - m
    v = jnp.mean(xc * xc, axis=-1, keepdims=True)
    return xc * lax.rsqrt(v + EPS)


def _gelu(x):
    c = math.sqrt(2.0 / math.pi)
    return 0.5 * x * (1.0 + jnp.tanh(x * (c + (c * 0.044715) * (x * x))))


def _store_keys(chains, packed, group, keys):
    kind, idx = SOURCE[group]
    if kind == "v":
        for d in range(DH):
            o = KB0 + (idx * DH + d) * 16
            chains[d % 2][o:o + 16, :] = jnp.broadcast_to(keys[:, d:d + 1], (16, 128))
        return
    packed[KS0 + idx * 8:KS0 + (idx + 1) * 8, :] = pltpu.bitcast(keys.astype(BF), F32)
    first, last = PV_TIMES[-1], PV_TIMES[0]
    if idx >= first:
        o = KX0 + (idx - first) * 8
        packed[o:o + 8, :] = pltpu.bitcast(keys.astype(BF), F32)
    elif idx < last:
        o = KX0 + (NM - first + idx) * 8
        packed[o:o + 8, :] = pltpu.bitcast(pltpu.roll(keys, DH, 1).astype(BF), F32)


def _result_rows(u, j):
    return j % 2, OT0[j % 2] + (u * NJ + j) * (DH + 8)


def _result_stores(u, acc, sums):
    stores = []
    for j in range(NJ):
        c, row = _result_rows(u, j)
        stores.append((c, row + DH, sums[j]))
        for half in range(DH // 8):
            stores.append((c, row + half * 8, acc[half * 8:(half + 1) * 8, j * 128:(j + 1) * 128]))
    return stores


def _pv(packed, t, p):
    vt = pltpu.bitcast(packed[VS0 + t * 8:VS0 + (t + 1) * 8, :], BF)
    return jnp.dot(vt, p.astype(BF), preferred_element_type=F32)


def _carried_row(pos, j):
    return PD0 + (pos * NJ + j) * 16


def _carried_p(even):
    return jnp.concatenate(
        [jnp.concatenate([even[_carried_row(pos, j):_carried_row(pos, j) + 16, :] for j in range(NJ)], axis=1)
         for pos in range(7, -1, -1)], axis=0)


def _carried_acc(even):
    return jnp.concatenate([even[AD0 + j * DH:AD0 + (j + 1) * DH, :] for j in range(NJ)], axis=1)


def _carried_sums(even):
    return [even[LD0 + j * 8:LD0 + (j + 1) * 8, :] for j in range(NJ)]


def _query_row(h, d, j):
    return QB0 + (((h % 2) * DH + d) * NJ + j) * 8


def _broadcast_query(even, u, d, j):
    return jnp.broadcast_to(even[pl.ds(QF0 + (u * NJ + j) * DH + d, 1), :], (8, 128))


def _attention_units(it, chains, packed, zero):
    even = chains[0]
    u0 = it * HU
    ngrp = HU * NM
    pace_base = (PACE0[0] + zero * 8, PACE0[1] + zero * 8)
    queries, sums, accs, probs, scores, first_pv, pv_results = {}, {}, {}, {}, {}, {}, {}
    staged, late = [], []

    def stage_queries(h):
        u = u0 + h if h < HU else jnp.minimum(u0 + h, NU - 1)
        for d in range(DH):
            for j in range(NJ):
                staged.append((d % 2, _query_row(h, d, j), _broadcast_query(even, u, d, j)))
                yield

    def exponentiate(h, key, j, s):
        e = jnp.exp2(s)
        pair = e[0:8] + e[8:16]
        sums[h, j] = sums[h, j] + pair if (h, j) in sums else pair
        t, pos = PLACE[key]
        if h == HU - 1 and t in DEFERRED:
            even[_carried_row(pos, j):_carried_row(pos, j) + 16, :] = e
        else:
            probs[h, key, j] = e
        return e

    partial, count = {}, {}

    def vpu_scores(c):
        for h in range(HU):
            for i in range(NV):
                for j0 in range(0, NJ, 2):
                    for d in range(c, DH, 2):
                        o = KB0 + (i * DH + d) * 16
                        k = chains[c][o:o + 16, :].reshape(2, 8, 128)
                        for j in (j0, j0 + 1):
                            o = _query_row(h, d, j)
                            term = k * chains[c][o:o + 8, :][None]
                            key = (h, i, j)
                            partial[key] = partial[key] + term if key in partial else term
                            count[key] = count.get(key, 0) + 1
                            if count[key] == DH:
                                exponentiate(h, ("v", i), j, partial.pop(key).reshape(16, 128))
                        yield

    pv_at, result_at, pin_at = {}, {}, {}
    for h in range(-1, HU):
        for t, (_, end) in enumerate(TILES):
            if (h == -1 and t not in DEFERRED) or (h == HU - 1 and t in DEFERRED):
                continue
            x = h * NM + end + PV_LAG
            pv_at.setdefault(x, []).append((h, t))
            if t == NTILE - 1:
                result_at[x + STORE_LAG] = h
            if t == 0:
                pin_at[x + STORE_LAG] = h
    cuts = sorted({0, ngrp} | {x for x in pv_at if x < ngrp})
    runs = dict(zip(cuts[:-1], cuts[1:]))

    vpu = (vpu_scores(0), vpu_scores(1))
    vpu_steps = NV * DH
    done, paced = [0, 0], [0, 0]

    def slots(g):
        h, r = divmod(g, NM)
        return h * (NM + NTILE) + r + 1 + sum(1 for _, end in TILES if (end + PV_LAG) % NM <= r)

    def tick(values, slot):
        for c, o, v in staged:
            chains[c][o:o + 8, :] = v
        staged.clear()
        for c in range(2):
            for item in [item for item in late if item[0] == c][:1]:
                late[:] = [other for other in late if other is not item]
                o = item[1] if isinstance(item[1], int) else pl.multiple_of(item[1], 8)
                chains[c][pl.ds(o, 8), :] = item[2]
            if values:
                paced[c] += 1
                o = pl.multiple_of(pace_base[c] + 8 * (paced[c] % NPACE), 8)
                chains[c][pl.ds(o, 8), :] = values[c]
            want = ((2 * (slot + VPU_LEAD) + c + 1) * vpu_steps * 4 + 6 * (NM + NTILE)) // (8 * (NM + NTILE))
            while done[c] < min(want, HU * vpu_steps):
                next(vpu[c])
                done[c] += 1

    staging = {}
    for x in range(-Q_LEAD, ngrp + PV_LAG + EXP_LAG + 32):
        if (x + Q_LEAD) % NM == 0 and (x + Q_LEAD) // NM < HU:
            h = (x + Q_LEAD) // NM
            o = QS0 + (u0 + h) * (NJ * 8)
            queries[h] = pltpu.bitcast(jnp.concatenate(
                [packed[pl.ds(pl.multiple_of(o + j * 8, 8), 8), :] for j in range(NJ)], axis=1), BF)
        for h, t in pv_at.get(x, []):
            if h == -1:
                p = _carried_p(even)
                accs[h] = _carried_acc(even)
            else:
                p = jnp.concatenate([jnp.concatenate([probs.pop((h, key, j)) for j in range(NJ)], axis=1)
                                     for key in reversed(TILES[t][0])], axis=0)
            pv = _pv(packed, t, p)
            pv_results[x] = pv
            accs[h] = pv if t == 0 else accs[h] + pv
            if t == 0:
                first_pv[h] = pv
        if x in pin_at:
            for j in range(NJ):
                late.append((j % 2, PIN0[j % 2] + j * 8, first_pv[pin_at[x]][0:8, j * 128:(j + 1) * 128]))
        if x in result_at:
            h = result_at[x]
            if h == -1:
                late.extend(_result_stores((u0 + NU - 1) % NU, accs[h], _carried_sums(even)))
            else:
                late.extend(_result_stores(u0 + h, accs[h], [sums[h, j] for j in range(NJ)]))
        if x in runs:
            h = x // NM
            if runs[x] > (h + 1) * NM:
                k = pltpu.bitcast(packed[KX0:KX0 + (runs[x] - x) * 8, :], BF)
                s = jnp.dot(k[:, 0:2 * DH], jnp.concatenate([queries[h], queries[h + 1]], axis=0),
                            preferred_element_type=F32)
            else:
                k = pltpu.bitcast(packed[KS0 + (x - h * NM) * 8:KS0 + (runs[x] - h * NM) * 8, :], BF)
                s = jnp.dot(k[:, 0:DH], queries[h], preferred_element_type=F32)
            for g in range(x, runs[x]):
                scores[g] = s[(g - x) * 16:(g - x + 1) * 16]
        g = x - EXP_LAG
        values = None
        if 0 <= g < ngrp:
            if g in pv_results:
                pv = pv_results[g]
                tick((pv[0:8, PACE[0] * 128:(PACE[0] + 1) * 128], pv[8:16, PACE[1] * 128:(PACE[1] + 1) * 128]),
                     slots(g) - 2)
            s = scores.pop(g)
            e = [exponentiate(g // NM, ("m", g % NM), j, s[:, j * 128:(j + 1) * 128]) for j in range(NJ)]
            values = (e[PACE[0]][0:8], e[PACE[1]][8:16])
        tick(values, slots(g) - 1)
        h, r = divmod(x + NM - 14, NM)
        if 1 <= h <= HU:
            if h not in staging:
                staging[h] = [stage_queries(h), 0]
            while staging[h][1] < min(DH * NJ, ((r + 1) * 4) // 5):
                next(staging[h][0])
                staging[h][1] += 1
    for j in range(NJ):
        even[AD0 + j * DH:AD0 + (j + 1) * DH, :] = accs[HU - 1][:, j * 128:(j + 1) * 128]
        even[LD0 + j * 8:LD0 + (j + 1) * 8, :] = sums[HU - 1, j]
    assert not probs and not scores and not staged and not late and not partial


def _kernel(x_hbm, wq_hbm, wkt_hbm, wvt_hbm, wo_hbm, win_hbm, wsp_hbm, bsp_hbm, wout_hbm, c_hbm, wmod_hbm,
            out_hbm,
            even, odd, packed, xz, wq_v, wo_v, win_v, wsp_v, wout_v, wmod_v, wt_s, k_s, x1_s, out_s,
            z2_s, wout_s, gb_s, bias_s, bsp_v, c_v, flags, sems, out_sems):
    chains = (even, odd)
    copies = [
        (wq_hbm, wq_v), (c_hbm, c_v),
        (wkt_hbm, wt_s.at[pl.ds(D, DH)]), (wvt_hbm, wt_s.at[pl.ds(D + DH, DH)]),
        (wmod_hbm.at[pl.ds(0, D // 2), pl.ds(0, 2 * D)], wmod_v.at[pl.ds(0, D // 2), pl.ds(0, 2 * D)]),
        (wmod_hbm.at[pl.ds(D // 2, D // 2), pl.ds(0, 2 * D)], wmod_v.at[pl.ds(D // 2, D // 2), pl.ds(0, 2 * D)]),
        (wmod_hbm.at[:, pl.ds(2 * D, 4 * D)], wmod_v.at[:, pl.ds(2 * D, 4 * D)]),
        (wo_hbm, wo_v), (win_hbm, win_v), (bsp_hbm, bsp_v), (wout_hbm, wout_v), (wsp_hbm, wsp_v),
    ]
    copies += [(x_hbm.at[pl.ds(i * RA, RA)], xz.at[pl.ds(i * RA, RA), pl.ds(0, D)]) for i in range(S // RA)]
    copies = [pltpu.make_async_copy(src, dst, sems.at[i]) for i, (src, dst) in enumerate(copies)]
    cp_wq, cp_c, cp_wk, cp_wv = copies[0:4]
    cp_mod, cp_late, cp_x = copies[4:6], copies[6:12], copies[12:]
    for cp in (cp_wq, cp_c, cp_wk, cp_wv, cp_x[0], *cp_mod, *cp_x[1:]):
        cp.start()

    cp_wq.wait()
    wt_s[0:D, :] = wq_v[...].astype(F32).T.astype(BF)
    cp_wk.wait()
    cp_wv.wait()
    cp_c.wait()
    cond = jnp.broadcast_to(c_v[...].astype(F32), (16, D))
    cond = (cond * jax.nn.sigmoid(cond)).astype(BF)
    cp_x[0].wait()
    first_norm = _layernorm(xz[0:RA, 0:D].astype(F32))
    mod = None
    for i, cp in enumerate(cp_mod):
        cp.wait()
        rows = slice(i * (D // 2), (i + 1) * (D // 2))
        part = jnp.dot(cond[:, rows], wmod_v[rows, 0:2 * D], preferred_element_type=F32)
        mod = part if mod is None else mod + part
    shift_a = mod[0:1, 0:D]
    scale_a = 1.0 + mod[0:1, D:2 * D]

    def modulated(i):
        n = first_norm if i == 0 else _layernorm(xz[i * RA:(i + 1) * RA, 0:D].astype(F32))
        return (n * scale_a + shift_a).astype(BF)

    def project(i, h, stats):
        q_max, k_max, v_max = stats
        kvt = lax.dot_general(wt_s[D:D + 2 * DH, :], h, NT, preferred_element_type=F32)
        qt = lax.dot_general(wt_s[0:D, :], h, NT, preferred_element_type=F32)
        kt = kvt[0:DH].astype(BF).astype(F32)
        vt = kvt[DH:2 * DH].astype(BF)
        v_words = pltpu.bitcast(vt, F32)
        keys = jnp.concatenate([kt, jnp.zeros((128 - DH, RA), F32)], axis=0).T
        k_s[i * RA:(i + 1) * RA, :] = keys[:, 0:DH].astype(BF)
        for g in range(RA // 16):
            _store_keys(chains, packed, i * (RA // 16) + g, keys[g * 16:(g + 1) * 16, :])
        q = (qt * QSCALE).astype(BF)
        qf = q.astype(F32)
        q_words = pltpu.bitcast(q, F32)
        for jj in range(RA // 128):
            t = i * (RA // 128) + jj
            block, j = divmod(t, NJ)
            lanes = slice(jj * 128, (jj + 1) * 128)
            packed[VS0 + t * 8:VS0 + (t + 1) * 8, :] = v_words[:, lanes]
            for head in range(H):
                r = (block * H + head) * NJ + j
                packed[QS0 + r * 8:QS0 + (r + 1) * 8, :] = q_words[head * 8:(head + 1) * 8, lanes]
                even[QF0 + r * DH:QF0 + (r + 1) * DH, :] = qf[head * DH:(head + 1) * DH, lanes]
        q2 = (qf * qf).reshape(H, 2, 8, RA)
        q2 = jnp.max(q2[:, 0] + q2[:, 1], axis=0)
        for j in range(RA // 128):
            q_max = jnp.maximum(q_max, q2[:, j * 128:(j + 1) * 128])
        k_max = jnp.maximum(k_max, jnp.sum(kt * kt, axis=0, keepdims=True))
        v_max = jnp.maximum(v_max, jnp.abs(vt.astype(F32)))
        return q_max, k_max, v_max

    stats = (jnp.zeros((8, 128), F32), jnp.zeros((1, RA), F32), jnp.zeros((DH, RA), F32))
    arrived, hs = 1, {}
    for n, upto in enumerate(X_WAITS):
        while arrived <= upto:
            cp_x[arrived].wait()
            arrived += 1
        last = n == len(X_WAITS) - 1
        if last:
            for cp in cp_late:
                cp.start()
        for i in range(X_WAITS[n - 1] if n else 0, S // RA if last else upto):
            for ahead in (i, i + 1):
                if ahead < arrived and ahead not in hs:
                    hs[ahead] = modulated(ahead)
            stats = project(i, hs[i], stats)
            if (i + 1) * RA == QB:
                even[PD0:LD0, :] = jnp.zeros((LD0 - PD0, 128), F32)
                even[LD0:LD0 + NJ * 8, :] = jnp.ones((NJ * 8, 128), F32)
                for d in range(DH):
                    for j in range(NJ):
                        o = _query_row(0, d, j)
                        chains[d % 2][o:o + 8, :] = _broadcast_query(even, 0, d, j)
    q_max, k_max, v_max = stats
    bound = jnp.max(jnp.sum(q_max, axis=0, keepdims=True)) * jnp.max(k_max)
    v_top = jnp.max(v_max)
    safe = (bound <= SCORE_LIMIT * SCORE_LIMIT) & (v_top <= V_MAX) & (v_top >= V_MIN)
    flags[0] = jnp.where(safe, 0, 1)
    for n in range(1, NFLAGS):
        flags[n] = jnp.minimum(jnp.where(safe, 0, 1), 0)

    @pl.when(safe)
    def _unshifted():
        def body(it, carry):
            _attention_units(it, chains, packed, flags[0])
            return carry

        lax.fori_loop(0, NU // HU, body, 0)

    @pl.when(jnp.logical_not(safe))
    def _shifted_by_row_max():
        def body(it, carry):
            q = pltpu.bitcast(packed[pl.ds(pl.multiple_of(QS0 + it * 8, 8), 8), :], BF)
            s = jnp.dot(k_s[...], q, preferred_element_type=F32)
            e = jnp.exp2(s - jnp.max(s, axis=0, keepdims=True))
            total = jnp.sum(e, axis=0, keepdims=True)
            vt = pltpu.bitcast(jnp.concatenate(
                [packed[VS0 + t * 8:VS0 + (t + 1) * 8, :] for t in range(NTILE)], axis=1), BF)
            o = jnp.dot(vt, e.astype(BF), preferred_element_type=F32)
            o = jnp.concatenate([o, jnp.broadcast_to(total * 0.125, (8, 128))], axis=0)
            for c in range(2):
                chains[c][pl.ds(pl.multiple_of(OT0[c] + it * (DH + 8), 8), DH + 8), :] = o
            return carry

        lax.fori_loop(0, NU * NJ, body, 0)

    for cp in cp_late:
        cp.wait()
    acc = _carried_acc(even) + _pv(packed, NTILE - 1, _carried_p(even))
    for c, o, v in _result_stores(NU - 1 + flags[0], acc, _carried_sums(even)):
        chains[c][pl.ds(pl.multiple_of(o, 8), 8), :] = v

    def modulation(i):
        return jnp.dot(cond, wmod_v[:, i * D:(i + 1) * D], preferred_element_type=F32)[0:8]

    gate_a, shift_b, scale_b = modulation(2)[0:1], modulation(3)[0:1], 1.0 + modulation(4)[0:1]
    gb_s[...] = modulation(5)
    blocks = [wout_v[k * OUT_K:(k + 1) * OUT_K, n * (D // 2):(n + 1) * (D // 2)].astype(F32)
              for k in range(2) for n in range(2)]
    for n, (_, terms, _) in enumerate(STRASSEN):
        if len(terms) > 1:
            wout_s[:, n * (D // 2):(n + 1) * (D // 2)] = _combine(terms, blocks).astype(BF)

    def mix(i):
        rows = slice(i * RC, (i + 1) * RC)
        block, j = divmod(i, NJ)
        heads = []
        for head in range(H):
            c, o = _result_rows(block * H + head, j)
            total = jnp.sum(chains[c][o + DH:o + DH + 8, :], axis=0, keepdims=True)
            r = pltpu.reciprocal(total, approx=True)
            heads.append(chains[c][o:o + DH, :] * (r * (2.0 - total * r)))
        a = _dot(jnp.concatenate(heads, axis=0).T.astype(BF), wo_v[...])
        x1 = xz[rows, 0:D].astype(F32) + gate_a * a
        x1_s[rows, :] = x1
        return (_layernorm(x1) * scale_b + shift_b).astype(BF)

    zero = flags[1]
    h = mix(0)
    for i in range(S // RC):
        rows = pl.ds(pl.multiple_of(i * RC + zero, RC), RC)
        h_next = mix(i + 1) if i + 1 < S // RC else None
        z2 = _gelu(_dot(h, win_v[:, FH:2 * FH]))
        xz[rows, D + FH:D + 2 * FH] = _layernorm(z2).astype(BF)
        z1 = _gelu(_dot(h, win_v[:, 0:FH]))
        xz[rows, D:D + FH] = z1.astype(BF)
        h = h_next
    bias = bsp_v[...].astype(F32)
    for r in range(S // 128):
        bias_s[r * 128:(r + 1) * 128, 0:128] = jnp.broadcast_to(bias[r:r + 1, :], (128, 128)).T

    def out_copy(i):
        rows = pl.ds(pl.multiple_of(i * RD, RD), RD)
        return pltpu.make_async_copy(out_s.at[rows], out_hbm.at[rows], out_sems.at[i])

    quarter = S // 4

    def prepare(it, carry):
        rows = pl.ds(pl.multiple_of(it * quarter, quarter), quarter)
        bias_s[rows, 128:256] = bias_s[rows, 0:128] + _dot(wsp_v[rows, :], xz[:, D + FH + 768:D + 2 * FH])
        for r0 in range(0, RD, 16):
            z = [xz[pl.ds(pl.multiple_of(q * quarter + it * RD + r0, 16), 16), D + FH:D + FH + 512].astype(F32)
                 for q in range(4)]
            part = pl.ds(pl.multiple_of(it * RD + r0, 16), 16)
            for p1, (_, b1, _) in enumerate(STRASSEN):
                y = [_combine(b1, [z[2 * ka + kb][:, (2 * na + nb) * 128:(2 * na + nb + 1) * 128]
                                   for ka in range(2) for na in range(2)])
                     for kb in range(2) for nb in range(2)]
                for p2, (_, b2, _) in enumerate(STRASSEN):
                    n = p1 * 7 + p2
                    if len(b1) * len(b2) > 1:
                        z2_s[part, n * 128:(n + 1) * 128] = _combine(b2, y).astype(BF)
        return carry

    lax.fori_loop(0, quarter // RD, prepare, 0)

    def finish(it, carry):
        rows = [pl.ds(pl.multiple_of(q * quarter + it * RD, RD), RD) for q in range(4)]

        def product(n, terms, width, rhs):
            base = it * RD + flags[2 + n]
            lhs = [wsp_v[pl.ds(pl.multiple_of(q * quarter + base, RD), RD), col:col + width]
                   for _, q, col in terms]
            if len(terms) > 1:
                lhs = [_combine([(sign, i) for i, (sign, _, _) in enumerate(terms)],
                                [block.astype(F32) for block in lhs]).astype(BF)]
            return _dot(lhs[0], rhs)

        def two_levels(p1, p2):
            (a1, b1, _), (a2, b2, _) = STRASSEN[p1], STRASSEN[p2]
            n = p1 * 7 + p2
            if len(b1) * len(b2) > 1:
                rhs = z2_s[:, n * 128:(n + 1) * 128]
            else:
                (ka, na), (kb, nb) = divmod(b1[0][1], 2), divmod(b2[0][1], 2)
                col = D + FH + (2 * na + nb) * 128
                rhs = xz[(2 * ka + kb) * quarter:(2 * ka + kb + 1) * quarter, col:col + 128]
            terms = [(s1 * s2, 2 * (i1 // 2) + i2 // 2, (2 * (i1 % 2) + i2 % 2) * quarter)
                     for s1, i1 in a1 for s2, i2 in a2]
            return product(n, terms, quarter, rhs)

        shared = {}

        def one_level(p1, b):
            a1, b1, _ = STRASSEN[p1]
            if len(b1) > 1:
                if b == 0:
                    blocks = {i: xz[pl.ds(pl.multiple_of((i // 2) * (S // 2) + flags[2 + p1], S // 2), S // 2),
                                    D + FH + 512 + (i % 2) * 128:D + FH + 640 + (i % 2) * 128].astype(F32)
                              for _, i in b1}
                    shared[p1] = _combine(b1, blocks).astype(BF)
                rhs = shared[p1]
            else:
                ka, na = divmod(b1[0][1], 2)
                col = D + FH + 512 + na * 128
                rhs = xz[ka * (S // 2):(ka + 1) * (S // 2), col:col + 128]
            terms = [(s1, 2 * (i1 // 2) + b, (i1 % 2) * (S // 2)) for s1, i1 in a1]
            return product(49 + 2 * p1 + b, terms, S // 2, rhs)

        two = [[None] * 4 for _ in range(4)]
        one = [[None] * 4 for _ in range(2)]
        for p1 in (1, 2, 6, 3, 5, 4, 0):
            c1 = STRASSEN[p1][2]
            inner = [None] * 4
            for p2 in (3, 5, 1, 6, 2, 4, 0):
                _scatter(inner, STRASSEN[p2][2], two_levels(p1, p2))
            for k in range(4):
                _scatter(two[k], c1, _total(inner[k]))
            for b in range(2):
                _scatter(one[b], c1, one_level(p1, b))
        ys = []
        for q in range(4):
            a, b = divmod(q, 2)
            parts = [_total(two[2 * b + nb][2 * a + na]) for na in range(2) for nb in range(2)]
            parts += [_total(one[b][2 * a]), _total(one[b][2 * a + 1])]
            bias_q = bias_s[rows[q], 0:128]
            g = jnp.concatenate([part + bias_q for part in parts] + [bias_s[rows[q], 128:256]], axis=1)
            ys.append(xz[rows[q], D:D + FH].astype(F32) * g)
        for b in range(2):
            blocks = [ys[q][:, k * OUT_K:(k + 1) * OUT_K] for q in (b, b + 2) for k in range(2)]
            acc = [None] * 4
            for n in (5, 6, 1, 4, 0, 2, 3):
                a_terms, b_terms, c_terms = STRASSEN[n]
                if len(b_terms) > 1:
                    rhs = wout_s[:, n * (D // 2):(n + 1) * (D // 2)]
                else:
                    k, m = divmod(b_terms[0][1], 2)
                    rhs = wout_v[k * OUT_K:(k + 1) * OUT_K, m * (D // 2):(m + 1) * (D // 2)]
                _scatter(acc, c_terms, _dot(_combine(a_terms, blocks).astype(BF), rhs))
            for n, q in enumerate((b, b + 2)):
                rest = _dot(ys[q][:, 2 * OUT_K:FH].astype(BF), wout_v[2 * OUT_K:FH, :])
                mixed = jnp.concatenate([_total(acc[2 * n]), _total(acc[2 * n + 1])], axis=1) + rest
                out_s[rows[q], :] = (x1_s[rows[q], :] + gb_s[0:1, :] * mixed).astype(BF)
                out_copy(q * (quarter // RD) + it).start()
        return carry

    lax.fori_loop(0, S // 4 // RD, finish, 0)
    for i in range(S // RD):
        out_copy(i).wait()


@jax.jit
def pallas_adaLN_cond__grouped_kv_mqa__mixer_gmlp__prompt_kernel(
    A_x: jax.Array,
    A_wq: jax.Array,
    A_wk: jax.Array,
    A_wv: jax.Array,
    A_wo: jax.Array,
    B_x: jax.Array,
    B_w_in: jax.Array,
    B_w_sp: jax.Array,
    B_b_sp: jax.Array,
    B_w_out: jax.Array,
    c: jax.Array,
    w_mod: jax.Array,
):
    del B_x
    vmem = pltpu.VMEM
    scratch = [
        vmem((_round_rows(PACE0[0] + (NPACE + 2) * 8), 128), F32),
        vmem((_round_rows(PACE0[1] + (NPACE + 2) * 8), 128), F32),
        vmem((_round_rows(QS0 + NU * NJ * 8), 128), F32),
        vmem((S, D + 2 * FH), BF),
        vmem((D, D), BF), vmem((D, D), BF), vmem((D, 2 * FH), BF), vmem((S, S), BF), vmem((FH, D), BF),
        vmem((D, 6 * D), BF), vmem((D + 2 * DH, D), BF), vmem((S, DH), BF),
        vmem((S, D), F32), vmem((S, D), BF),
        vmem((S // 4, 49 * 128), BF), vmem((OUT_K, 7 * D // 2), BF),
        vmem((8, D), F32), vmem((S, 256), F32),
        vmem((S // 128, 128), BF), vmem((1, D), BF),
        pltpu.SMEM((NFLAGS,), jnp.int32),
        pltpu.SemaphoreType.DMA((12 + S // RA,)), pltpu.SemaphoreType.DMA((S // RD,)),
    ]
    out = pl.pallas_call(
        _kernel,
        out_shape=jax.ShapeDtypeStruct((S, D), BF),
        in_specs=[pl.BlockSpec(memory_space=pl.ANY)] * 11,
        out_specs=pl.BlockSpec(memory_space=pl.ANY),
        scratch_shapes=scratch,
        compiler_params=pltpu.CompilerParams(vmem_limit_bytes=110 * 1024 * 1024),
        name="fused",
    )(A_x.reshape(S, D), A_wq, A_wk.T, A_wv.T, A_wo, B_w_in, B_w_sp, B_b_sp.reshape(S // 128, 128),
      B_w_out, c, w_mod)
    return out.reshape(1, S, D)
```
